```python
import jax
import jax.numpy as jnp

def _softmax(x, axis=-1):
    return jax.nn.softmax(x, axis=axis)

def _gelu(x):
    return jax.nn.gelu(x, approximate=True)

def _silu(x):
    return jax.nn.silu(x)

def _sigmoid(x):
    return jax.nn.sigmoid(x)

def _layernorm(x, axis=-1, eps=1e-05):
    m = jnp.mean(x, axis=axis, keepdims=True)
    v = jnp.var(x, axis=axis, keepdims=True)
    return (x - m) / jnp.sqrt(v + eps)

def _scatter_add(tgt, idx, src, axis=0):
    return tgt.at[idx].add(src)

def _segment_sum(src, seg, n):
    return jax.ops.segment_sum(src, seg, n)

class _Rng:

    def __init__(self, key):
        self._k = key

    def _next(self):
        self._k, sub = jax.random.split(self._k)
        return sub

    def normal(self, shape):
        return jax.random.normal(self._next(), shape, dtype=jnp.bfloat16)

    def randint(self, lo, hi, shape):
        return jax.random.randint(self._next(), shape, lo, hi, dtype=jnp.int32)

    def uniform(self, shape, lo=0.0, hi=1.0):
        return jax.random.uniform(self._next(), shape, jnp.bfloat16, lo, hi)

    def permutation(self, n):
        return jax.random.permutation(self._next(), n)
kernel_name = 'adaLN_cond__memory_aug_recurrent_mem_tr__mixer_s_mlp__prompt'

def setup_inputs():
    _rng = _Rng(jax.random.key(int.from_bytes(__import__("os").urandom(4), "little")))
    _w = lambda a: (lambda t: t.astype(jnp.bfloat16) if jnp.issubdtype(t.dtype, jnp.floating) else t)(jnp.asarray(a))

    def _A_setup():
        B, S, Dm = (1, 2048, 1024)
        H, Dh = (32, 128)
        M, seg = (8, 32)
        seg = min(seg, S)
        S = S // seg * seg
        return {'x': _w((lambda *s: _rng.normal(s) * 0.05)(B, S, Dm)), 'mem0': _w((lambda *s: _rng.normal(s) * 0.05)(B, M, Dm)), 'Wq': _w((lambda *s: _rng.normal(s) * 0.05)(Dm, H, Dh) * Dm ** (-0.5)), 'Wk': _w((lambda *s: _rng.normal(s) * 0.05)(Dm, H, Dh) * Dm ** (-0.5)), 'Wv': _w((lambda *s: _rng.normal(s) * 0.05)(Dm, H, Dh) * Dm ** (-0.5)), 'Wo': _w((lambda *s: _rng.normal(s) * 0.05)(H, Dh, Dm) * (H * Dh) ** (-0.5)), 'seg_len': seg}
    _A_in = _A_setup()

    def _B_setup():
        B, S, D, F = (1, 2048, 1024, 3584)
        return {'x': _w((lambda *s: _rng.normal(s) * 0.05)(B, S, D)), 'w1': _w((lambda *s: _rng.normal(s) * 0.05)(D, D) * D ** (-0.5)), 'w2': _w((lambda *s: _rng.normal(s) * 0.05)(D, D) * D ** (-0.5)), 'w3': _w((lambda *s: _rng.normal(s) * 0.05)(D, F) * D ** (-0.5)), 'w4': _w((lambda *s: _rng.normal(s) * 0.05)(F, D) * F ** (-0.5))}
    _B_in = _B_setup()
    return {'A_x': _A_in['x'], 'A_mem0': _A_in['mem0'], 'A_Wq': _A_in['Wq'], 'A_Wk': _A_in['Wk'], 'A_Wv': _A_in['Wv'], 'A_Wo': _A_in['Wo'], 'A_seg_len': _A_in['seg_len'], 'B_x': _B_in['x'], 'B_w1': _B_in['w1'], 'B_w2': _B_in['w2'], 'B_w3': _B_in['w3'], 'B_w4': _B_in['w4'], 'c': _w((lambda *s: _rng.normal(s) * 0.05)(1, 1024)), 'w_mod': _w((lambda *s: _rng.normal(s) * 0.05)(1024, 6 * 1024) * 1024 ** (-0.5))}

def reference(A_x, A_mem0, A_Wq, A_Wk, A_Wv, A_Wo, A_seg_len, B_x, B_w1, B_w2, B_w3, B_w4, c, w_mod):

    def _A_ref(x, mem0, Wq, Wk, Wv, Wo, seg_len):
        B, S, Dm = x.shape
        H, Dh = (Wq.shape[1], Wq.shape[2])
        M = mem0.shape[1]
        scale = Dh ** (-0.5)
        n_seg = S // seg_len
        L = M + seg_len
        idx = jnp.arange(L)
        mask = (idx[:, None] < M) | (idx[:, None] >= idx[None, :])
        mem = mem0
        outs = []
        for s in range(n_seg):
            xs = x[:, s * seg_len:(s + 1) * seg_len, :].copy()
            h = jnp.concatenate([mem, xs], axis=1)
            q = jnp.einsum('btd,dhe->bhte', h, Wq)
            k = jnp.einsum('btd,dhe->bhte', h, Wk)
            v = jnp.einsum('btd,dhe->bhte', h, Wv)
            scores = jnp.einsum('bhqe,bhke->bhqk', q, k) * scale
            scores = jnp.where(mask[None, None], scores, -1000000000.0)
            p = _softmax(scores, axis=-1)
            o = jnp.einsum('bhqk,bhke->bhqe', p, v)
            o = jnp.einsum('bhte,hed->btd', o, Wo)
            mem = o[:, :M, :].copy()
            outs.append(o[:, M:, :])
        return jnp.concatenate(outs, axis=1)

    def _B_ref(x, w1, w2, w3, w4):
        B, S, D = x.shape
        h = _gelu(_layernorm(x, axis=-1) @ w1)
        c = D // 4
        g0 = jnp.pad(h[:, :, 0 * c:1 * c], ((0, 0), (1, 0), (0, 0)))[:, :S, :]
        g1 = jnp.pad(h[:, :, 1 * c:2 * c], ((0, 0), (0, 1), (0, 0)))[:, 1:, :]
        g2 = jnp.pad(h[:, :, 2 * c:3 * c], ((0, 0), (2, 0), (0, 0)))[:, :S, :]
        g3 = jnp.pad(h[:, :, 3 * c:], ((0, 0), (0, 2), (0, 0)))[:, 2:, :]
        hs = jnp.concatenate([g0, g1, g2, g3], axis=-1) @ w2
        x1 = x + hs
        h2 = _gelu(_layernorm(x1, axis=-1) @ w3) @ w4
        return x1 + h2
    x = A_x
    mod = (_silu(c) @ w_mod).reshape(c.shape[0], 6, 1, -1)
    sa, ca, ga, sb, cb, gb = (mod[:, 0].copy(), mod[:, 1].copy(), mod[:, 2].copy(), mod[:, 3].copy(), mod[:, 4].copy(), mod[:, 5].copy())
    h = _layernorm(x, axis=-1) * (1 + ca) + sa
    x = x + ga * _A_ref(h, A_mem0, A_Wq, A_Wk, A_Wv, A_Wo, A_seg_len)
    h = _layernorm(x, axis=-1) * (1 + cb) + sb
    x = x + gb * _B_ref(h, B_w1, B_w2, B_w3, B_w4)
    return x
```

```python
import functools

import jax
import jax.numpy as jnp
from jax import lax
import jax.experimental.pallas as pl
import jax.experimental.pallas.tpu as pltpu

F32 = jnp.float32
BF16 = jnp.bfloat16
U32 = jnp.uint32
LANES = 128
EPS = 1e-5

HEAD_GROUP = 4
STAGE_SLOTS = 8
TM = 256
FC = 512


def _ln(x):
    m = jnp.mean(x, axis=-1, keepdims=True)
    d = x - m
    v = jnp.mean(d * d, axis=-1, keepdims=True)
    return d * lax.rsqrt(v + EPS)


def _dot(a, b):
    return jnp.dot(a, b, preferred_element_type=F32)


def _dot_nt(a, b):
    return lax.dot_general(a, b, (((1,), (1,)), ((), ())), preferred_element_type=F32)


def _panel(ref, p, r0=None, nr=None):
    w = ref[p] if r0 is None else ref[p, pl.ds(r0, nr), :]
    return pltpu.bitcast(w, BF16)


def _panels(ref, p0, n, r0=None, nr=None):
    return jnp.concatenate([_panel(ref, p0 + j, r0, nr) for j in range(n)], axis=1)


def _kernel(x_hbm, mem0_ref, wq_hbm, wk_hbm, wv_hbm, wo_hbm, w1_hbm, w2_hbm, w3_hbm, w4_hbm,
            c_ref, wmod_hbm, out_hbm,
            wqkv, wo, wb, w4, xs, x1s, hs, hns, mod, sem_x, sem_mod, sem_wo, sem_b, sem_out,
            *, S, D, H, M, SEG, F):
    NSEG = S // SEG
    E = 8
    L = M + SEG
    LP = -(-L // 16) * 16
    ND = D // LANES
    NF = F // LANES
    scale = LANES ** -0.5

    def lanes(j, n=1):
        return pl.ds(j * LANES, n * LANES)

    w_u = [r.bitcast(U32) for r in (wq_hbm, wk_hbm, wv_hbm)]
    wo_u, w1_u, w2_u, w3_u, w4_u, wmod_u = (
        r.bitcast(U32) for r in (wo_hbm, w1_hbm, w2_hbm, w3_hbm, w4_hbm, wmod_hbm))

    def mod_copy(j):
        return pltpu.make_async_copy(wmod_u.at[:, lanes(j)], wb.at[j], sem_mod.at[j])

    def wo_copy(j):
        return pltpu.make_async_copy(wo_u.at[:, lanes(j)], wo.at[j], sem_wo.at[j])

    b_copies = []
    for j in range(ND):
        b_copies.append((w1_u.at[:, lanes(j)], wb.at[j]))
        b_copies.append((w2_u.at[:, lanes(j)], wb.at[ND + j]))
    for j in range(NF):
        b_copies.append((w3_u.at[:, lanes(j)], wb.at[2 * ND + j]))
    for j in range(ND):
        b_copies.append((w4_u.at[:, lanes(j)], w4.at[j]))
    b_copies = [pltpu.make_async_copy(s, d, sem_b.at[i]) for i, (s, d) in enumerate(b_copies)]
    x_copy = pltpu.make_async_copy(x_hbm, xs, sem_x.at[0])

    def mod_chunk(i):
        cv = c_ref[...].astype(F32)
        sc = jnp.broadcast_to(cv * jax.nn.sigmoid(cv), (8, D))
        for j in range(ND):
            mod_copy(i * ND + j).wait()
        for j in range(ND):
            mod[i, :, lanes(j)] = _dot(sc, _panel(wb, i * ND + j))

    def rows(v, n):
        return jnp.concatenate([v] * (n // 8), axis=0)

    def attention_phase(stage, early, he, lhs, obuf, aout, sem_st):
        NP = 3 * (H // 2)

        def stage_copy(i, src):
            slot = i % STAGE_SLOTS
            return pltpu.make_async_copy(src, stage.at[slot], sem_st.at[slot])

        for j in range(2 * ND):
            mod_copy(j).start()
        x_copy.start()
        for i in range(STAGE_SLOTS):
            stage_copy(i, w_u[i % 3].at[:, i // 3, :]).start()

        mod_chunk(0)
        mod_chunk(1)
        x_copy.wait()

        def modulate_a(xv):
            n = xv.shape[0]
            return _ln(xv) * rows(1.0 + mod[1], n) + rows(mod[0], n)

        def early_rows(t, carry):
            parts = []
            for u in range(4):
                r = pl.multiple_of((4 * t + u) * SEG, SEG)
                parts.append(xs[pl.ds(r, 16), :].astype(F32)[:E])
            he[pl.ds(pl.multiple_of(t * 4 * E, 4 * E), 4 * E), :] = (
                modulate_a(jnp.concatenate(parts, axis=0)).astype(BF16))
            return carry
        lax.fori_loop(0, NSEG // 4, early_rows, 0)

        extra = [wo_copy(j) for j in range(ND)] + [mod_copy(j) for j in range(2 * ND, 6 * ND)]
        for i in range(NP):
            hp, m = i // 3, i % 3
            slot = i % STAGE_SLOTS
            stage_copy(i, w_u[m].at[:, hp, :]).wait()
            a = stage[slot, pl.ds(0, D // 2, stride=2), :]
            b = stage[slot, pl.ds(1, D // 2, stride=2), :]
            p0, p1 = 3 * (2 * hp) + m, 3 * (2 * hp + 1) + m
            wqkv[p0] = (a & jnp.uint32(0xFFFF)) | (b << 16)
            wqkv[p1] = (a >> 16) | (b & jnp.uint32(0xFFFF0000))
            n = i + STAGE_SLOTS
            if n < NP:
                stage_copy(n, w_u[n % 3].at[:, n // 3, :]).start()
            if i < len(extra):
                extra[i].start()
            for p in (p0, p1):
                early[:, p] = _dot(he[...], _panel(wqkv, p)).reshape(NSEG, E, LANES)
        for cp in extra[NP:]:
            cp.start()

        for i in range(2, 6):
            mod_chunk(i)
        for j in range(ND):
            wo_copy(j).wait()
        for cp in b_copies:
            cp.start()

        def stage_tokens(s):
            r = pl.multiple_of(s * SEG, SEG)
            lhs[pl.ds(M, SEG - E), :] = modulate_a(xs[pl.ds(r, SEG), :].astype(F32)[E:])

        def finish_tokens(s):
            r = pl.multiple_of(s * SEG, SEG)
            x1 = xs[pl.ds(r, SEG), :].astype(F32) + rows(mod[2], SEG) * aout[...]
            h = _ln(x1) * rows(1.0 + mod[4], SEG) + rows(mod[3], SEG)
            x1s[pl.ds(r, SEG), :] = x1
            hs[pl.ds(r, SEG), :] = h
            hns[pl.ds(r, SEG), :] = _ln(h).astype(BF16)

        lhs[pl.ds(0, M), :] = mem0_ref[...].astype(F32)
        stage_tokens(0)
        aout[...] = jnp.zeros_like(aout)

        def step(s, carry):
            ri = lax.broadcasted_iota(jnp.int32, (L, LP), 0)
            ci = lax.broadcasted_iota(jnp.int32, (L, LP), 1)
            keep = ((ri < M) | (ri >= ci)) & (ci < L)
            fill = jnp.where(ci < L, -1e9, -jnp.inf).astype(F32)
            zpad = jnp.zeros((LP - L, LANES), F32)

            def project(h, m):
                p = 3 * h + m
                y = _dot(lhs[...], _panel(wqkv, p))
                parts = [y[:M], early[s, p], y[M:]]
                if m == 0:
                    return jnp.concatenate(parts, axis=0)
                return jnp.concatenate(parts + [zpad], axis=0).astype(BF16)

            def probs(q, k):
                sc = jnp.where(keep, _dot_nt(q, k) * scale, fill)
                e = jnp.exp(sc - jnp.max(sc, axis=-1, keepdims=True))
                return e / jnp.sum(e, axis=-1, keepdims=True)

            finish_tokens(jnp.maximum(s - 1, 0))
            G = HEAD_GROUP
            NG = H // G
            prev = None
            for g in range(NG + 1):
                heads = range(g * G, (g + 1) * G) if g < NG else ()
                q = [project(h, 0) for h in heads]
                if prev is not None:
                    pr = [probs(a, b) for a, b in zip(prev[0], prev[1])]
                k = [project(h, 1) for h in heads]
                v = [project(h, 2) for h in heads]
                if g == NG:
                    KH = (H - G) * LANES
                    acc = [_dot(obuf[:, pl.ds(0, KH)], _panel(wo, j, 0, KH // 2)) for j in range(ND)]
                if prev is not None:
                    for u in range(G):
                        obuf[:, lanes((g - 1) * G + u)] = _dot(pr[u], prev[2][u])
                prev = (q, k, v)
            stage_tokens(jnp.minimum(s + 1, NSEG - 1))
            for j in range(ND):
                y = acc[j] + _dot(obuf[:, lanes(H - G, G)], _panel(wo, j, KH // 2, G * LANES // 2))
                lhs[pl.ds(0, M), lanes(j)] = y[:M]
                aout[:, lanes(j)] = y[M:]
            return carry
        lax.fori_loop(0, NSEG, step, 0)
        finish_tokens(NSEG - 1)

    pl.run_scoped(
        attention_phase,
        pltpu.VMEM((STAGE_SLOTS, D, LANES), U32),
        pltpu.VMEM((NSEG, 3 * H, E, LANES), F32),
        pltpu.VMEM((NSEG * E, D), BF16),
        pltpu.VMEM((M + SEG - E, D), F32),
        pltpu.VMEM((L, H * LANES), F32),
        pltpu.VMEM((SEG, D), F32),
        pltpu.SemaphoreType.DMA((STAGE_SLOTS,)),
    )

    def mixer_phase(gbuf, obuf):
        NT = S // TM
        for cp in b_copies:
            cp.wait()
        gbuf[pl.ds(0, 8), :] = jnp.zeros((8, D), F32)
        gbuf[pl.ds(S + 8, 8), :] = jnp.zeros((8, D), F32)

        def gate(t, carry):
            r = pl.multiple_of(t * TM, TM)
            a = _dot(hns[pl.ds(r, TM), :], _panels(wb, 0, ND))
            gbuf[pl.ds(pl.multiple_of(r + 8, 8), TM), :] = jax.nn.gelu(a, approximate=True)
            return carry
        lax.fori_loop(0, NT, gate, 0)

        def out_copy(t):
            r = pl.multiple_of(t * TM, TM)
            return pltpu.make_async_copy(obuf.at[pl.ds(r, TM)], out_hbm.at[pl.ds(r, TM)], sem_out.at[t])

        def mlp(t, carry):
            r = pl.multiple_of(t * TM, TM)
            C = D // 4
            parts = []
            for i, shift in enumerate((-1, 1, -2, 2)):
                w = gbuf[pl.ds(r, TM + 16), pl.ds(i * C, C)]
                parts.append(w[8 + shift:8 + shift + TM].astype(BF16))
            y1 = hs[pl.ds(r, TM), :] + _dot(jnp.concatenate(parts, axis=1), _panels(wb, ND, ND))
            n2 = _ln(y1).astype(BF16)
            acc = y1
            NC = FC // LANES
            for f in range(F // FC):
                a = jax.nn.gelu(_dot(n2, _panels(wb, 2 * ND + f * NC, NC)), approximate=True)
                acc = acc + _dot(a.astype(BF16), _panels(w4, 0, ND, f * FC // 2, FC // 2))
            obuf[pl.ds(r, TM), :] = (x1s[pl.ds(r, TM), :] + rows(mod[5], TM) * acc).astype(BF16)
            out_copy(t).start()
            return carry
        lax.fori_loop(0, NT, mlp, 0)
        for t in range(NT):
            out_copy(t).wait()

    pl.run_scoped(mixer_phase, pltpu.VMEM((S + 16, D), F32), pltpu.VMEM((S, D), BF16))


@functools.partial(jax.jit, static_argnames=("A_seg_len",))
def pallas_adaLN_cond__memory_aug_recurrent_mem_tr__mixer_s_mlp__prompt_kernel(
    A_x, A_mem0, A_Wq, A_Wk, A_Wv, A_Wo, A_seg_len, B_x, B_w1, B_w2, B_w3, B_w4, c, w_mod,
):
    del B_x
    B, S, D = A_x.shape
    H, Dh = A_Wq.shape[1:]
    M = A_mem0.shape[1]
    F = B_w3.shape[1]
    assert B == 1 and Dh == LANES and M == 8 and A_seg_len % 16 == 0 and S % A_seg_len == 0
    ND, NF = D // LANES, F // LANES
    hbm = pl.BlockSpec(memory_space=pl.ANY)
    vmem = pl.BlockSpec(memory_space=pltpu.VMEM)
    out = pl.pallas_call(
        functools.partial(_kernel, S=S, D=D, H=H, M=M, SEG=A_seg_len, F=F),
        out_shape=jax.ShapeDtypeStruct((S, D), A_x.dtype),
        in_specs=[hbm, vmem, hbm, hbm, hbm, hbm, hbm, hbm, hbm, hbm, vmem, hbm],
        out_specs=hbm,
        scratch_shapes=[
            pltpu.VMEM((3 * H, D // 2, LANES), U32),
            pltpu.VMEM((ND, H * Dh // 2, LANES), U32),
            pltpu.VMEM((max(6 * ND, 2 * ND + NF), D // 2, LANES), U32),
            pltpu.VMEM((ND, F // 2, LANES), U32),
            pltpu.VMEM((S, D), BF16),
            pltpu.VMEM((S, D), F32),
            pltpu.VMEM((S, D), F32),
            pltpu.VMEM((S, D), BF16),
            pltpu.VMEM((6, 8, D), F32),
            pltpu.SemaphoreType.DMA((1,)),
            pltpu.SemaphoreType.DMA((6 * ND,)),
            pltpu.SemaphoreType.DMA((ND,)),
            pltpu.SemaphoreType.DMA((3 * ND + NF,)),
            pltpu.SemaphoreType.DMA((S // TM,)),
        ],
        compiler_params=pltpu.CompilerParams(vmem_limit_bytes=124 * 1024 * 1024),
    )(A_x.reshape(S, D), A_mem0.reshape(M, D), A_Wq, A_Wk, A_Wv, A_Wo.reshape(H * Dh, D),
      B_w1, B_w2, B_w3, B_w4, c, w_mod)
    return out.reshape(B, S, D)
```

```python
import functools

import jax
import jax.numpy as jnp
from jax import lax
import jax.experimental.pallas as pl
import jax.experimental.pallas.tpu as pltpu

F32 = jnp.float32
BF16 = jnp.bfloat16
U32 = jnp.uint32
LANES = 128
EPS = 1e-5

HEAD_GROUP = 4
PREFETCH = 3
X_SPLIT = 8
FINISH_AT = 2
WO_SPLIT = 6
TM = 128
FC = 896


def _ln(x):
    m = jnp.mean(x, axis=-1, keepdims=True)
    d = x - m
    v = jnp.mean(d * d, axis=-1, keepdims=True)
    return d * lax.rsqrt(v + EPS)


def _dot(a, b):
    return jnp.dot(a, b, preferred_element_type=F32)


def _dot_nt(a, b):
    return lax.dot_general(a, b, (((1,), (1,)), ((), ())), preferred_element_type=F32)


def _panel(ref, p, r0=None, nr=None):
    w = ref[p] if r0 is None else ref[p, pl.ds(r0, nr), :]
    return pltpu.bitcast(w, BF16)


def _panels(ref, p0, n, r0=None, nr=None):
    return jnp.concatenate([_panel(ref, p0 + j, r0, nr) for j in range(n)], axis=1)


def _kernel(x_hbm, mem0_ref, wq_hbm, wk_hbm, wv_hbm, wo_hbm, w1_hbm, w2_hbm, w3_hbm, w4_hbm,
            c_ref, wmod_hbm, out_hbm,
            wb, w4, seg, mod, sem_mod, sem_b,
            *, S, D, H, M, SEG, F):
    NSEG = S // SEG
    E = M
    L = M + SEG
    LP = -(-L // 16) * 16
    ND = D // LANES
    NF = F // LANES
    R = SEG // 8
    scale = LANES ** -0.5
    TOK = 3 * H
    X1, HB, HN = 0, R * ND, 2 * R * ND

    def lanes(j, n=1):
        start = j * LANES
        return pl.ds(start if isinstance(j, int) else pl.multiple_of(start, LANES), n * LANES)

    def seg_put(row, slot, v):
        if v.dtype != F32:
            v = pltpu.bitcast(v, F32)
        r = v.shape[0] // 8
        for j in range(ND):
            seg[row, pl.ds(slot + j * r, r)] = v[:, j * LANES:(j + 1) * LANES].reshape(r, 8, LANES)

    def seg_get(row, n, slot, dtype):
        r = R if dtype == F32 else R // 2
        v = jnp.concatenate(
            [seg[pl.ds(row, n), pl.ds(slot + j * r, r)].reshape(n * r * 8, LANES) for j in range(ND)],
            axis=1)
        return v if dtype == F32 else pltpu.bitcast(v, dtype)

    w_u = [r.bitcast(U32) for r in (wq_hbm, wk_hbm, wv_hbm)]
    wo_u, w1_u, w2_u, w3_u, w4_u, wmod_u = (
        r.bitcast(U32) for r in (wo_hbm, w1_hbm, w2_hbm, w3_hbm, w4_hbm, wmod_hbm))

    def mod_copy(j):
        return pltpu.make_async_copy(wmod_u.at[:, lanes(j)], wb.at[j], sem_mod.at[j])

    b_copies = []
    for j in range(ND):
        b_copies.append((w1_u.at[:, lanes(j)], wb.at[j]))
        b_copies.append((w2_u.at[:, lanes(j)], wb.at[ND + j]))
    for j in range(NF):
        b_copies.append((w3_u.at[:, lanes(j)], wb.at[2 * ND + j]))
    for j in range(ND):
        b_copies.append((w4_u.at[:, lanes(j)], w4.at[j]))
    b_copies = [pltpu.make_async_copy(s, d, sem_b.at[i]) for i, (s, d) in enumerate(b_copies)]

    def mod_chunks(lo, hi):
        cv = c_ref[...].astype(F32)
        sc = jnp.broadcast_to(cv * jax.nn.sigmoid(cv), (8, D))
        for j in range(lo * ND, hi * ND):
            mod_copy(j).wait()
        for j in range(lo * ND, hi * ND):
            mod[j // ND, :, lanes(j % ND)] = _dot(sc, _panel(wb, j))

    def rows(v, n):
        return jnp.concatenate([v] * (n // 8), axis=0)

    def attention_phase(wqkv, wo, xs, xn, he, lhs, obuf, aout, acc, sem_w, sem_x, sem_wo):
        HP = H // 2

        def w_copies(hp, m):
            return [pltpu.make_async_copy(w_u[m].at[:, i, hp, :], wqkv.at[6 * hp + 3 * i + m],
                                          sem_w.at[6 * hp + 3 * i + m]) for i in range(2)]

        def wo_copy(j):
            return pltpu.make_async_copy(wo_u.at[:, lanes(j)], wo.at[j], sem_wo.at[j])

        def x_copy(i):
            n = NSEG // X_SPLIT
            idx = ((pl.ds(i * n, n), pl.ds(0, E)) if i < X_SPLIT
                   else (pl.ds(0, NSEG), pl.ds(E, SEG - E)))
            return pltpu.make_async_copy(x_hbm.at[idx], xs.at[idx], sem_x.at[i])

        def modulate_a(n):
            return n * rows(1.0 + mod[1], n.shape[0]) + rows(mod[0], n.shape[0])

        for i in range(X_SPLIT):
            x_copy(i).start()
        for j in range(2 * ND):
            mod_copy(j).start()
        for m in range(3):
            for cp in w_copies(0, m):
                cp.start()

        with jax.named_scope("early_ln"):
            for i in range(X_SPLIT):
                x_copy(i).wait()

            def early_norm(t, carry):
                xv = xs[pl.ds(t * 16, 16), pl.ds(0, E), :].astype(F32).reshape(16 * E, D)
                xn[pl.ds(pl.multiple_of(t * 16 * E, 16 * E), 16 * E), :] = _ln(xv)
                return carry
            lax.fori_loop(0, NSEG // 16, early_norm, 0)

        with jax.named_scope("mod_a"):
            mod_chunks(0, 2)
            for hp in range(1, PREFETCH):
                for m in range(3):
                    for cp in w_copies(hp, m):
                        cp.start()
            x_copy(X_SPLIT).start()
            hv = pltpu.bitcast(modulate_a(xn[...]).astype(BF16), U32)
            for j in range(ND):
                he[j] = hv[:, j * LANES:(j + 1) * LANES]

        def look_ahead(hp, tokens):
            @pl.when(hp + PREFETCH < HP)
            def _():
                for m in range(3):
                    for cp in w_copies(hp + PREFETCH, m):
                        cp.start()

            @pl.when(hp < ND)
            def _():
                wo_copy(hp).start()
            for u in range(4 * ND // HP):
                mod_copy(2 * ND + hp * (4 * ND // HP) + u).start()
            for m in range(3):
                for cp in w_copies(hp, m):
                    cp.wait()
            for m in range(3):
                p = 6 * hp + m
                a, b = wqkv[p], wqkv[p + 3]
                w = ((a & jnp.uint32(0xFFFF)) | (b << 16), (a >> 16) | (b & jnp.uint32(0xFFFF0000)))
                for i in range(2):
                    wqkv[p + 3 * i] = w[i]
                    y = _dot(_panels(he, 0, ND), pltpu.bitcast(w[i], BF16))
                    seg[pl.ds(1, NSEG), p + 3 * i] = y.reshape(NSEG, E, LANES)
                    if tokens is not None and 2 * m + i < 4:
                        for s in tokens(2 * m + i):
                            seg_put(1 + s, TOK, modulate_a(_ln(xs[s].astype(F32))).astype(BF16))

        with jax.named_scope("look_ahead"):
            per = 2 * NSEG // HP // 4
            lax.fori_loop(0, HP // 2, lambda hp, c: look_ahead(hp, None), None)
            x_copy(X_SPLIT).wait()
            lax.fori_loop(
                HP // 2, HP,
                lambda hp, c: look_ahead(
                    hp, lambda i: [((hp - HP // 2) * 4 + i) * per + u for u in range(per)]),
                None)

        with jax.named_scope("mod_b"):
            mod_chunks(2, 6)
            for j in range(ND):
                wo_copy(j).wait()
            for cp in b_copies:
                cp.start()

        def set_lhs(mem, s, j):
            tok = seg[1 + s, pl.ds(TOK + j * R // 2, R // 2)].reshape(SEG // 2, LANES)
            tok = pltpu.bitcast(tok, BF16)
            head = jnp.concatenate([mem, tok[:16].astype(F32)[E:]], axis=0).astype(BF16)
            lhs[j] = pltpu.bitcast(jnp.concatenate([head, tok[16:]], axis=0), U32)

        def finish_tokens(s, row):
            x1 = xs[s].astype(F32) + rows(mod[2], SEG) * aout[...]
            h = _ln(x1) * rows(1.0 + mod[4], SEG) + rows(mod[3], SEG)
            seg_put(row, X1, x1)
            seg_put(row, HB, h)
            seg_put(row, HN, _ln(h).astype(BF16))

        for j in range(ND):
            set_lhs(mem0_ref[:, lanes(j)].astype(F32), 0, j)
        aout[...] = jnp.zeros_like(aout)

        def step(s, carry):
            ri = lax.broadcasted_iota(jnp.int32, (L, LP), 0)
            ci = lax.broadcasted_iota(jnp.int32, (L, LP), 1)
            keep = ((ri < M) | (ri >= ci)) & (ci < L)
            fill = jnp.where(ci < L, -1e9, -jnp.inf).astype(F32)
            zpad = jnp.zeros((LP - L, LANES), F32)

            def project(h, m):
                p = 3 * h + m
                y = _dot(_panels(lhs, 0, ND), _panel(wqkv, p))
                parts = [y[:M], seg[1 + s, p], y[M:]]
                if m == 0:
                    return jnp.concatenate(parts, axis=0)
                return jnp.concatenate(parts + [zpad], axis=0).astype(BF16)

            def probs(q, k):
                sc = jnp.where(keep, _dot_nt(q, k) * scale, fill)
                e = jnp.exp(sc - jnp.max(sc, axis=-1, keepdims=True))
                return e / jnp.sum(e, axis=-1, keepdims=True)

            G = HEAD_GROUP
            NG = H // G
            KH = (H - G) * LANES

            def out_head(j):
                acc[:, lanes(j)] = _dot(obuf[:, pl.ds(0, KH)], _panel(wo, j, 0, KH // 2))

            prev = None
            for g in range(NG + 1):
                if g == FINISH_AT:
                    finish_tokens(jnp.maximum(s - 1, 0), s)
                heads = range(g * G, (g + 1) * G) if g < NG else ()
                q = [project(h, 0) for h in heads]
                if prev is not None:
                    pr = [probs(a, b) for a, b in zip(prev[0], prev[1])]
                k = [project(h, 1) for h in heads]
                v = [project(h, 2) for h in heads]
                if g == NG:
                    for j in range(WO_SPLIT):
                        out_head(j)
                if prev is not None:
                    for u in range(G):
                        obuf[:, lanes((g - 1) * G + u)] = _dot(pr[u], prev[2][u])
                prev = (q, k, v)
            for j in list(range(WO_SPLIT, ND)) + list(range(WO_SPLIT)):
                if j < WO_SPLIT:
                    y = acc[:, lanes(j)] + _dot(
                        obuf[:, lanes(H - G, G)], _panel(wo, j, KH // 2, G * LANES // 2))
                else:
                    y = _dot(obuf[...], _panel(wo, j))
                set_lhs(y[:M], jnp.minimum(s + 1, NSEG - 1), j)
                aout[:, lanes(j)] = y[M:]
            return carry
        with jax.named_scope("steps"):
            lax.fori_loop(0, NSEG, step, 0)
        finish_tokens(NSEG - 1, NSEG)

    pl.run_scoped(
        attention_phase,
        pltpu.VMEM((3 * H, D // 2, LANES), U32),
        pltpu.VMEM((ND, H * LANES // 2, LANES), U32),
        pltpu.VMEM((NSEG, SEG, D), BF16),
        pltpu.VMEM((NSEG * E, D), F32),
        pltpu.VMEM((ND, NSEG * E // 2, LANES), U32),
        pltpu.VMEM((ND, SEG // 2, LANES), U32),
        pltpu.VMEM((L, H * LANES), F32),
        pltpu.VMEM((SEG, D), F32),
        pltpu.VMEM((L, D), F32),
        pltpu.SemaphoreType.DMA((3 * H,)),
        pltpu.SemaphoreType.DMA((X_SPLIT + 1,)),
        pltpu.SemaphoreType.DMA((ND,)),
    )

    def mixer_phase(gbuf, obuf, sem_out):
        NT = S // TM
        TS = TM // SEG
        for cp in b_copies:
            cp.wait()
        gbuf[pl.ds(0, 8), :] = jnp.zeros((8, D), F32)
        gbuf[pl.ds(S + 8, 8), :] = jnp.zeros((8, D), F32)

        def gate(t):
            a = _dot(seg_get(1 + t * TS, TS, HN, BF16), _panels(wb, 0, ND))
            gbuf[pl.ds(pl.multiple_of(t * TM + 8, 8), TM), :] = jax.nn.gelu(a, approximate=True)

        def out_copy(t):
            r = pl.multiple_of(t * TM, TM)
            return pltpu.make_async_copy(obuf.at[pl.ds(r, TM)], out_hbm.at[pl.ds(r, TM)], sem_out.at[t])

        def mlp(t, gate_ahead):
            r = pl.multiple_of(t * TM, TM)
            C = D // 4
            parts = []
            for i, shift in enumerate((-1, 1, -2, 2)):
                w = gbuf[pl.ds(r, TM + 16), pl.ds(i * C, C)]
                parts.append(w[8 + shift:8 + shift + TM].astype(BF16))
            y1 = seg_get(1 + t * TS, TS, HB, F32) + _dot(
                jnp.concatenate(parts, axis=1), _panels(wb, ND, ND))
            if gate_ahead:
                gate(t + 2)
            n2 = _ln(y1).astype(BF16)
            acc = y1
            NC = FC // LANES
            for f in range(F // FC):
                a = jax.nn.gelu(_dot(n2, _panels(wb, 2 * ND + f * NC, NC)), approximate=True)
                acc = acc + _dot(a.astype(BF16), _panels(w4, 0, ND, f * FC // 2, FC // 2))
            x1 = seg_get(1 + t * TS, TS, X1, F32)
            obuf[pl.ds(r, TM), :] = (x1 + rows(mod[5], TM) * acc).astype(BF16)
            out_copy(t).start()

        with jax.named_scope("gate"):
            gate(0)
            gate(1)
        with jax.named_scope("mlp"):
            lax.fori_loop(0, NT - 2, lambda t, c: mlp(t, True), None)
        with jax.named_scope("mlp2"):
            lax.fori_loop(NT - 2, NT, lambda t, c: mlp(t, False), None)
        for t in range(NT):
            out_copy(t).wait()

    pl.run_scoped(mixer_phase, pltpu.VMEM((S + 16, D), F32), pltpu.VMEM((S, D), BF16),
                  pltpu.SemaphoreType.DMA((S // TM,)))


@functools.partial(jax.jit, static_argnames=("A_seg_len",))
def pallas_adaLN_cond__memory_aug_recurrent_mem_tr__mixer_s_mlp__prompt_kernel(
    A_x, A_mem0, A_Wq, A_Wk, A_Wv, A_Wo, A_seg_len, B_x, B_w1, B_w2, B_w3, B_w4, c, w_mod,
):
    del B_x
    B, S, D = A_x.shape
    H, Dh = A_Wq.shape[1:]
    M = A_mem0.shape[1]
    F = B_w3.shape[1]
    SEG = A_seg_len
    assert B == 1 and Dh == LANES and M == 8 and SEG % 16 == 0 and S % SEG == 0
    ND, NF = D // LANES, F // LANES
    hbm = pl.BlockSpec(memory_space=pl.ANY)
    vmem = pl.BlockSpec(memory_space=pltpu.VMEM)
    out = pl.pallas_call(
        functools.partial(_kernel, S=S, D=D, H=H, M=M, SEG=SEG, F=F),
        out_shape=jax.ShapeDtypeStruct((S, D), A_x.dtype),
        in_specs=[hbm, vmem, hbm, hbm, hbm, hbm, hbm, hbm, hbm, hbm, vmem, hbm],
        out_specs=hbm,
        scratch_shapes=[
            pltpu.VMEM((max(6 * ND, 2 * ND + NF), D // 2, LANES), U32),
            pltpu.VMEM((ND, F // 2, LANES), U32),
            pltpu.VMEM((S // SEG + 1, 3 * H + ND * SEG // 16, 8, LANES), F32),
            pltpu.VMEM((6, 8, D), F32),
            pltpu.SemaphoreType.DMA((6 * ND,)),
            pltpu.SemaphoreType.DMA((3 * ND + NF,)),
        ],
        compiler_params=pltpu.CompilerParams(vmem_limit_bytes=124 * 1024 * 1024),
    )(A_x.reshape(S // SEG, SEG, D), A_mem0.reshape(M, D),
      *(w.reshape(D // 2, 2, H, Dh) for w in (A_Wq, A_Wk, A_Wv)),
      A_Wo.reshape(H * Dh, D), B_w1, B_w2, B_w3, B_w4, c, w_mod)
    return out.reshape(B, S, D)
```

```python
import functools

import jax
import jax.numpy as jnp
import numpy as np
from jax import lax
import jax.experimental.pallas as pl
import jax.experimental.pallas.tpu as pltpu

F32 = jnp.float32
BF16 = jnp.bfloat16
U32 = jnp.uint32
LANES = 128
EPS = 1e-5

HEAD_GROUP = 4
PREFETCH = 3
FINISH_AT = 2
SUMS_IN_STEPS = True
PIN_FINISH = 0
WO_SPLIT = 6
PLAIN_STEPS = 16
LA_ROWS = 64
TM = 128

B11, B12, B21, B22 = 1, 2, 3, 4


def _ln(x):
    m = jnp.mean(x, axis=-1, keepdims=True)
    d = x - m
    v = jnp.mean(d * d, axis=-1, keepdims=True)
    return d * lax.rsqrt(v + EPS)


def _dot(a, b):
    return jnp.dot(a, b, preferred_element_type=F32)


def _dot_nt(a, b):
    return lax.dot_general(a, b, (((1,), (1,)), ((), ())), preferred_element_type=F32)


def _panel(ref, p, r0=None, nr=None):
    w = ref[p] if r0 is None else ref[p, pl.ds(r0, nr), :]
    return pltpu.bitcast(w, BF16)


def _panels(ref, p0, n):
    return jnp.concatenate([_panel(ref, p0 + j) for j in range(n)], axis=1)


def _strassen_lhs(a11, a12, a21, a22):
    return [a11 + a22, a21 + a22, a11, a22, a11 + a12, a21 - a11, a12 - a22]


def _strassen_rhs(b11, b12, b21, b22):
    c11, c12, c21, c22 = (b.astype(F32) for b in (b11, b12, b21, b22))
    return [(c11 + c22).astype(BF16), b11, (c12 - c22).astype(BF16), (c21 - c11).astype(BF16),
            b22, (c11 + c12).astype(BF16), (c21 + c22).astype(BF16)]


def _strassen_out(m):
    return m[0] + m[3] - m[4] + m[6], m[2] + m[4], m[1] + m[3], m[0] - m[1] + m[2] + m[5]


def _quarters(v):
    r, c = v.shape[0] // 2, v.shape[1] // 2
    return v[:r, :c], v[:r, c:], v[r:, :c], v[r:, c:]


def _pin(i):
    return i >> 24


def _kernel(x_hbm, mem0_ref, wq_hbm, wk_hbm, wv_hbm, wo_hbm, w1_hbm, w2_hbm, w3_hbm, w4_hbm,
            c_ref, wmod_hbm, out_hbm,
            wm, seg, mod, sem_mod, sem_b,
            *, S, D, H, M, SEG, F):
    NSEG = S // SEG
    E = M
    L = M + SEG
    LP = -(-L // 16) * 16
    ND = D // LANES
    NF = F // LANES
    R = SEG // 8
    scale = LANES ** -0.5
    TOK = 3 * H
    X1, HB, HN = 0, R * ND, 2 * R * ND

    def lanes(j, n=1):
        start = j * LANES
        return pl.ds(start if isinstance(j, int) else pl.multiple_of(start, LANES), n * LANES)

    def seg_put(row, slot, v, n=1):
        if v.dtype != F32:
            v = pltpu.bitcast(v, F32)
        r = v.shape[0] // (8 * n)
        for j in range(v.shape[1] // LANES):
            seg[pl.ds(row, n), pl.ds(slot + j * r, r)] = (
                v[:, j * LANES:(j + 1) * LANES].reshape(n, r, 8, LANES))

    def seg_get(row, n, slot, cols=ND):
        return jnp.concatenate(
            [seg[pl.ds(row, n), pl.ds(slot + j * R, R)].reshape(n * SEG, LANES) for j in range(cols)],
            axis=1)

    w_u = [r.bitcast(U32) for r in (wq_hbm, wk_hbm, wv_hbm)]
    wo_u = wo_hbm.bitcast(U32)
    wm_u = wm.bitcast(U32)

    WM_AT = np.cumsum([0, ND * D // 4, ND * D // 4, NF * D // 4]).tolist()
    b_copies = []
    for w, at in zip((w1_hbm, w2_hbm, w3_hbm, w4_hbm), WM_AT):
        kh, nh = w.shape[0] // 2, w.shape[1] // LANES // 2
        for j in range(nh):
            for i, r0, p in ((B11, 0, j), (B12, 0, j + nh), (B21, kh, j), (B22, kh, j + nh)):
                b_copies.append(pltpu.make_async_copy(
                    w.at[pl.ds(r0, kh), lanes(p)], wm.at[i, pl.ds(at + j * kh, kh)],
                    sem_b.at[len(b_copies)]))

    def mod_place(j):
        third = j // (2 * ND)
        return third + 4 * ((third + 1) // 2), j % (2 * ND)

    def mod_copy(j):
        i, k = mod_place(j)
        start = k * D if isinstance(j, int) else pl.multiple_of(k * D, D)
        return pltpu.make_async_copy(
            wmod_hbm.at[:, lanes(j)], wm.at[i, pl.ds(start, D)], sem_mod.at[j])

    def mod_chunks(lo, hi):
        cv = c_ref[...].astype(F32)
        sc = jnp.broadcast_to(cv * jax.nn.sigmoid(cv), (8, D))
        for j in range(lo * ND, hi * ND):
            mod_copy(j).wait()
        for j in range(lo * ND, hi * ND):
            i, k = mod_place(j)
            mod[j // ND, :, lanes(j % ND)] = _dot(sc, _panel(wm_u, i, k * D // 2, D // 2))

    def rows(v, n):
        return jnp.concatenate([v] * (n // 8), axis=0)

    def attention_phase(wqkv, wo, xs, xn, he, we, lhs, obuf, aout, acc, sem_w, sem_x, sem_wo):
        HP = H // 2

        def w_copies(hp, which=(0, 1, 2)):
            return [pltpu.make_async_copy(w_u[m].at[:, i, hp, :], wqkv.at[6 * hp + 3 * i + m],
                                          sem_w.at[6 * hp + 3 * i + m])
                    for m in which for i in range(2)]

        def wo_copy(j):
            return pltpu.make_async_copy(wo_u.at[:, lanes(j)], wo.at[j], sem_wo.at[j])

        def x_copy(i):
            sl = (pl.ds(0, E), pl.ds(E, SEG - E))[i]
            return pltpu.make_async_copy(x_hbm.at[:, sl, :], xs.at[:, sl, :], sem_x.at[i])

        def modulate_a(n):
            return n * rows(1.0 + mod[1], n.shape[0]) + rows(mod[0], n.shape[0])

        x_copy(0).start()
        for j in range(2 * ND):
            mod_copy(j).start()

        with jax.named_scope("early_ln"):
            x_copy(0).wait()
            for cp in w_copies(0):
                cp.start()

            def early_norm(t, carry):
                xv = xs[pl.ds(t * 16, 16), pl.ds(0, E), :].astype(F32).reshape(16 * E, D)
                xn[pl.ds(pl.multiple_of(t * 16 * E, 16 * E), 16 * E), :] = _ln(xv)
                return carry
            lax.fori_loop(0, NSEG // 16, early_norm, 0)

        with jax.named_scope("mod_a"):
            mod_chunks(0, 2)
            for hp in range(1, PREFETCH):
                for cp in w_copies(hp):
                    cp.start()

            def early_operands(t, carry):
                top, low = (
                    modulate_a(xn[pl.ds(pl.multiple_of(r0 + t * 32, 32), 32), :])
                    for r0 in (0, NSEG * E // 2))
                for i, v in enumerate(_strassen_lhs(*_quarters(jnp.concatenate([top, low], axis=0)))):
                    he[i, pl.ds(pl.multiple_of(t * 32, 32), 32), :] = v
                return carry
            lax.fori_loop(0, NSEG * E // 64, early_operands, 0)

        NU = NSEG * E // 2 // LA_ROWS

        NPIECE = 16
        we_u = we.bitcast(U32)

        def repack(hp, m, u):
            p = 6 * hp + m
            nr = D // 4 // NPIECE
            w = []
            for r0 in (u * nr, D // 4 + u * nr):
                a, b = wqkv[p, pl.ds(r0, nr), :], wqkv[p + 3, pl.ds(r0, nr), :]
                w.append((a & np.uint32(0xFFFF)) | (b << 16))
                w.append((a >> 16) | (b & np.uint32(0xFFFF0000)))
                wqkv[p, pl.ds(r0, nr), :], wqkv[p + 3, pl.ds(r0, nr), :] = w[-2:]
            for i, v in enumerate(_strassen_rhs(*(pltpu.bitcast(v, BF16) for v in w))):
                if i not in (B11, B22):
                    we[m, i, pl.ds(2 * u * nr, 2 * nr), :] = v

        def look_ahead(hp, last, tokens):
            @pl.when(hp + PREFETCH < HP)
            def _():
                for cp in w_copies(hp + PREFETCH):
                    cp.start()

            if tokens is None:
                wo_copy(hp).start()

                @pl.when(hp == 2)
                def _():
                    x_copy(1).start()
            for u in range(4 * ND // HP):
                mod_copy(2 * ND + hp * (4 * ND // HP) + u).start()
            for cp in w_copies(hp, (1, 2)) + ([] if last else w_copies(hp + 1, (0,))):
                cp.wait()
            n = LA_ROWS // E
            for m in range(3):
                p = 6 * hp + m
                todo = list(range(NPIECE)) if m < 2 or not last else []
                for u in range(NU):
                    prods = []
                    for i in range(7):
                        if i == B11:
                            w = wqkv[p, pl.ds(0, D // 4), :]
                        elif i == B22:
                            w = wqkv[p + 3, pl.ds(D // 4, D // 4), :]
                        else:
                            if i > 0:
                                for _ in range(NPIECE // NU // 4):
                                    if todo:
                                        repack(hp + (m + 1) // 3, (m + 1) % 3, todo.pop(0))
                            w = jnp.concatenate([we_u[m + _pin(hp), i, pl.ds(0, 8), :],
                                                 we_u[m, i, pl.ds(8, D // 4 - 8), :]], axis=0)
                        prods.append(
                            _dot(he[i, pl.ds(u * LA_ROWS, LA_ROWS), :], pltpu.bitcast(w, BF16)))
                    c = _strassen_out(prods)
                    for v, s0, q in zip(c, (0, 0, NSEG // 2, NSEG // 2), (p, p + 3, p, p + 3)):
                        seg[pl.ds(1 + s0 + u * n, n), q] = v.reshape(n, E, LANES)
                    if tokens is not None and m < 2:
                        for s in tokens(m * NU + u):
                            seg_put(1 + s, TOK, modulate_a(_ln(xs[s].astype(F32))).astype(BF16))

        with jax.named_scope("look_ahead"):
            for cp in w_copies(0, (0,)):
                cp.wait()
            for u in range(NPIECE):
                repack(0, 0, u)
            per = NSEG // HP // NU

            def tokens_of(hp):
                return lambda i: [((hp - HP // 2) * 2 * NU + i) * per + u for u in range(per)]
            lax.fori_loop(0, HP // 2, lambda hp, c: look_ahead(hp, False, None), None)
            x_copy(1).wait()
        with jax.named_scope("look_ahead2"):
            lax.fori_loop(HP // 2, HP - 1, lambda hp, c: look_ahead(hp, False, tokens_of(hp)), None)
            lax.fori_loop(HP - 1, HP, lambda hp, c: look_ahead(hp, True, tokens_of(hp)), None)

        with jax.named_scope("mod_b"):
            mod_chunks(2, 6)
            for j in range(ND):
                wo_copy(j).wait()
            for cp in b_copies[:len(b_copies) // 2]:
                cp.start()

        def set_lhs(mem, s, j):
            tok = seg[1 + s, pl.ds(TOK + j * R // 2, R // 2)].reshape(SEG // 2, LANES)
            tok = pltpu.bitcast(tok, BF16)
            head = jnp.concatenate([mem, tok[:16].astype(F32)[E:]], axis=0).astype(BF16)
            lhs[j] = pltpu.bitcast(jnp.concatenate([head, tok[16:]], axis=0), U32)

        def finish_tokens(s, row):
            x1 = xs[s].astype(F32) + rows(mod[2], SEG) * aout[...]
            h = _ln(x1) * rows(1.0 + mod[4], SEG) + rows(mod[3], SEG)
            seg_put(row, X1, x1)
            seg_put(row, HB, h)
            seg_put(row, HN, _ln(h))

        def weight_sums(u):
            n = wm.shape[1] // (NSEG - PLAIN_STEPS) // (H // HEAD_GROUP)
            at = pl.ds(pl.multiple_of(u * n, n), n)
            for i, v in enumerate(_strassen_rhs(*(wm[i, at, :] for i in (B11, B12, B21, B22)))):
                if i not in (B11, B22):
                    wm[i, at, :] = v

        for j in range(ND):
            set_lhs(mem0_ref[:, lanes(j)].astype(F32), 0, j)
        aout[...] = jnp.zeros_like(aout)

        def step(s, sums):
            if not sums:
                @pl.when(s == PLAIN_STEPS // 2)
                def _():
                    for cp in b_copies[len(b_copies) // 2:]:
                        cp.start()
            ri = lax.broadcasted_iota(jnp.int32, (L, LP), 0)
            ci = lax.broadcasted_iota(jnp.int32, (L, LP), 1)
            keep = ((ri < M) | (ri >= ci)) & (ci < L)
            fill = jnp.where(ci < L, -1e9, -jnp.inf).astype(F32)
            zpad = jnp.zeros((LP - L, LANES), F32)

            def project(h, m):
                p = 3 * h + m
                y = _dot(_panels(lhs, 0, ND), _panel(wqkv, p))
                parts = [y[:M], seg[1 + s, p], y[M:]]
                if m == 0:
                    return jnp.concatenate(parts, axis=0)
                return jnp.concatenate(parts + [zpad], axis=0).astype(BF16)

            def probs(q, k):
                sc = jnp.where(keep, _dot_nt(q, k) * scale, fill)
                e = jnp.exp(sc - jnp.max(sc, axis=-1, keepdims=True))
                return e / jnp.sum(e, axis=-1, keepdims=True)

            G = HEAD_GROUP
            NG = H // G
            KH = (H - G) * LANES

            prev = None
            for g in range(NG + 1):
                if g == FINISH_AT:
                    finish_tokens(jnp.maximum(s - 1, 0), s + _pin(s) * PIN_FINISH)
                if g < NG and sums and SUMS_IN_STEPS:
                    weight_sums((s - PLAIN_STEPS) * NG + g)
                heads = range(g * G, (g + 1) * G) if g < NG else ()
                q = [project(h, 0) for h in heads]
                if prev is not None:
                    pr = [probs(a, b) for a, b in zip(prev[0], prev[1])]
                k = [project(h, 1) for h in heads]
                v = [project(h, 2) for h in heads]
                if g == NG:
                    for j in range(WO_SPLIT):
                        acc[:, lanes(j)] = _dot(obuf[:, pl.ds(0, KH)], _panel(wo, j, 0, KH // 2))
                if prev is not None:
                    for u in range(G):
                        obuf[:, lanes((g - 1) * G + u)] = _dot(pr[u], prev[2][u])
                prev = (q, k, v)
            for j in list(range(WO_SPLIT, ND)) + list(range(WO_SPLIT)):
                if j < WO_SPLIT:
                    y = acc[:, lanes(j)] + _dot(
                        obuf[:, lanes(H - G, G)], _panel(wo, j, KH // 2, G * LANES // 2))
                else:
                    y = _dot(obuf[...], _panel(wo, j))
                set_lhs(y[:M], jnp.minimum(s + 1, NSEG - 1), j)
                aout[:, lanes(j)] = y[M:]

        with jax.named_scope("steps"):
            lax.fori_loop(0, PLAIN_STEPS, lambda s, c: step(s, False), None)
        with jax.named_scope("steps2"):
            for cp in b_copies:
                cp.wait()
            lax.fori_loop(PLAIN_STEPS, NSEG, lambda s, c: step(s, True), None)
        finish_tokens(NSEG - 1, NSEG)
        if not SUMS_IN_STEPS:
            with jax.named_scope("sums"):
                lax.fori_loop(0, (NSEG - PLAIN_STEPS) * (H // HEAD_GROUP), lambda u, c: weight_sums(u), None, unroll=8)

    pl.run_scoped(
        attention_phase,
        pltpu.VMEM((3 * H, D // 2, LANES), U32),
        pltpu.VMEM((ND, H * LANES // 2, LANES), U32),
        pltpu.VMEM((NSEG, SEG, D), BF16),
        pltpu.VMEM((NSEG * E, D), F32),
        pltpu.VMEM((7, NSEG * E // 2, D // 2), F32),
        pltpu.VMEM((3, 7, D // 2, LANES), BF16),
        pltpu.VMEM((ND, SEG // 2, LANES), U32),
        pltpu.VMEM((L, H * LANES), F32),
        pltpu.VMEM((SEG, D), F32),
        pltpu.VMEM((L, D), F32),
        pltpu.SemaphoreType.DMA((3 * H,)),
        pltpu.SemaphoreType.DMA((2,)),
        pltpu.SemaphoreType.DMA((ND,)),
    )

    def mixer_phase(gbuf, obuf, ops, sem_out):
        NT = S // TM
        TS = TM // SEG
        TH = TM // 2
        KS = (D // 2, D // 2, D // 2, F // 2)
        gbuf[pl.ds(0, 8), :] = jnp.zeros((8, D), F32)
        gbuf[pl.ds(S + 8, 8), :] = jnp.zeros((8, D), F32)

        def put_lhs(w, piece):
            def task(r):
                v = jnp.concatenate([piece(r), piece(TH + r)], axis=0)
                for i, a in enumerate(_strassen_lhs(*_quarters(v))):
                    ops[i, pl.ds(r, 8), pl.ds(w * D // 2, D // 2)] = a
            return [functools.partial(task, r) for r in range(0, TH, 8)]

        def run(tasks):
            for task in tasks:
                task()

        def product(w, j, pin=0, tasks=()):
            nh = (NF if w == 2 else ND) // 2
            prods = []
            for i in range(7):
                if tasks:
                    tasks.pop(0)()
                a = jnp.concatenate([ops[i + pin, :, pl.ds(w * D // 2, LANES)],
                                     ops[i, :, pl.ds(w * D // 2 + LANES, KS[w] - LANES)]], axis=1)
                prods.append(_dot(a, _panel(wm_u, i, (WM_AT[w] + j * KS[w]) // 2, KS[w] // 2)))
            return zip((0, 0, TH, TH), (j, j + nh, j, j + nh), _strassen_out(prods))

        def seg_rows(t, slot, r):
            return jnp.concatenate(
                [seg[1 + t * TS + r // SEG, slot + j * R + r % SEG // 8] for j in range(ND)], axis=1)

        def block(t, r0, slot, n):
            return 1 + t * TS + r0 // SEG, slot + n * R

        def gate_in(t):
            return put_lhs(0, lambda r: seg_rows(t, HN, r))

        def gate(t):
            for j in range(ND // 2):
                for r0, n, v in product(0, j):
                    gbuf[pl.ds(pl.multiple_of(t * TM + 8 + r0, 8), TH), lanes(n)] = (
                        jax.nn.gelu(v, approximate=True))

        def mix_in(t):
            C = D // 4

            def shifted(r):
                return jnp.concatenate([
                    gbuf[pl.ds(pl.multiple_of(t * TM + r + (8 if by > 0 else 0), 8), 16),
                         pl.ds(i * C, C)][by % 8:by % 8 + 8]
                    for i, by in enumerate((-1, 1, -2, 2))], axis=1)
            return put_lhs(1, shifted)

        def mix(t):
            for j in range(ND // 2):
                for r0, n, v in product(1, j):
                    row, slot = block(t, r0, HB, n)
                    seg_put(row, slot, seg_get(row, TS // 2, slot, 1) + v, TS // 2)

        def up_in(t):
            return put_lhs(2, lambda r: _ln(seg_rows(t, HB, r)))

        def up():
            for j in range(NF // 2):
                g = [jax.nn.gelu(v, approximate=True) for _, _, v in product(2, j)]
                for i, a in enumerate(_strassen_lhs(*g)):
                    ops[i, :, lanes(3 * ND // 2 + j)] = a

        def down(t, j, tasks):
            for r0, n, v in product(3, j, _pin(t), tasks):
                row, slot = block(t, r0, HB, n)
                y = seg_get(row, TS // 2, slot, 1) + v
                row, slot = block(t, r0, X1, n)
                y = seg_get(row, TS // 2, slot, 1) + rows(mod[5, :, lanes(n)], TH) * y
                obuf[pl.ds(pl.multiple_of(t * TM + r0, TH), TH), lanes(n)] = y.astype(BF16)

        def out_copy(t):
            r = pl.multiple_of(t * TM, TM)
            return pltpu.make_async_copy(obuf.at[pl.ds(r, TM)], out_hbm.at[pl.ds(r, TM)], sem_out.at[t])

        def tile(t, ahead):
            up()
            if ahead >= 1:
                mix(t + 1)
            if ahead >= 3:
                gate(t + 3)
            tasks = [lambda: None] * 2
            if ahead >= 3:
                tasks += gate_in(jnp.minimum(t + 4, NT - 1))
            if ahead >= 1:
                tasks += up_in(t + 1)
            if ahead >= 2:
                tasks += mix_in(t + 2)
            for j in range(ND // 2):
                down(t, j, tasks)
            run(tasks)
            out_copy(t).start()

        with jax.named_scope("gate"):
            run(gate_in(0))
            gate(0)
            run(gate_in(1))
            gate(1)
            run(mix_in(0))
            mix(0)
            run(gate_in(2))
            gate(2)
            run(up_in(0))
            run(mix_in(1))
            run(gate_in(3))
        with jax.named_scope("mlp"):
            lax.fori_loop(0, NT - 3, lambda t, c: tile(t, 3), None)
        with jax.named_scope("mlp2"):
            for t in range(NT - 3, NT):
                tile(t, NT - 1 - t)
        for t in range(NT):
            out_copy(t).wait()

    pl.run_scoped(
        mixer_phase,
        pltpu.VMEM((S + 16, D), F32),
        pltpu.VMEM((S, D), BF16),
        pltpu.VMEM((7, TM // 2, 3 * D // 2 + F // 2), F32),
        pltpu.SemaphoreType.DMA((S // TM,)))


@functools.partial(jax.jit, static_argnames=("A_seg_len",))
def pallas_adaLN_cond__memory_aug_recurrent_mem_tr__mixer_s_mlp__prompt_kernel(
    A_x, A_mem0, A_Wq, A_Wk, A_Wv, A_Wo, A_seg_len, B_x, B_w1, B_w2, B_w3, B_w4, c, w_mod,
):
    del B_x
    B, S, D = A_x.shape
    H, Dh = A_Wq.shape[1:]
    M = A_mem0.shape[1]
    F = B_w3.shape[1]
    SEG = A_seg_len
    assert B == 1 and Dh == LANES and M == 8 and SEG % 16 == 0 and S % SEG == 0
    ND, NF = D // LANES, F // LANES
    hbm = pl.BlockSpec(memory_space=pl.ANY)
    vmem = pl.BlockSpec(memory_space=pltpu.VMEM)
    out = pl.pallas_call(
        functools.partial(_kernel, S=S, D=D, H=H, M=M, SEG=SEG, F=F),
        out_shape=jax.ShapeDtypeStruct((S, D), A_x.dtype),
        in_specs=[hbm, vmem, hbm, hbm, hbm, hbm, hbm, hbm, hbm, hbm, vmem, hbm],
        out_specs=hbm,
        scratch_shapes=[
            pltpu.VMEM((7, (ND + NF) * D // 2, LANES), BF16),
            pltpu.VMEM((S // SEG + 1, 3 * H + ND * SEG // 16, 8, LANES), F32),
            pltpu.VMEM((6, 8, D), F32),
            pltpu.SemaphoreType.DMA((6 * ND,)),
            pltpu.SemaphoreType.DMA((2 * (3 * ND + NF),)),
        ],
        compiler_params=pltpu.CompilerParams(vmem_limit_bytes=124 * 1024 * 1024),
    )(A_x.reshape(S // SEG, SEG, D), A_mem0.reshape(M, D),
      *(w.reshape(D // 2, 2, H, Dh) for w in (A_Wq, A_Wk, A_Wv)),
      A_Wo.reshape(H * Dh, D), B_w1, B_w2, B_w3, B_w4, c, w_mod)
    return out.reshape(B, S, D)
```

```python
import functools

import jax
import jax.numpy as jnp
import numpy as np
from jax import lax
import jax.experimental.pallas as pl
import jax.experimental.pallas.tpu as pltpu

F32 = jnp.float32
BF16 = jnp.bfloat16
U32 = jnp.uint32
LANES = 128
EPS = 1e-5

HEAD_GROUP = 4
PREFETCH = 3
FINISH_AT = 2
SUMS_IN_STEPS = True
PIN_FINISH = 0
TASK_LAG = 4
LA_LAG = 5
EXTRA = (0, 0, 0, 0, 4, 4, 4, 4, 4, 4, 4, 4, 4, 10, 10, 0)
WO_SPLIT = 6
PLAIN_STEPS = 16
LA_ROWS = 64
TM = 128

B11, B12, B21, B22 = 1, 2, 3, 4


def _ln(x):
    m = jnp.mean(x, axis=-1, keepdims=True)
    d = x - m
    v = jnp.mean(d * d, axis=-1, keepdims=True)
    return d * lax.rsqrt(v + EPS)


def _dot(a, b):
    return jnp.dot(a, b, preferred_element_type=F32)


def _dot_nt(a, b):
    return lax.dot_general(a, b, (((1,), (1,)), ((), ())), preferred_element_type=F32)


def _panel(ref, p, r0=None, nr=None):
    w = ref[p] if r0 is None else ref[p, pl.ds(r0, nr), :]
    return pltpu.bitcast(w, BF16)


def _panels(ref, p0, n):
    return jnp.concatenate([_panel(ref, p0 + j) for j in range(n)], axis=1)


def _strassen_lhs(a11, a12, a21, a22):
    return [a11 + a22, a21 + a22, a11, a22, a11 + a12, a21 - a11, a12 - a22]


def _strassen_rhs(b11, b12, b21, b22):
    c11, c12, c21, c22 = (b.astype(F32) for b in (b11, b12, b21, b22))
    return [(c11 + c22).astype(BF16), b11, (c12 - c22).astype(BF16), (c21 - c11).astype(BF16),
            b22, (c11 + c12).astype(BF16), (c21 + c22).astype(BF16)]


def _strassen_out(m):
    return m[0] + m[3] - m[4] + m[6], m[2] + m[4], m[1] + m[3], m[0] - m[1] + m[2] + m[5]


def _quarters(v):
    r, c = v.shape[0] // 2, v.shape[1] // 2
    return v[:r, :c], v[:r, c:], v[r:, :c], v[r:, c:]


def _pin(i):
    return i >> 24


def _kernel(x_hbm, mem0_ref, wq_hbm, wk_hbm, wv_hbm, wo_hbm, w1_hbm, w2_hbm, w3_hbm, w4_hbm,
            c_ref, wmod_hbm, out_hbm,
            wm, seg, mod, sem_mod, sem_b,
            *, S, D, H, M, SEG, F):
    NSEG = S // SEG
    E = M
    L = M + SEG
    LP = -(-L // 16) * 16
    ND = D // LANES
    NF = F // LANES
    R = SEG // 8
    scale = LANES ** -0.5
    TOK = 3 * H
    X1, HB, HN = 0, R * ND, 2 * R * ND

    def lanes(j, n=1):
        start = j * LANES
        return pl.ds(start if isinstance(j, int) else pl.multiple_of(start, LANES), n * LANES)

    def seg_put(row, slot, v, n=1):
        if v.dtype != F32:
            v = pltpu.bitcast(v, F32)
        r = v.shape[0] // (8 * n)
        for j in range(v.shape[1] // LANES):
            seg[pl.ds(row, n), pl.ds(slot + j * r, r)] = (
                v[:, j * LANES:(j + 1) * LANES].reshape(n, r, 8, LANES))

    def seg_get(row, n, slot, cols=ND):
        return jnp.concatenate(
            [seg[pl.ds(row, n), pl.ds(slot + j * R, R)].reshape(n * SEG, LANES) for j in range(cols)],
            axis=1)

    w_u = [r.bitcast(U32) for r in (wq_hbm, wk_hbm, wv_hbm)]
    wo_u = wo_hbm.bitcast(U32)
    wm_u = wm.bitcast(U32)

    WM_AT = np.cumsum([0, ND * D // 4, ND * D // 4, NF * D // 4]).tolist()
    b_copies = []
    for w, at in zip((w1_hbm, w2_hbm, w3_hbm, w4_hbm), WM_AT):
        kh, nh = w.shape[0] // 2, w.shape[1] // LANES // 2
        for j in range(nh):
            for i, r0, p in ((B11, 0, j), (B12, 0, j + nh), (B21, kh, j), (B22, kh, j + nh)):
                b_copies.append(pltpu.make_async_copy(
                    w.at[pl.ds(r0, kh), lanes(p)], wm.at[i, pl.ds(at + j * kh, kh)],
                    sem_b.at[len(b_copies)]))

    def mod_place(j):
        third = j // (2 * ND)
        return third + 4 * ((third + 1) // 2), j % (2 * ND)

    def mod_copy(j):
        i, k = mod_place(j)
        start = k * D if isinstance(j, int) else pl.multiple_of(k * D, D)
        return pltpu.make_async_copy(
            wmod_hbm.at[:, lanes(j)], wm.at[i, pl.ds(start, D)], sem_mod.at[j])

    def mod_chunks(lo, hi):
        cv = c_ref[...].astype(F32)
        sc = jnp.broadcast_to(cv * jax.nn.sigmoid(cv), (8, D))
        for j in range(lo * ND, hi * ND):
            mod_copy(j).wait()
        for j in range(lo * ND, hi * ND):
            i, k = mod_place(j)
            mod[j // ND, :, lanes(j % ND)] = _dot(sc, _panel(wm_u, i, k * D // 2, D // 2))

    def rows(v, n):
        return jnp.concatenate([v] * (n // 8), axis=0)

    def attention_phase(wqkv, wo, xs, xn, he, we, lhs, obuf, aout, acc, sem_w, sem_x, sem_wo):
        HP = H // 2

        def w_copies(hp, which=(0, 1, 2)):
            return [pltpu.make_async_copy(w_u[m].at[:, i, hp, :], wqkv.at[6 * hp + 3 * i + m],
                                          sem_w.at[6 * hp + 3 * i + m])
                    for m in which for i in range(2)]

        def wo_copy(j):
            part = pl.ds(j % 4 * (wo.shape[1] // 4), wo.shape[1] // 4)
            return pltpu.make_async_copy(
                wo_u.at[part, lanes(j // 4)], wo.at[j // 4, part], sem_wo.at[j])

        def x_copy(i):
            sl = pl.ds(i * E, E)
            return pltpu.make_async_copy(x_hbm.at[:, sl, :], xs.at[:, sl, :], sem_x.at[i])

        def modulate_a(n):
            return n * rows(1.0 + mod[1], n.shape[0]) + rows(mod[0], n.shape[0])

        x_copy(0).start()
        for j in range(2 * ND):
            mod_copy(j).start()

        with jax.named_scope("early_ln"):
            x_copy(0).wait()
            for cp in w_copies(0):
                cp.start()

            def early_norm(t, carry):
                xv = xs[pl.ds(t * 16, 16), pl.ds(0, E), :].astype(F32).reshape(16 * E, D)
                xn[pl.ds(pl.multiple_of(t * 16 * E, 16 * E), 16 * E), :] = _ln(xv)
                return carry
            lax.fori_loop(0, NSEG // 16, early_norm, 0)

        with jax.named_scope("mod_a"):
            mod_chunks(0, 2)
            for hp in range(1, PREFETCH):
                for cp in w_copies(hp):
                    cp.start()

            def early_operands(t, carry):
                top, low = (
                    modulate_a(xn[pl.ds(pl.multiple_of(r0 + t * 32, 32), 32), :])
                    for r0 in (0, NSEG * E // 2))
                for i, v in enumerate(_strassen_lhs(*_quarters(jnp.concatenate([top, low], axis=0)))):
                    he[i, pl.ds(pl.multiple_of(t * 32, 32), 32), :] = v
                return carry
            lax.fori_loop(0, NSEG * E // 64, early_operands, 0)

        NU = NSEG * E // 2 // LA_ROWS

        NPIECE = 16
        we_u = we.bitcast(U32)

        def repack(hp, m, u, after=lambda v: v):
            p = 6 * hp + m
            nr = D // 4 // NPIECE
            w = []
            for r0 in (u * nr, D // 4 + u * nr):
                a, b = after(wqkv[p, pl.ds(r0, nr), :]), wqkv[p + 3, pl.ds(r0, nr), :]
                w.append((a & np.uint32(0xFFFF)) | (b << 16))
                w.append((a >> 16) | (b & np.uint32(0xFFFF0000)))
                wqkv[p, pl.ds(r0, nr), :], wqkv[p + 3, pl.ds(r0, nr), :] = w[-2:]
            for i, v in enumerate(_strassen_rhs(*(pltpu.bitcast(v, BF16) for v in w))):
                if i in (B11, B22):
                    we_u[m, i, pl.ds(u * nr, nr), :] = w[i - B11]
                else:
                    we[m, i, pl.ds(2 * u * nr, 2 * nr), :] = v

        rest = ([functools.partial(mod_copy, j) for j in range(2 * ND, 5 * ND)]
                + [functools.partial(wo_copy, j) for j in range(4 * ND)])
        extra = []
        for k, n in enumerate(EXTRA):
            extra.append(rest[:n] + ([functools.partial(x_copy, k)] if 1 <= k <= 3 else []))
            rest = rest[n:]
        assert not rest and len(extra) == HP

        def look_ahead(hp, pin, span, last, tokens):
            @pl.when(hp + PREFETCH < HP)
            def _():
                for cp in w_copies(hp + PREFETCH):
                    cp.start()

            for k in span:
                @pl.when(hp == k)
                def _():
                    for cp in extra[k]:
                        cp().start()
            for cp in w_copies(hp, (1, 2)) + ([] if last else w_copies(hp + 1, (0,))):
                cp.wait()
            n = LA_ROWS // E
            done = []
            for m in range(3):
                p = 6 * hp + m
                todo = list(range(NPIECE)) if m < 2 or not last else []
                for u in range(NU):
                    prods = []
                    for i in range(7):
                        if todo and len(done) >= LA_LAG and i % 3 != 2:
                            y = pltpu.bitcast(done[-LA_LAG][:D // 4 // NPIECE], U32)
                            repack(hp + (m + 1) // 3, (m + 1) % 3, todo.pop(0),
                                   lambda v: jnp.where(pin == 0, v, y))
                        w = jnp.concatenate([we_u[m + pin, i, pl.ds(0, 8), :],
                                             we_u[m, i, pl.ds(8, D // 4 - 8), :]], axis=0)
                        prods.append(
                            _dot(he[i, pl.ds(u * LA_ROWS, LA_ROWS), :], pltpu.bitcast(w, BF16)))
                        done.append(prods[-1])
                    c = _strassen_out(prods)
                    for v, s0, q in zip(c, (0, 0, NSEG // 2, NSEG // 2), (p, p + 3, p, p + 3)):
                        seg[pl.ds(1 + s0 + u * n, n), q] = v.reshape(n, E, LANES)
                    if tokens is not None and m < 2:
                        for s in tokens(m * NU + u):
                            seg_put(1 + s + pin, TOK,
                                    modulate_a(_ln(xs[s].astype(F32))).astype(BF16))
                assert not todo
            return pin

        with jax.named_scope("look_ahead"):
            for cp in w_copies(0, (0,)):
                cp.wait()
            for u in range(NPIECE):
                repack(0, 0, u)
            per = NSEG // HP // NU

            def tokens_of(hp):
                return lambda i: [((hp - HP // 2) * 2 * NU + i) * per + u for u in range(per)]
            lax.fori_loop(0, HP // 2, lambda hp, c: look_ahead(
                hp, _pin(hp), range(HP // 2), False, None), 0)
            for i in range(1, R):
                x_copy(i).wait()
        with jax.named_scope("look_ahead2"):
            pin = lax.fori_loop(
                HP // 2, HP - 1, lambda hp, c: look_ahead(
                    hp, _pin(hp), range(HP // 2, HP - 1), False, tokens_of(hp)), 0)
            look_ahead(HP - 1, pin, [HP - 1], True, tokens_of(HP - 1))

        with jax.named_scope("mod_b"):
            mod_chunks(2, 5)
            for j in range(4 * ND):
                wo_copy(j).wait()
            for j in range(5 * ND, 6 * ND):
                mod_copy(j).start()
            for cp in b_copies[:len(b_copies) // 2]:
                cp.start()

        def set_lhs(mem, s, j):
            tok = seg[1 + s, pl.ds(TOK + j * R // 2, R // 2)].reshape(SEG // 2, LANES)
            tok = pltpu.bitcast(tok, BF16)
            head = jnp.concatenate([mem, tok[:16].astype(F32)[E:]], axis=0).astype(BF16)
            lhs[j] = pltpu.bitcast(jnp.concatenate([head, tok[16:]], axis=0), U32)

        def finish_tokens(s, row):
            x1 = xs[s].astype(F32) + rows(mod[2], SEG) * aout[...]
            h = _ln(x1) * rows(1.0 + mod[4], SEG) + rows(mod[3], SEG)
            seg_put(row, X1, x1)
            seg_put(row, HB, h)
            seg_put(row, HN, _ln(h))

        def weight_sums(u):
            n = wm.shape[1] // (NSEG - PLAIN_STEPS) // (H // HEAD_GROUP)
            at = pl.ds(pl.multiple_of(u * n, n), n)
            for i, v in enumerate(_strassen_rhs(*(wm[i, at, :] for i in (B11, B12, B21, B22)))):
                if i not in (B11, B22):
                    wm[i, at, :] = v

        for j in range(ND):
            set_lhs(mem0_ref[:, lanes(j)].astype(F32), 0, j)
        aout[...] = jnp.zeros_like(aout)

        def step(s, sums):
            if not sums:
                @pl.when(s == PLAIN_STEPS // 2)
                def _():
                    for cp in b_copies[len(b_copies) // 2:]:
                        cp.start()
            ri = lax.broadcasted_iota(jnp.int32, (L, LP), 0)
            ci = lax.broadcasted_iota(jnp.int32, (L, LP), 1)
            keep = ((ri < M) | (ri >= ci)) & (ci < L)
            fill = jnp.where(ci < L, -1e9, -jnp.inf).astype(F32)
            zpad = jnp.zeros((LP - L, LANES), F32)

            def project(h, m):
                p = 3 * h + m
                y = _dot(_panels(lhs, 0, ND), _panel(wqkv, p))
                parts = [y[:M], seg[1 + s, p], y[M:]]
                if m == 0:
                    return jnp.concatenate(parts, axis=0)
                return jnp.concatenate(parts + [zpad], axis=0).astype(BF16)

            def probs(q, k):
                sc = jnp.where(keep, _dot_nt(q, k) * scale, fill)
                e = jnp.exp(sc - jnp.max(sc, axis=-1, keepdims=True))
                return e / jnp.sum(e, axis=-1, keepdims=True)

            G = HEAD_GROUP
            NG = H // G
            KH = (H - G) * LANES

            prev = None
            for g in range(NG + 1):
                if g == FINISH_AT:
                    finish_tokens(jnp.maximum(s - 1, 0), s + _pin(s) * PIN_FINISH)
                if g < NG and sums and SUMS_IN_STEPS:
                    weight_sums((s - PLAIN_STEPS) * NG + g)
                heads = range(g * G, (g + 1) * G) if g < NG else ()
                q = [project(h, 0) for h in heads]
                if prev is not None:
                    pr = [probs(a, b) for a, b in zip(prev[0], prev[1])]
                k = [project(h, 1) for h in heads]
                v = [project(h, 2) for h in heads]
                if g == NG:
                    for j in range(WO_SPLIT):
                        acc[:, lanes(j)] = _dot(obuf[:, pl.ds(0, KH)], _panel(wo, j, 0, KH // 2))
                if prev is not None:
                    for u in range(G):
                        obuf[:, lanes((g - 1) * G + u)] = _dot(pr[u], prev[2][u])
                prev = (q, k, v)
            for j in list(range(WO_SPLIT, ND)) + list(range(WO_SPLIT)):
                if j < WO_SPLIT:
                    y = acc[:, lanes(j)] + _dot(
                        obuf[:, lanes(H - G, G)], _panel(wo, j, KH // 2, G * LANES // 2))
                else:
                    y = _dot(obuf[...], _panel(wo, j))
                set_lhs(y[:M], jnp.minimum(s + 1, NSEG - 1), j)
                aout[:, lanes(j)] = y[M:]

        with jax.named_scope("steps"):
            lax.fori_loop(0, PLAIN_STEPS, lambda s, c: step(s, False), None)
        with jax.named_scope("steps2"):
            mod_chunks(5, 6)
            for cp in b_copies:
                cp.wait()
            lax.fori_loop(PLAIN_STEPS, NSEG, lambda s, c: step(s, True), None)
        finish_tokens(NSEG - 1, NSEG)
        if not SUMS_IN_STEPS:
            with jax.named_scope("sums"):
                lax.fori_loop(0, (NSEG - PLAIN_STEPS) * (H // HEAD_GROUP), lambda u, c: weight_sums(u), None, unroll=8)

    pl.run_scoped(
        attention_phase,
        pltpu.VMEM((3 * H, D // 2, LANES), U32),
        pltpu.VMEM((ND, H * LANES // 2, LANES), U32),
        pltpu.VMEM((NSEG, SEG, D), BF16),
        pltpu.VMEM((NSEG * E, D), F32),
        pltpu.VMEM((7, NSEG * E // 2, D // 2), F32),
        pltpu.VMEM((3, 7, D // 2, LANES), BF16),
        pltpu.VMEM((ND, SEG // 2, LANES), U32),
        pltpu.VMEM((L, H * LANES), F32),
        pltpu.VMEM((SEG, D), F32),
        pltpu.VMEM((L, D), F32),
        pltpu.SemaphoreType.DMA((3 * H,)),
        pltpu.SemaphoreType.DMA((R,)),
        pltpu.SemaphoreType.DMA((4 * ND,)),
    )

    def mixer_phase(gbuf, obuf, ops, sem_out):
        NT = S // TM
        TS = TM // SEG
        TH = TM // 2
        KS = (D // 2, D // 2, D // 2, F // 2)
        gbuf[pl.ds(0, 8), :] = jnp.zeros((8, D), F32)
        gbuf[pl.ds(S + 8, 8), :] = jnp.zeros((8, D), F32)

        def put_lhs(w, piece):
            def task(r, after=lambda v: v):
                v = after(jnp.concatenate([piece(r), piece(TH + r)], axis=0))
                if w == 2:
                    v = _ln(v)
                for i, a in enumerate(_strassen_lhs(*_quarters(v))):
                    ops[i, pl.ds(r, 8), pl.ds(w * D // 2, D // 2)] = a
            return [functools.partial(task, r) for r in range(0, TH, 8)]

        def run(tasks):
            for task in tasks:
                task()

        def product(w, j, pin=0, tasks=(), done=None):
            nh = (NF if w == 2 else ND) // 2
            prods = []
            for i in range(7):
                if tasks and len(done) >= TASK_LAG:
                    m = jnp.concatenate([done[-TASK_LAG][:16]] * ND, axis=1)
                    tasks.pop(0)(lambda v: jnp.where(pin == 0, v, m))
                a = jnp.concatenate([ops[i + pin, :, pl.ds(w * D // 2, LANES)],
                                     ops[i, :, pl.ds(w * D // 2 + LANES, KS[w] - LANES)]], axis=1)
                prods.append(_dot(a, _panel(wm_u, i, (WM_AT[w] + j * KS[w]) // 2, KS[w] // 2)))
                if done is not None:
                    done.append(prods[-1])
            return zip((0, 0, TH, TH), (j, j + nh, j, j + nh), _strassen_out(prods))

        def seg_rows(t, slot, r):
            return jnp.concatenate(
                [seg[1 + t * TS + r // SEG, slot + j * R + r % SEG // 8] for j in range(ND)], axis=1)

        def block(t, r0, slot, n):
            return 1 + t * TS + r0 // SEG, slot + n * R

        def gate_in(t):
            return put_lhs(0, lambda r: seg_rows(t, HN, r))

        def gate(t):
            for j in range(ND // 2):
                for r0, n, v in product(0, j):
                    gbuf[pl.ds(pl.multiple_of(t * TM + 8 + r0, 8), TH), lanes(n)] = (
                        jax.nn.gelu(v, approximate=True))

        def mix_in(t):
            C = D // 4

            def shifted(r):
                return jnp.concatenate([
                    gbuf[pl.ds(pl.multiple_of(t * TM + r + (8 if by > 0 else 0), 8), 16),
                         pl.ds(i * C, C)][by % 8:by % 8 + 8]
                    for i, by in enumerate((-1, 1, -2, 2))], axis=1)
            return put_lhs(1, shifted)

        def mix(t):
            for j in range(ND // 2):
                for r0, n, v in product(1, j):
                    row, slot = block(t, r0, HB, n)
                    seg_put(row, slot, seg_get(row, TS // 2, slot, 1) + v, TS // 2)

        def up_in(t):
            return put_lhs(2, lambda r: seg_rows(t, HB, r))

        def up():
            for j in range(NF // 2):
                g = [jax.nn.gelu(v, approximate=True) for _, _, v in product(2, j)]
                for i, a in enumerate(_strassen_lhs(*g)):
                    ops[i, :, lanes(3 * ND // 2 + j)] = a

        def down(t, j, pin, tasks, done):
            for r0, n, v in product(3, j, pin, tasks, done):
                row, slot = block(t, r0, HB, n)
                y = seg_get(row, TS // 2, slot, 1) + v
                row, slot = block(t, r0, X1, n)
                y = seg_get(row, TS // 2, slot, 1) + rows(mod[5, :, lanes(n)], TH) * y
                obuf[pl.ds(pl.multiple_of(t * TM + r0, TH), TH), lanes(n)] = y.astype(BF16)

        def out_copy(t):
            r = pl.multiple_of(t * TM, TM)
            return pltpu.make_async_copy(obuf.at[pl.ds(r, TM)], out_hbm.at[pl.ds(r, TM)], sem_out.at[t])

        def tile(t, pin, ahead):
            up()
            if ahead >= 1:
                mix(t + 1)
            if ahead >= 3:
                gate(t + 3)
            tasks, done = [], []
            if ahead >= 3:
                tasks += gate_in(jnp.minimum(t + 4, NT - 1))
            if ahead >= 1:
                tasks += up_in(t + 1)
            if ahead >= 2:
                tasks += mix_in(t + 2)
            for j in range(ND // 2):
                down(t, j, pin, tasks, done)
            run(tasks)
            out_copy(t).start()
            return pin

        with jax.named_scope("gate"):
            run(gate_in(0))
            gate(0)
            run(gate_in(1))
            gate(1)
            run(mix_in(0))
            mix(0)
            run(gate_in(2))
            gate(2)
            run(up_in(0))
            run(mix_in(1))
            run(gate_in(3))
        with jax.named_scope("mlp"):
            pin = lax.fori_loop(0, NT - 3, lambda t, c: tile(t, _pin(t), 3), 0)
        with jax.named_scope("mlp2"):
            for t in range(NT - 3, NT):
                tile(t, pin, NT - 1 - t)
        for t in range(NT):
            out_copy(t).wait()

    pl.run_scoped(
        mixer_phase,
        pltpu.VMEM((S + 16, D), F32),
        pltpu.VMEM((S, D), BF16),
        pltpu.VMEM((7, TM // 2, 3 * D // 2 + F // 2), F32),
        pltpu.SemaphoreType.DMA((S // TM,)))


@functools.partial(jax.jit, static_argnames=("A_seg_len",))
def pallas_adaLN_cond__memory_aug_recurrent_mem_tr__mixer_s_mlp__prompt_kernel(
    A_x, A_mem0, A_Wq, A_Wk, A_Wv, A_Wo, A_seg_len, B_x, B_w1, B_w2, B_w3, B_w4, c, w_mod,
):
    del B_x
    B, S, D = A_x.shape
    H, Dh = A_Wq.shape[1:]
    M = A_mem0.shape[1]
    F = B_w3.shape[1]
    SEG = A_seg_len
    assert B == 1 and Dh == LANES and M == 8 and SEG % 16 == 0 and S % SEG == 0
    ND, NF = D // LANES, F // LANES
    hbm = pl.BlockSpec(memory_space=pl.ANY)
    vmem = pl.BlockSpec(memory_space=pltpu.VMEM)
    out = pl.pallas_call(
        functools.partial(_kernel, S=S, D=D, H=H, M=M, SEG=SEG, F=F),
        out_shape=jax.ShapeDtypeStruct((S, D), A_x.dtype),
        in_specs=[hbm, vmem, hbm, hbm, hbm, hbm, hbm, hbm, hbm, hbm, vmem, hbm],
        out_specs=hbm,
        scratch_shapes=[
            pltpu.VMEM((7, (ND + NF) * D // 2, LANES), BF16),
            pltpu.VMEM((S // SEG + 1, 3 * H + ND * SEG // 16, 8, LANES), F32),
            pltpu.VMEM((6, 8, D), F32),
            pltpu.SemaphoreType.DMA((6 * ND,)),
            pltpu.SemaphoreType.DMA((2 * (3 * ND + NF),)),
        ],
        compiler_params=pltpu.CompilerParams(vmem_limit_bytes=124 * 1024 * 1024),
    )(A_x.reshape(S // SEG, SEG, D), A_mem0.reshape(M, D),
      *(w.reshape(D // 2, 2, H, Dh) for w in (A_Wq, A_Wk, A_Wv)),
      A_Wo.reshape(H * Dh, D), B_w1, B_w2, B_w3, B_w4, c, w_mod)
    return out.reshape(B, S, D)
```

```python
import functools

import jax
import jax.numpy as jnp
import numpy as np
from jax import lax
import jax.experimental.pallas as pl
import jax.experimental.pallas.tpu as pltpu

F32 = jnp.float32
BF16 = jnp.bfloat16
U32 = jnp.uint32
LANES = 128
EPS = 1e-5

HEAD_GROUP = 4
PREFETCH = 3
FINISH_AT = 2
SUMS_IN_STEPS = True
PIN_FINISH = 0
TASK_LAG = 4
MOD_FIRST = 2
UNROLL = 2
KSPLIT = 4
LA_LAG = 5
EXTRA = (0, 0, 0, 0, 4, 4, 4, 4, 4, 4, 4, 4, 4, 10, 10, 0)
WO_SPLIT = 4
PLAIN_STEPS = 16
LA_ROWS = 64
TM = 128

B11, B12, B21, B22 = 1, 2, 3, 4


def _ln(x):
    m = jnp.mean(x, axis=-1, keepdims=True)
    d = x - m
    v = jnp.mean(d * d, axis=-1, keepdims=True)
    return d * lax.rsqrt(v + EPS)


def _dot(a, b):
    return jnp.dot(a, b, preferred_element_type=F32)


def _dot_nt(a, b):
    return lax.dot_general(a, b, (((1,), (1,)), ((), ())), preferred_element_type=F32)


def _panel(ref, p, r0=None, nr=None):
    w = ref[p] if r0 is None else ref[p, pl.ds(r0, nr), :]
    return pltpu.bitcast(w, BF16)


def _panels(ref, p0, n):
    return jnp.concatenate([_panel(ref, p0 + j) for j in range(n)], axis=1)


def _strassen_lhs(a11, a12, a21, a22):
    return [a11 + a22, a21 + a22, a11, a22, a11 + a12, a21 - a11, a12 - a22]


def _strassen_rhs(b11, b12, b21, b22):
    c11, c12, c21, c22 = (b.astype(F32) for b in (b11, b12, b21, b22))
    return [(c11 + c22).astype(BF16), b11, (c12 - c22).astype(BF16), (c21 - c11).astype(BF16),
            b22, (c11 + c12).astype(BF16), (c21 + c22).astype(BF16)]


def _strassen_out(m):
    return m[0] + m[3] - m[4] + m[6], m[2] + m[4], m[1] + m[3], m[0] - m[1] + m[2] + m[5]


def _quarters(v):
    r, c = v.shape[0] // 2, v.shape[1] // 2
    return v[:r, :c], v[:r, c:], v[r:, :c], v[r:, c:]


def _pin(i):
    return i >> 24


def _kernel(x_hbm, mem0_ref, wq_hbm, wk_hbm, wv_hbm, wo_hbm, w1_hbm, w2_hbm, w3_hbm, w4_hbm,
            c_ref, wmod_hbm, out_hbm,
            wm, seg, mod, sem_mod, sem_b,
            *, S, D, H, M, SEG, F):
    NSEG = S // SEG
    E = M
    L = M + SEG
    LP = -(-L // 16) * 16
    ND = D // LANES
    NF = F // LANES
    R = SEG // 8
    scale = LANES ** -0.5
    TOK = 3 * H
    X1, HB, HN = 0, R * ND, 2 * R * ND

    def lanes(j, n=1):
        start = j * LANES
        return pl.ds(start if isinstance(j, int) else pl.multiple_of(start, LANES), n * LANES)

    def seg_put(row, slot, v, n=1):
        if v.dtype != F32:
            v = pltpu.bitcast(v, F32)
        r = v.shape[0] // (8 * n)
        for j in range(v.shape[1] // LANES):
            seg[pl.ds(row, n), pl.ds(slot + j * r, r)] = (
                v[:, j * LANES:(j + 1) * LANES].reshape(n, r, 8, LANES))

    def seg_get(row, n, slot, cols=ND):
        return jnp.concatenate(
            [seg[pl.ds(row, n), pl.ds(slot + j * R, R)].reshape(n * SEG, LANES) for j in range(cols)],
            axis=1)

    w_u = [r.bitcast(U32) for r in (wq_hbm, wk_hbm, wv_hbm)]
    wo_u = wo_hbm.bitcast(U32)
    wm_u = wm.bitcast(U32)

    WM_AT = np.cumsum([0, ND * D // 4, ND * D // 4, NF * D // 4]).tolist()
    b_copies = []
    for w, at in zip((w1_hbm, w2_hbm, w3_hbm, w4_hbm), WM_AT):
        kh, nh = w.shape[0] // 2, w.shape[1] // LANES // 2
        for j in range(nh):
            for i, r0, p in ((B11, 0, j), (B12, 0, j + nh), (B21, kh, j), (B22, kh, j + nh)):
                b_copies.append(pltpu.make_async_copy(
                    w.at[pl.ds(r0, kh), lanes(p)], wm.at[i, pl.ds(at + j * kh, kh)],
                    sem_b.at[0]))

    def mod_place(j):
        third = j // (2 * ND)
        return third + 4 * ((third + 1) // 2), j % (2 * ND)

    def mod_copy(j):
        i, k = mod_place(j)
        return pltpu.make_async_copy(
            wmod_hbm.at[:, lanes(j)], wm.at[i, pl.ds(k * D, D)], sem_mod.at[j // ND])

    def mod_chunks(lo, hi, arrived=lambda: None):
        cv = c_ref[...].astype(F32)
        sc = jnp.broadcast_to(cv * jax.nn.sigmoid(cv), (8, D))
        for j in range(lo * ND, hi * ND):
            mod_copy(j).wait()
        arrived()
        for j in range(lo * ND, hi * ND):
            i, k = mod_place(j)
            mod[j // ND, :, lanes(j % ND)] = _dot(sc, _panel(wm_u, i, k * D // 2, D // 2))

    def rows(v, n):
        return jnp.concatenate([v] * (n // 8), axis=0)

    def attention_phase(wqkv, wo, xs, xn, he, we, lhs, obuf, aout, acc, sem_w, sem_x, sem_wo):
        HP = H // 2

        def w_copies(hp, which=(0, 1, 2)):
            return [pltpu.make_async_copy(w_u[m].at[:, i, hp, :], wqkv.at[6 * hp + 3 * i + m],
                                          sem_w.at[3 * hp + m])
                    for m in which for i in range(2)]

        def wo_copy(j):
            part = pl.ds(j % 4 * (wo.shape[1] // 4), wo.shape[1] // 4)
            return pltpu.make_async_copy(
                wo_u.at[part, lanes(j // 4)], wo.at[j // 4, part], sem_wo.at[0])

        def x_copy(i):
            sl = pl.ds(i * E, E)
            return pltpu.make_async_copy(x_hbm.at[:, sl, :], xs.at[:, sl, :], sem_x.at[i])

        def modulate_a(n):
            return n * rows(1.0 + mod[1], n.shape[0]) + rows(mod[0], n.shape[0])

        NU = NSEG * E // 2 // LA_ROWS

        NPIECE = 16
        we_u = we.bitcast(U32)

        def repack(hp, m, u, after=lambda v: v):
            p = 6 * hp + m
            nr = D // 4 // NPIECE
            w = []
            for r0 in (u * nr, D // 4 + u * nr):
                a, b = after(wqkv[p, pl.ds(r0, nr), :]), wqkv[p + 3, pl.ds(r0, nr), :]
                w.append((a & np.uint32(0xFFFF)) | (b << 16))
                w.append((a >> 16) | (b & np.uint32(0xFFFF0000)))
                wqkv[p, pl.ds(r0, nr), :], wqkv[p + 3, pl.ds(r0, nr), :] = w[-2:]
            for i, v in enumerate(_strassen_rhs(*(pltpu.bitcast(v, BF16) for v in w))):
                if i in (B11, B22):
                    we_u[m, i, pl.ds(u * nr, nr), :] = w[i - B11]
                else:
                    we[m, i, pl.ds(2 * u * nr, 2 * nr), :] = v

        x_copy(0).start()
        for j in range(MOD_FIRST):
            mod_copy(j).start()
        for cp in w_copies(0, (0,)):
            cp.start()

        with jax.named_scope("early_ln"):
            x_copy(0).wait()
            for j in range(MOD_FIRST, 2 * ND):
                mod_copy(j).start()

            def early_norm(t, carry):
                xv = xs[pl.ds(t * 16, 16), pl.ds(0, E), :].astype(F32).reshape(16 * E, D)
                xn[pl.ds(pl.multiple_of(t * 16 * E, 16 * E), 16 * E), :] = _ln(xv)
                return carry
            lax.fori_loop(0, NSEG // 16, early_norm, 0)

        with jax.named_scope("mod_a"):
            for cp in w_copies(0, (0,)):
                cp.wait()
            for u in range(NPIECE):
                repack(0, 0, u)
            mod_chunks(0, 2, lambda: [cp.start() for cp in w_copies(0, (1, 2)) + w_copies(1, (0,))])
            for cp in w_copies(1, (1, 2)):
                cp.start()
            for hp in range(2, PREFETCH):
                for cp in w_copies(hp):
                    cp.start()

            def early_operands(t, carry):
                top, low = (
                    modulate_a(xn[pl.ds(pl.multiple_of(r0 + t * 32, 32), 32), :])
                    for r0 in (0, NSEG * E // 2))
                for i, v in enumerate(_strassen_lhs(*_quarters(jnp.concatenate([top, low], axis=0)))):
                    he[i, pl.ds(pl.multiple_of(t * 32, 32), 32), :] = v
                return carry
            lax.fori_loop(0, NSEG * E // 64, early_operands, 0)

        rest = ([functools.partial(mod_copy, j) for j in range(2 * ND, 5 * ND)]
                + [functools.partial(wo_copy, j) for j in range(4 * ND)])
        extra = []
        for k, n in enumerate(EXTRA):
            extra.append(rest[:n] + ([functools.partial(x_copy, k)] if 1 <= k <= 3 else []))
            rest = rest[n:]
        assert not rest and len(extra) == HP

        def look_ahead(hp, pin, span, last, tokens):
            @pl.when(hp + PREFETCH < HP)
            def _():
                for cp in w_copies(hp + PREFETCH):
                    cp.start()

            for k in span:
                @pl.when(hp == k)
                def _():
                    for cp in extra[k]:
                        cp().start()
            for cp in w_copies(hp, (1, 2)) + ([] if last else w_copies(hp + 1, (0,))):
                cp.wait()
            n = LA_ROWS // E
            done = []
            for m in range(3):
                p = 6 * hp + m
                todo = list(range(NPIECE)) if m < 2 or not last else []
                for u in range(NU):
                    prods = []
                    for i in range(7):
                        if todo and len(done) >= LA_LAG and i % 3 != 2:
                            y = pltpu.bitcast(done[-LA_LAG][:D // 4 // NPIECE], U32)
                            repack(hp + (m + 1) // 3, (m + 1) % 3, todo.pop(0),
                                   lambda v: jnp.where(pin == 0, v, y))
                        w = jnp.concatenate([we_u[m + pin, i, pl.ds(0, 8), :],
                                             we_u[m, i, pl.ds(8, D // 4 - 8), :]], axis=0)
                        prods.append(
                            _dot(he[i, pl.ds(u * LA_ROWS, LA_ROWS), :], pltpu.bitcast(w, BF16)))
                        done.append(prods[-1])
                    c = _strassen_out(prods)
                    for v, s0, q in zip(c, (0, 0, NSEG // 2, NSEG // 2), (p, p + 3, p, p + 3)):
                        seg[pl.ds(1 + s0 + u * n, n), q] = v.reshape(n, E, LANES)
                    if tokens is not None and m < 2:
                        for s in tokens(m * NU + u):
                            seg_put(1 + s + pin, TOK,
                                    modulate_a(_ln(xs[s].astype(F32))).astype(BF16))
                assert not todo
            return pin

        with jax.named_scope("look_ahead"):
            per = NSEG // HP // NU

            def tokens_of(hp):
                return lambda i: [((hp - HP // 2) * 2 * NU + i) * per + u for u in range(per)]
            lax.fori_loop(0, HP // 2, lambda hp, c: look_ahead(
                hp, _pin(hp), range(HP // 2), False, None), 0)
            for i in range(1, R):
                x_copy(i).wait()
        with jax.named_scope("look_ahead2"):
            pin = lax.fori_loop(
                HP // 2, HP - 1, lambda hp, c: look_ahead(
                    hp, _pin(hp), range(HP // 2, HP - 1), False, tokens_of(hp)), 0)
            look_ahead(HP - 1, pin, [HP - 1], True, tokens_of(HP - 1))

        with jax.named_scope("mod_b"):
            mod_chunks(2, 5)
            for j in range(4 * ND):
                wo_copy(j).wait()
            for j in range(5 * ND, 6 * ND):
                mod_copy(j).start()
            for cp in b_copies[:len(b_copies) // 2]:
                cp.start()

        def set_lhs(mem, s, j):
            tok = seg[1 + s, pl.ds(TOK + j * R // 2, R // 2)].reshape(SEG // 2, LANES)
            tok = pltpu.bitcast(tok, BF16)
            head = jnp.concatenate([mem, tok[:16].astype(F32)[E:]], axis=0).astype(BF16)
            lhs[j] = pltpu.bitcast(jnp.concatenate([head, tok[16:]], axis=0), U32)

        def finish_tokens(s, row):
            x1 = xs[s].astype(F32) + rows(mod[2], SEG) * aout[...]
            h = _ln(x1) * rows(1.0 + mod[4], SEG) + rows(mod[3], SEG)
            seg_put(row, X1, x1)
            seg_put(row, HB, h)
            seg_put(row, HN, _ln(h))

        def weight_sums(u):
            n = wm.shape[1] // (NSEG - PLAIN_STEPS) // (H // HEAD_GROUP)
            at = pl.ds(pl.multiple_of(u * n, n), n)
            for i, v in enumerate(_strassen_rhs(*(wm[i, at, :] for i in (B11, B12, B21, B22)))):
                if i not in (B11, B22):
                    wm[i, at, :] = v

        for j in range(ND):
            set_lhs(mem0_ref[:, lanes(j)].astype(F32), 0, j)
        aout[...] = jnp.zeros_like(aout)

        def step(s, sums):
            ri = lax.broadcasted_iota(jnp.int32, (L, LP), 0)
            ci = lax.broadcasted_iota(jnp.int32, (L, LP), 1)
            keep = ((ri < M) | (ri >= ci)) & (ci < L)
            fill = jnp.where(ci < L, -1e9, -jnp.inf).astype(F32)
            zpad = jnp.zeros((LP - L, LANES), F32)

            def project(h, m):
                p = 3 * h + m
                if h < KSPLIT and m == 0:
                    y = acc[pl.ds(0, SEG), lanes(h)] + _dot(
                        _panels(lhs, 0, ND // 2), _panel(wqkv, p, 0, D // 4))
                else:
                    y = _dot(_panels(lhs, 0, ND), _panel(wqkv, p))
                parts = [y[:M], seg[1 + s, p], y[M:]]
                if m == 0:
                    return jnp.concatenate(parts, axis=0)
                return jnp.concatenate(parts + [zpad], axis=0).astype(BF16)

            def probs(q, k):
                sc = jnp.where(keep, _dot_nt(q, k) * scale, fill)
                e = jnp.exp(sc - jnp.max(sc, axis=-1, keepdims=True))
                return e / jnp.sum(e, axis=-1, keepdims=True)

            G = HEAD_GROUP
            NG = H // G
            KH = (H - G) * LANES

            for h in range(KSPLIT):
                acc[pl.ds(0, SEG), lanes(h)] = _dot(
                    _panels(lhs, ND // 2, ND // 2), _panel(wqkv, 3 * h, D // 4, D // 4))
            prev = None
            for g in range(NG + 1):
                if g == FINISH_AT:
                    finish_tokens(jnp.maximum(s - 1, 0), s + _pin(s) * PIN_FINISH)
                if g < NG and sums and SUMS_IN_STEPS:
                    weight_sums((s - PLAIN_STEPS) * NG + g)
                heads = range(g * G, (g + 1) * G) if g < NG else ()
                q = [project(h, 0) for h in heads]
                if prev is not None:
                    pr = [probs(a, b) for a, b in zip(prev[0], prev[1])]
                k = [project(h, 1) for h in heads]
                v = [project(h, 2) for h in heads]
                if g == NG:
                    for j in range(WO_SPLIT):
                        acc[:, lanes(j)] = _dot(obuf[:, pl.ds(0, KH)], _panel(wo, j, 0, KH // 2))
                if prev is not None:
                    for u in range(G):
                        obuf[:, lanes((g - 1) * G + u)] = _dot(pr[u], prev[2][u])
                prev = (q, k, v)
            for j in reversed(range(ND)):
                if j < WO_SPLIT:
                    y = acc[:, lanes(j)] + _dot(
                        obuf[:, lanes(H - G, G)], _panel(wo, j, KH // 2, G * LANES // 2))
                else:
                    y = _dot(obuf[...], _panel(wo, j))
                set_lhs(y[:M], jnp.minimum(s + 1, NSEG - 1), j)
                aout[:, lanes(j)] = y[M:]

        def steps(i, sums):
            if not sums:
                @pl.when(i == PLAIN_STEPS // UNROLL // 2)
                def _():
                    for cp in b_copies[len(b_copies) // 2:]:
                        cp.start()
            for u in range(UNROLL):
                step(i * UNROLL + u, sums)

        with jax.named_scope("steps"):
            lax.fori_loop(0, PLAIN_STEPS // UNROLL, lambda i, c: steps(i, False), None)
        with jax.named_scope("steps2"):
            mod_chunks(5, 6)
            for cp in b_copies:
                cp.wait()
            lax.fori_loop(PLAIN_STEPS // UNROLL, NSEG // UNROLL, lambda i, c: steps(i, True), None)
        finish_tokens(NSEG - 1, NSEG)
        if not SUMS_IN_STEPS:
            with jax.named_scope("sums"):
                lax.fori_loop(0, (NSEG - PLAIN_STEPS) * (H // HEAD_GROUP), lambda u, c: weight_sums(u), None, unroll=8)

    pl.run_scoped(
        attention_phase,
        pltpu.VMEM((3 * H, D // 2, LANES), U32),
        pltpu.VMEM((ND, H * LANES // 2, LANES), U32),
        pltpu.VMEM((NSEG, SEG, D), BF16),
        pltpu.VMEM((NSEG * E, D), F32),
        pltpu.VMEM((7, NSEG * E // 2, D // 2), F32),
        pltpu.VMEM((3, 7, D // 2, LANES), BF16),
        pltpu.VMEM((ND, SEG // 2, LANES), U32),
        pltpu.VMEM((L, H * LANES), F32),
        pltpu.VMEM((SEG, D), F32),
        pltpu.VMEM((L, D), F32),
        pltpu.SemaphoreType.DMA((3 * H // 2,)),
        pltpu.SemaphoreType.DMA((R,)),
        pltpu.SemaphoreType.DMA((1,)),
    )

    def mixer_phase(gbuf, obuf, ops, sem_out):
        NT = S // TM
        TS = TM // SEG
        TH = TM // 2
        KS = (D // 2, D // 2, D // 2, F // 2)
        gbuf[pl.ds(0, 8), :] = jnp.zeros((8, D), F32)
        gbuf[pl.ds(S + 8, 8), :] = jnp.zeros((8, D), F32)

        def put_lhs(w, piece):
            def task(r, after=lambda v: v):
                v = after(jnp.concatenate([piece(r), piece(TH + r)], axis=0))
                if w == 2:
                    v = _ln(v)
                for i, a in enumerate(_strassen_lhs(*_quarters(v))):
                    ops[i, pl.ds(r, 8), pl.ds(w * D // 2, D // 2)] = a
            return [functools.partial(task, r) for r in range(0, TH, 8)]

        def run(tasks):
            for task in tasks:
                task()

        def product(w, j, pin=0, tasks=(), done=None):
            nh = (NF if w == 2 else ND) // 2
            prods = []
            for i in range(7):
                if tasks and len(done) >= TASK_LAG:
                    m = jnp.concatenate([done[-TASK_LAG][:16]] * ND, axis=1)
                    tasks.pop(0)(lambda v: jnp.where(pin == 0, v, m))
                a = jnp.concatenate([ops[i + pin, :, pl.ds(w * D // 2, LANES)],
                                     ops[i, :, pl.ds(w * D // 2 + LANES, KS[w] - LANES)]], axis=1)
                prods.append(_dot(a, _panel(wm_u, i, (WM_AT[w] + j * KS[w]) // 2, KS[w] // 2)))
                if done is not None:
                    done.append(prods[-1])
            return zip((0, 0, TH, TH), (j, j + nh, j, j + nh), _strassen_out(prods))

        def seg_rows(t, slot, r):
            return jnp.concatenate(
                [seg[1 + t * TS + r // SEG, slot + j * R + r % SEG // 8] for j in range(ND)], axis=1)

        def block(t, r0, slot, n):
            return 1 + t * TS + r0 // SEG, slot + n * R

        def gate_in(t):
            return put_lhs(0, lambda r: seg_rows(t, HN, r))

        def gate(t):
            for j in range(ND // 2):
                for r0, n, v in product(0, j):
                    gbuf[pl.ds(pl.multiple_of(t * TM + 8 + r0, 8), TH), lanes(n)] = (
                        jax.nn.gelu(v, approximate=True))

        def mix_in(t):
            C = D // 4

            def shifted(r):
                return jnp.concatenate([
                    gbuf[pl.ds(pl.multiple_of(t * TM + r + (8 if by > 0 else 0), 8), 16),
                         pl.ds(i * C, C)][by % 8:by % 8 + 8]
                    for i, by in enumerate((-1, 1, -2, 2))], axis=1)
            return put_lhs(1, shifted)

        def mix(t):
            for j in range(ND // 2):
                for r0, n, v in product(1, j):
                    row, slot = block(t, r0, HB, n)
                    seg_put(row, slot, seg_get(row, TS // 2, slot, 1) + v, TS // 2)

        def up_in(t):
            return put_lhs(2, lambda r: seg_rows(t, HB, r))

        def up():
            for j in range(NF // 2):
                g = [jax.nn.gelu(v, approximate=True) for _, _, v in product(2, j)]
                for i, a in enumerate(_strassen_lhs(*g)):
                    ops[i, :, lanes(3 * ND // 2 + j)] = a

        def down(t, j, pin, tasks, done):
            for r0, n, v in product(3, j, pin, tasks, done):
                row, slot = block(t, r0, HB, n)
                y = seg_get(row, TS // 2, slot, 1) + v
                row, slot = block(t, r0, X1, n)
                y = seg_get(row, TS // 2, slot, 1) + rows(mod[5, :, lanes(n)], TH) * y
                obuf[pl.ds(pl.multiple_of(t * TM + r0, TH), TH), lanes(n)] = y.astype(BF16)

        def out_copy(t):
            r = pl.multiple_of(t * TM, TM)
            return pltpu.make_async_copy(obuf.at[pl.ds(r, TM)], out_hbm.at[pl.ds(r, TM)], sem_out.at[0])

        def tile(t, pin, ahead):
            up()
            if ahead >= 1:
                mix(t + 1)
            if ahead >= 3:
                gate(t + 3)
            tasks, done = [], []
            if ahead >= 3:
                tasks += gate_in(jnp.minimum(t + 4, NT - 1))
            if ahead >= 1:
                tasks += up_in(t + 1)
            if ahead >= 2:
                tasks += mix_in(t + 2)
            for j in range(ND // 2):
                down(t, j, pin, tasks, done)
            run(tasks)
            out_copy(t).start()
            return pin

        with jax.named_scope("gate"):
            run(gate_in(0))
            gate(0)
            run(gate_in(1))
            gate(1)
            run(mix_in(0))
            mix(0)
            run(gate_in(2))
            gate(2)
            run(up_in(0))
            run(mix_in(1))
            run(gate_in(3))
        with jax.named_scope("mlp"):
            pin = lax.fori_loop(0, NT - 3, lambda t, c: tile(t, _pin(t), 3), 0)
        with jax.named_scope("mlp2"):
            for t in range(NT - 3, NT):
                tile(t, pin, NT - 1 - t)
        for t in range(NT):
            out_copy(t).wait()

    pl.run_scoped(
        mixer_phase,
        pltpu.VMEM((S + 16, D), F32),
        pltpu.VMEM((S, D), BF16),
        pltpu.VMEM((7, TM // 2, 3 * D // 2 + F // 2), F32),
        pltpu.SemaphoreType.DMA((1,)))


@functools.partial(jax.jit, static_argnames=("A_seg_len",))
def pallas_adaLN_cond__memory_aug_recurrent_mem_tr__mixer_s_mlp__prompt_kernel(
    A_x, A_mem0, A_Wq, A_Wk, A_Wv, A_Wo, A_seg_len, B_x, B_w1, B_w2, B_w3, B_w4, c, w_mod,
):
    del B_x
    B, S, D = A_x.shape
    H, Dh = A_Wq.shape[1:]
    M = A_mem0.shape[1]
    F = B_w3.shape[1]
    SEG = A_seg_len
    assert B == 1 and Dh == LANES and M == 8 and SEG % 16 == 0 and S % SEG == 0
    ND, NF = D // LANES, F // LANES
    hbm = pl.BlockSpec(memory_space=pl.ANY)
    vmem = pl.BlockSpec(memory_space=pltpu.VMEM)
    out = pl.pallas_call(
        functools.partial(_kernel, S=S, D=D, H=H, M=M, SEG=SEG, F=F),
        out_shape=jax.ShapeDtypeStruct((S, D), A_x.dtype),
        in_specs=[hbm, vmem, hbm, hbm, hbm, hbm, hbm, hbm, hbm, hbm, vmem, hbm],
        out_specs=hbm,
        scratch_shapes=[
            pltpu.VMEM((7, (ND + NF) * D // 2, LANES), BF16),
            pltpu.VMEM((S // SEG + 1, 3 * H + ND * SEG // 16, 8, LANES), F32),
            pltpu.VMEM((6, 8, D), F32),
            pltpu.SemaphoreType.DMA((6,)),
            pltpu.SemaphoreType.DMA((1,)),
        ],
        compiler_params=pltpu.CompilerParams(vmem_limit_bytes=124 * 1024 * 1024),
    )(A_x.reshape(S // SEG, SEG, D), A_mem0.reshape(M, D),
      *(w.reshape(D // 2, 2, H, Dh) for w in (A_Wq, A_Wk, A_Wv)),
      A_Wo.reshape(H * Dh, D), B_w1, B_w2, B_w3, B_w4, c, w_mod)
    return out.reshape(B, S, D)
```

```python
import functools

import jax
import jax.numpy as jnp
import numpy as np
from jax import lax
import jax.experimental.pallas as pl
import jax.experimental.pallas.tpu as pltpu

F32 = jnp.float32
BF16 = jnp.bfloat16
U32 = jnp.uint32
LANES = 128
EPS = 1e-5

HEAD_GROUP = 4
UNROLL = 2
KSPLIT = 4
WO_SPLIT = 4
FINISH_AT = 2
PAIRS = 1
PREFETCH = 3
MOD_FIRST = 2
TM = 128
GATE_AHEAD = True
DOWN_SPLIT = 1
TASK_LAG = 2


def _ln(x):
    m = jnp.mean(x, axis=-1, keepdims=True)
    d = x - m
    v = jnp.mean(d * d, axis=-1, keepdims=True)
    return d * lax.rsqrt(v + EPS)


def _dot(a, b):
    return jnp.dot(a, b, preferred_element_type=F32)


def _dot_nt(a, b):
    return lax.dot_general(a, b, (((1,), (1,)), ((), ())), preferred_element_type=F32)


def _panel(ref, p, r0=None, nr=None):
    w = ref[p] if r0 is None else ref[p, pl.ds(r0, nr), :]
    return pltpu.bitcast(w, BF16)


def _panels(ref, p0, n):
    return jnp.concatenate([_panel(ref, p0 + j) for j in range(n)], axis=1)


def _pin(i):
    return i >> 24


def _lanes(j, n=1):
    return pl.ds(j * LANES, n * LANES)


def _rows(v, n):
    return jnp.concatenate([v] * (n // 8), axis=0)


def _kernel(x_hbm, mem0_ref, wq_hbm, wk_hbm, wv_hbm, wo_hbm, w1_hbm, w2_hbm, w3_hbm, w4_hbm,
            c_ref, wmod_hbm, out_hbm,
            wb, w4, seg, mod, sem_mod, sem_b,
            *, S, D, H, M, SEG, F):
    NSEG = S // SEG
    E = M
    L = M + SEG
    LP = -(-L // 16) * 16
    ND = D // LANES
    NF = F // LANES
    R = SEG // 8
    scale = LANES ** -0.5
    TOK = 3 * H
    X1, HB, HN = 0, R * ND, 2 * R * ND

    def seg_put(row, slot, v, n=1):
        if v.dtype != F32:
            v = pltpu.bitcast(v, F32)
        r = v.shape[0] // (8 * n)
        for j in range(v.shape[1] // LANES):
            seg[pl.ds(row, n), pl.ds(slot + j * r, r)] = (
                v[:, j * LANES:(j + 1) * LANES].reshape(n, r, 8, LANES))

    def seg_get(row, n, slot, cols, r=R):
        return jnp.concatenate(
            [seg[pl.ds(row, n), pl.ds(slot + j * r, r)].reshape(n * r * 8, LANES)
             for j in range(cols)], axis=1)

    w_u = [r.bitcast(U32) for r in (wq_hbm, wk_hbm, wv_hbm)]
    wo_u, w1_u, w2_u, w3_u, w4_u, wmod_u = (
        r.bitcast(U32) for r in (wo_hbm, w1_hbm, w2_hbm, w3_hbm, w4_hbm, wmod_hbm))

    b_copies = [
        pltpu.make_async_copy(w.at[:, _lanes(j)], dst.at[p0 + j], sem_b)
        for w, dst, p0 in ((w1_u, wb, 0), (w2_u, wb, ND), (w3_u, wb, 2 * ND), (w4_u, w4, 0))
        for j in range(w.shape[1] // LANES)]

    def mod_copy(j):
        return pltpu.make_async_copy(wmod_u.at[:, _lanes(j)], wb.at[j], sem_mod.at[j // ND])

    def mod_chunks(lo, hi, arrived=()):
        cv = c_ref[...].astype(F32)
        sc = jnp.broadcast_to(cv * jax.nn.sigmoid(cv), (8, D))
        for j in range(lo * ND, hi * ND):
            mod_copy(j).wait()
        for cp in arrived:
            cp.start()
        for j in range(lo * ND, hi * ND):
            mod[j // ND, :, _lanes(j % ND)] = _dot(sc, _panel(wb, j))

    def attention_phase(wqkv, wo, xs, xn, he, lhs, obuf, aout, acc, sem_w, sem_x, sem_wo):
        HP = H // 2
        NI = HP // PAIRS

        def w_copies(hp):
            return [pltpu.make_async_copy(w_u[m].at[:, i, hp, :], wqkv.at[6 * hp + 3 * i + m],
                                          sem_w.at[hp]) for m in range(3) for i in range(2)]

        def wo_copy(j):
            return pltpu.make_async_copy(wo_u.at[:, _lanes(j)], wo.at[j], sem_wo)

        def x_copy(i):
            sl = pl.ds(i * E, E)
            return pltpu.make_async_copy(x_hbm.at[:, sl, :], xs.at[:, sl, :], sem_x.at[min(i, 1)])

        def modulate_a(n):
            return n * _rows(1.0 + mod[1], n.shape[0]) + _rows(mod[0], n.shape[0])

        x_copy(0).start()
        for j in range(MOD_FIRST):
            mod_copy(j).start()

        with jax.named_scope("early_ln"):
            x_copy(0).wait()
            for j in range(MOD_FIRST, 2 * ND):
                mod_copy(j).start()

            def early_norm(t, carry):
                xv = xs[pl.ds(t * 16, 16), pl.ds(0, E), :].astype(F32).reshape(16 * E, D)
                xn[pl.ds(pl.multiple_of(t * 16 * E, 16 * E), 16 * E), :] = _ln(xv)
            lax.fori_loop(0, NSEG // 16, early_norm, None)

        with jax.named_scope("mod_a"):
            mod_chunks(0, 2, w_copies(0))
            hv = modulate_a(xn[...]).astype(BF16)
            for j in range(ND):
                he[j] = hv[:, j * LANES:(j + 1) * LANES]
            for hp in range(1, PREFETCH):
                for cp in w_copies(hp):
                    cp.start()

        extra = ([[functools.partial(x_copy, i)] for i in range(1, R)]
                 + [[functools.partial(mod_copy, j + u) for u in range(4)]
                    for j in range(2 * ND, 6 * ND, 4)]
                 + [[functools.partial(wo_copy, j + u) for u in range(2)] for j in range(0, ND, 2)])

        def look_ahead(i, span, tokens):
            for v in range(PAIRS):
                @pl.when(i * PAIRS + v + PREFETCH < HP)
                def _():
                    for cp in w_copies(i * PAIRS + v + PREFETCH):
                        cp.start()
            for k in span:
                @pl.when(i == k)
                def _():
                    for cp in sum(extra[k * PAIRS:(k + 1) * PAIRS], []):
                        cp().start()
            for v in range(PAIRS):
                for cp in w_copies(i * PAIRS + v):
                    cp.wait()
            for v in range(PAIRS):
                hp = i * PAIRS + v
                for m in range(3):
                    p = 6 * hp + m
                    a, b = wqkv[p], wqkv[p + 3]
                    w = ((a & np.uint32(0xFFFF)) | (b << 16),
                         (a >> 16) | (b & np.uint32(0xFFFF0000)))
                    for u in range(2):
                        wqkv[p + 3 * u] = w[u]
                        y = _dot(_panels(he.bitcast(U32), 0, ND), pltpu.bitcast(w[u], BF16))
                        seg[pl.ds(1, NSEG), p + 3 * u] = y.reshape(NSEG, E, LANES)
                        if tokens and m < 2:
                            n = NSEG // (HP // 2) // 4
                            for k in range(n):
                                s = ((hp - HP // 2) * 4 + 2 * m + u) * n + k
                                seg_put(1 + s, TOK, modulate_a(_ln(xs[s].astype(F32))).astype(BF16))

        with jax.named_scope("look_ahead"):
            lax.fori_loop(0, NI // 2, lambda i, c: look_ahead(i, range(NI // 2), False), None)
            for i in range(1, R):
                x_copy(i).wait()
        with jax.named_scope("look_ahead2"):
            lax.fori_loop(NI // 2, NI, lambda i, c: look_ahead(i, range(NI // 2, NI), True), None)

        with jax.named_scope("mod_b"):
            mod_chunks(2, 6)
            for j in range(ND):
                wo_copy(j).wait()
            for cp in b_copies:
                cp.start()

        def set_lhs(mem, s, j):
            tok = pltpu.bitcast(seg_get(1 + s, 1, TOK + j * R // 2, 1, R // 2), BF16)
            head = jnp.concatenate([mem, tok[:16].astype(F32)[E:]], axis=0).astype(BF16)
            lhs[j] = jnp.concatenate([head, tok[16:]], axis=0)

        def finish_tokens(s, row):
            x1 = xs[s].astype(F32) + _rows(mod[2], SEG) * aout[...]
            h = _ln(x1) * _rows(1.0 + mod[4], SEG) + _rows(mod[3], SEG)
            seg_put(row, X1, x1)
            seg_put(row, HB, h)
            seg_put(row, HN, _ln(h).astype(BF16))

        for j in range(ND):
            set_lhs(mem0_ref[:, _lanes(j)].astype(F32), 0, j)
        aout[...] = jnp.zeros_like(aout)
        lhs_u = lhs.bitcast(U32)

        def step(s):
            ri = lax.broadcasted_iota(jnp.int32, (L, LP), 0)
            ci = lax.broadcasted_iota(jnp.int32, (L, LP), 1)
            keep = ((ri < M) | (ri >= ci)) & (ci < L)
            fill = jnp.where(ci < L, -1e9, -jnp.inf).astype(F32)
            zpad = jnp.zeros((LP - L, LANES), F32)

            def project(h, m):
                p = 3 * h + m
                if h < KSPLIT and m == 0:
                    y = acc[pl.ds(0, SEG), _lanes(h)] + _dot(
                        _panels(lhs_u, 0, ND // 2), _panel(wqkv, p, 0, D // 4))
                else:
                    y = _dot(_panels(lhs_u, 0, ND), _panel(wqkv, p))
                parts = [y[:M], seg[1 + s, p], y[M:]]
                if m == 0:
                    return jnp.concatenate(parts, axis=0)
                return jnp.concatenate(parts + [zpad], axis=0).astype(BF16)

            def probs(q, k):
                sc = jnp.where(keep, _dot_nt(q, k) * scale, fill)
                e = jnp.exp(sc - jnp.max(sc, axis=-1, keepdims=True))
                return e / jnp.sum(e, axis=-1, keepdims=True)

            G = HEAD_GROUP
            NG = H // G
            KH = (H - G) * LANES

            for h in range(KSPLIT):
                acc[pl.ds(0, SEG), _lanes(h)] = _dot(
                    _panels(lhs_u, ND // 2, ND // 2), _panel(wqkv, 3 * h, D // 4, D // 4))
            prev = None
            for g in range(NG + 1):
                if g == FINISH_AT:
                    finish_tokens(jnp.maximum(s - 1, 0), s)
                heads = range(g * G, (g + 1) * G) if g < NG else ()
                q = [project(h, 0) for h in heads]
                if prev is not None:
                    pr = [probs(a, b) for a, b in zip(prev[0], prev[1])]
                k = [project(h, 1) for h in heads]
                v = [project(h, 2) for h in heads]
                if g == NG:
                    for j in range(WO_SPLIT):
                        acc[:, _lanes(j)] = _dot(obuf[:, pl.ds(0, KH)], _panel(wo, j, 0, KH // 2))
                if prev is not None:
                    for u in range(G):
                        obuf[:, _lanes((g - 1) * G + u)] = _dot(pr[u], prev[2][u])
                prev = (q, k, v)
            for j in reversed(range(ND)):
                if j < WO_SPLIT:
                    y = acc[:, _lanes(j)] + _dot(
                        obuf[:, _lanes(H - G, G)], _panel(wo, j, KH // 2, G * LANES // 2))
                else:
                    y = _dot(obuf[...], _panel(wo, j))
                set_lhs(y[:M], jnp.minimum(s + 1, NSEG - 1), j)
                aout[:, _lanes(j)] = y[M:]

        def steps(i, carry):
            for u in range(UNROLL):
                step(i * UNROLL + u)

        with jax.named_scope("steps"):
            lax.fori_loop(0, NSEG // UNROLL, steps, None)
            for s in range(NSEG // UNROLL * UNROLL, NSEG):
                step(s)
        finish_tokens(NSEG - 1, NSEG)

    pl.run_scoped(
        attention_phase,
        pltpu.VMEM((3 * H, D // 2, LANES), U32),
        pltpu.VMEM((ND, H * LANES // 2, LANES), U32),
        pltpu.VMEM((NSEG, SEG, D), BF16),
        pltpu.VMEM((NSEG * E, D), F32),
        pltpu.VMEM((ND, NSEG * E, LANES), BF16),
        pltpu.VMEM((ND, SEG, LANES), BF16),
        pltpu.VMEM((L, H * LANES), F32),
        pltpu.VMEM((SEG, D), F32),
        pltpu.VMEM((L, D), F32),
        pltpu.SemaphoreType.DMA((H // 2,)),
        pltpu.SemaphoreType.DMA((2,)),
        pltpu.SemaphoreType.DMA(()),
    )

    def mixer_phase(gbuf, obuf, ops, sem_out):
        NT = S // TM
        TS = TM // SEG
        ops_u = ops.bitcast(U32)
        for cp in b_copies:
            cp.wait()
        gbuf[pl.ds(0, 8), :] = jnp.zeros((8, D), F32)
        gbuf[pl.ds(S + 8, 8), :] = jnp.zeros((8, D), F32)

        def operand_tasks(p0, rows_of, norm):
            def task(u, after=lambda v: v):
                v = norm(after(rows_of(u))).astype(BF16)
                for j in range(ND):
                    ops[p0 + j, pl.ds(u * SEG, SEG), :] = v[:, j * LANES:(j + 1) * LANES]
            return [functools.partial(task, u) for u in range(TS)]

        def gate(t):
            for j in range(ND):
                a = pltpu.bitcast(seg_get(1 + t * TS, TS, HN, ND, R // 2), BF16)
                gbuf[pl.ds(pl.multiple_of(t * TM + 8, 8), TM), _lanes(j)] = jax.nn.gelu(
                    _dot(a, _panel(wb, j)), approximate=True)

        def mix_in(t):
            def shifted(u):
                return jnp.concatenate([
                    gbuf[pl.ds(pl.multiple_of(t * TM + u * SEG + (8 if by > 0 else 0), 8), SEG + 8),
                         pl.ds(i * D // 4, D // 4)][by % 8:by % 8 + SEG]
                    for i, by in enumerate((-1, 1, -2, 2))], axis=1)
            return operand_tasks(0, shifted, lambda v: v)

        def mix(t):
            for j in range(ND):
                y = seg_get(1 + t * TS, TS, HB + j * R, 1) + _dot(
                    _panels(ops_u, 0, ND), _panel(wb, ND + j))
                seg_put(1 + t * TS, HB + j * R, y, TS)

        def up_in(t):
            return operand_tasks(ND, lambda u: seg_get(1 + t * TS + u, 1, HB, ND), _ln)

        def up():
            for j in range(NF):
                ops[2 * ND + j] = jax.nn.gelu(
                    _dot(_panels(ops_u, ND, ND), _panel(wb, 2 * ND + j)),
                    approximate=True).astype(BF16)

        def down(t, pin, tasks):
            done = []
            nk = NF // DOWN_SPLIT
            per = -(-len(tasks) // (ND * DOWN_SPLIT - TASK_LAG))
            for j in range(ND):
                y = seg_get(1 + t * TS, TS, HB + j * R, 1)
                for k in range(0, NF, nk):
                    if len(done) >= TASK_LAG:
                        m = jnp.concatenate([done[-TASK_LAG][:SEG]] * ND, axis=1)
                        for task in tasks[:per]:
                            task(lambda v: jnp.where(pin == 0, v, m))
                        tasks = tasks[per:]
                    a = jnp.concatenate([_panel(ops_u, 2 * ND + k + pin),
                                         _panels(ops_u, 2 * ND + k + 1, nk - 1)], axis=1)
                    y = y + _dot(a, _panel(w4, j, k * LANES // 2, nk * LANES // 2))
                    done.append(y)
                y = seg_get(1 + t * TS, TS, X1 + j * R, 1) + _rows(mod[5, :, _lanes(j)], TM) * y
                obuf[pl.ds(pl.multiple_of(t * TM, TM), TM), _lanes(j)] = y.astype(BF16)

        def out_copy(t):
            r = pl.ds(pl.multiple_of(t * TM, TM), TM)
            return pltpu.make_async_copy(obuf.at[r], out_hbm.at[r], sem_out)

        def tile(t, pin, ahead):
            up()
            if ahead >= 1:
                mix(t + 1)
            if ahead >= 3 and GATE_AHEAD:
                gate(t + 3)
            down(t, pin, (up_in(t + 1) if ahead >= 1 else []) + (mix_in(t + 2) if ahead >= 2 else []))
            out_copy(t).start()
            return pin

        with jax.named_scope("gate"):
            if GATE_AHEAD:
                gate(0)
                gate(1)
            else:
                lax.fori_loop(0, NT, lambda t, c: gate(t), None, unroll=2)
            for task in mix_in(0):
                task()
            mix(0)
            if GATE_AHEAD:
                gate(2)
            for task in up_in(0) + mix_in(1):
                task()
        last = 3 if GATE_AHEAD else 2
        with jax.named_scope("mlp"):
            pin = lax.fori_loop(0, NT - last, lambda t, c: tile(t, _pin(t), 3), 0)
        with jax.named_scope("mlp2"):
            for t in range(NT - last, NT):
                tile(t, pin, NT - 1 - t)
        for t in range(NT):
            out_copy(t).wait()

    pl.run_scoped(
        mixer_phase,
        pltpu.VMEM((S + 16, D), F32),
        pltpu.VMEM((S, D), BF16),
        pltpu.VMEM((2 * ND + NF, TM, LANES), BF16),
        pltpu.SemaphoreType.DMA(()))


@functools.partial(jax.jit, static_argnames=("A_seg_len",))
def pallas_adaLN_cond__memory_aug_recurrent_mem_tr__mixer_s_mlp__prompt_kernel(
    A_x, A_mem0, A_Wq, A_Wk, A_Wv, A_Wo, A_seg_len, B_x, B_w1, B_w2, B_w3, B_w4, c, w_mod,
):
    del B_x
    B, S, D = A_x.shape
    H, Dh = A_Wq.shape[1:]
    M = A_mem0.shape[1]
    F = B_w3.shape[1]
    SEG = A_seg_len
    assert B == 1 and Dh == LANES and M == 8 and SEG % 16 == 0 and S % SEG == 0
    ND, NF = D // LANES, F // LANES
    hbm = pl.BlockSpec(memory_space=pl.ANY)
    vmem = pl.BlockSpec(memory_space=pltpu.VMEM)
    out = pl.pallas_call(
        functools.partial(_kernel, S=S, D=D, H=H, M=M, SEG=SEG, F=F),
        out_shape=jax.ShapeDtypeStruct((S, D), A_x.dtype),
        in_specs=[hbm, vmem, hbm, hbm, hbm, hbm, hbm, hbm, hbm, hbm, vmem, hbm],
        out_specs=hbm,
        scratch_shapes=[
            pltpu.VMEM((max(6 * ND, 2 * ND + NF), D // 2, LANES), U32),
            pltpu.VMEM((ND, F // 2, LANES), U32),
            pltpu.VMEM((S // SEG + 1, 3 * H + ND * SEG // 16, 8, LANES), F32),
            pltpu.VMEM((6, 8, D), F32),
            pltpu.SemaphoreType.DMA((6,)),
            pltpu.SemaphoreType.DMA(()),
        ],
        compiler_params=pltpu.CompilerParams(vmem_limit_bytes=110 * 1024 * 1024),
    )(A_x.reshape(S // SEG, SEG, D), A_mem0.reshape(M, D),
      *(w.reshape(D // 2, 2, H, Dh) for w in (A_Wq, A_Wk, A_Wv)),
      A_Wo.reshape(H * Dh, D), B_w1, B_w2, B_w3, B_w4, c, w_mod)
    return out.reshape(B, S, D)
```

```python
import functools

import jax
import jax.numpy as jnp
import numpy as np
from jax import lax
import jax.experimental.pallas as pl
import jax.experimental.pallas.tpu as pltpu

F32 = jnp.float32
BF16 = jnp.bfloat16
U32 = jnp.uint32
LANES = 128
EPS = 1e-5

HEAD_GROUP = 4
UNROLL = 2
KSPLIT = 4
WO_SPLIT = 4
FINISH_AT = 2
PAIRS = 1
PREFETCH = 4
MOD_FIRST = 4
TM = 128
GATE_AHEAD = True
TOK_FROM = 8
TOK_LATE = True
PAIRS2 = 2
W_FIRST = 4
DOWN_SPLIT = 1
TASK_LAG = 2


def _ln(x):
    m = jnp.mean(x, axis=-1, keepdims=True)
    d = x - m
    v = jnp.mean(d * d, axis=-1, keepdims=True)
    return d * lax.rsqrt(v + EPS)


def _dot(a, b):
    return jnp.dot(a, b, preferred_element_type=F32)


def _dot_nt(a, b):
    return lax.dot_general(a, b, (((1,), (1,)), ((), ())), preferred_element_type=F32)


def _panel(ref, p, r0=None, nr=None):
    w = ref[p] if r0 is None else ref[p, pl.ds(r0, nr), :]
    return pltpu.bitcast(w, BF16)


def _panels(ref, p0, n):
    return jnp.concatenate([_panel(ref, p0 + j) for j in range(n)], axis=1)


def _pin(i):
    return i >> 24


def _lanes(j, n=1):
    return pl.ds(j * LANES, n * LANES)


def _rows(v, n):
    return jnp.concatenate([v] * (n // 8), axis=0)


def _kernel(x_hbm, mem0_ref, wq_hbm, wk_hbm, wv_hbm, wo_hbm, w1_hbm, w2_hbm, w3_hbm, w4_hbm,
            c_ref, wmod_hbm, out_hbm,
            wb, w4, seg, mod, sem_mod, sem_b,
            *, S, D, H, M, SEG, F):
    NSEG = S // SEG
    E = M
    L = M + SEG
    LP = -(-L // 16) * 16
    ND = D // LANES
    NF = F // LANES
    R = SEG // 8
    scale = LANES ** -0.5
    TOK = 3 * H
    X1, HB, HN = 0, R * ND, 2 * R * ND

    def seg_put(row, slot, v, n=1):
        if v.dtype != F32:
            v = pltpu.bitcast(v, F32)
        r = v.shape[0] // (8 * n)
        for j in range(v.shape[1] // LANES):
            seg[pl.ds(row, n), pl.ds(slot + j * r, r)] = (
                v[:, j * LANES:(j + 1) * LANES].reshape(n, r, 8, LANES))

    def seg_get(row, n, slot, cols, r=R):
        return jnp.concatenate(
            [seg[pl.ds(row, n), pl.ds(slot + j * r, r)].reshape(n * r * 8, LANES)
             for j in range(cols)], axis=1)

    w_u = [r.bitcast(U32) for r in (wq_hbm, wk_hbm, wv_hbm)]
    wo_u, w1_u, w2_u, w3_u, w4_u, wmod_u = (
        r.bitcast(U32) for r in (wo_hbm, w1_hbm, w2_hbm, w3_hbm, w4_hbm, wmod_hbm))

    b_copies = [
        pltpu.make_async_copy(w.at[:, _lanes(j)], dst.at[p0 + j], sem_b)
        for w, dst, p0 in ((w1_u, wb, 0), (w2_u, wb, ND), (w3_u, wb, 2 * ND), (w4_u, w4, 0))
        for j in range(w.shape[1] // LANES)]

    def mod_copy(j):
        return pltpu.make_async_copy(wmod_u.at[:, _lanes(j)], wb.at[j], sem_mod.at[j // ND])

    def mod_chunks(lo, hi, arrived=()):
        cv = c_ref[...].astype(F32)
        sc = jnp.broadcast_to(cv * jax.nn.sigmoid(cv), (8, D))
        for j in range(lo * ND, hi * ND):
            mod_copy(j).wait()
        for cp in arrived:
            cp.start()
        for j in range(lo * ND, hi * ND):
            mod[j // ND, :, _lanes(j % ND)] = _dot(sc, _panel(wb, j))

    def attention_phase(wqkv, wo, xs, xn, he, lhs, obuf, aout, acc, sem_w, sem_x, sem_wo):
        HP = H // 2
        NI = HP // PAIRS

        def w_copies(hp):
            return [pltpu.make_async_copy(w_u[m].at[:, i, hp, :], wqkv.at[6 * hp + 3 * i + m],
                                          sem_w.at[hp]) for m in range(3) for i in range(2)]

        def wo_copy(j):
            return pltpu.make_async_copy(wo_u.at[:, _lanes(j)], wo.at[j], sem_wo)

        def x_copy(i):
            sl = pl.ds(i * E, E)
            return pltpu.make_async_copy(x_hbm.at[:, sl, :], xs.at[:, sl, :], sem_x.at[min(i, 1)])

        def modulate_a(n):
            return n * _rows(1.0 + mod[1], n.shape[0]) + _rows(mod[0], n.shape[0])

        x_copy(0).start()
        for j in range(MOD_FIRST):
            mod_copy(j).start()

        with jax.named_scope("early_ln"):
            x_copy(0).wait()
            for j in range(MOD_FIRST, 2 * ND):
                mod_copy(j).start()
            first = w_copies(0)
            for cp in first[:W_FIRST]:
                cp.start()

            def early_norm(t, carry):
                xv = xs[pl.ds(t * 16, 16), pl.ds(0, E), :].astype(F32).reshape(16 * E, D)
                xn[pl.ds(pl.multiple_of(t * 16 * E, 16 * E), 16 * E), :] = _ln(xv)
            lax.fori_loop(0, NSEG // 16, early_norm, None)

        with jax.named_scope("mod_a"):
            mod_chunks(0, 1)
            mod_chunks(1, 2, first[W_FIRST:])
            hv = modulate_a(xn[...]).astype(BF16)
            for j in range(ND):
                he[j] = hv[:, j * LANES:(j + 1) * LANES]
            for cp in first:
                cp.wait()
            for hp in range(1, PREFETCH):
                for cp in w_copies(hp):
                    cp.start()

        extra = ([[functools.partial(x_copy, i)] for i in range(1, R)]
                 + [[functools.partial(mod_copy, j + u) for u in range(4)]
                    for j in range(2 * ND, 6 * ND, 4)]
                 + [[functools.partial(wo_copy, j + u) for u in range(2)] for j in range(0, ND, 2)])

        def look_ahead(hp0, pairs, span, tokens):
            for v in range(pairs):
                @pl.when(hp0 + v + PREFETCH < HP)
                def _():
                    for cp in w_copies(hp0 + v + PREFETCH):
                        cp.start()
            for k in span:
                @pl.when(hp0 == k)
                def _():
                    for cp in sum(extra[k:k + pairs], []):
                        cp().start()

            @pl.when(hp0 > 0)
            def _():
                for v in range(pairs):
                    for cp in w_copies(hp0 + v):
                        cp.wait()
            n = NSEG // (HP - TOK_FROM)
            for v in range(pairs):
                hp = hp0 + v
                todo = list(range(n)) if tokens else []
                for m in range(3):
                    p = 6 * hp + m
                    a, b = wqkv[p], wqkv[p + 3]
                    w = ((a & np.uint32(0xFFFF)) | (b << 16),
                         (a >> 16) | (b & np.uint32(0xFFFF0000)))
                    for u in range(2):
                        wqkv[p + 3 * u] = w[u]
                        y = _dot(_panels(he.bitcast(U32), 0, ND), pltpu.bitcast(w[u], BF16))
                        seg[pl.ds(1, NSEG), p + 3 * u] = y.reshape(NSEG, E, LANES)
                        for _ in range(-(-n // 5)):
                            if todo:
                                s = (hp - TOK_FROM) * n + todo.pop(0)
                                xv = xs[s].astype(F32)
                                if TOK_LATE:
                                    xv = jnp.where(
                                        _pin(hp0) == 0, xv, jnp.concatenate([y[:SEG]] * ND, axis=1))
                                seg_put(1 + s, TOK, modulate_a(_ln(xv)).astype(BF16))

        with jax.named_scope("look_ahead"):
            lax.fori_loop(0, TOK_FROM, lambda i, c: look_ahead(i, 1, range(TOK_FROM), False), None)
            for i in range(1, R):
                x_copy(i).wait()
        with jax.named_scope("look_ahead2"):
            lax.fori_loop(0, (HP - TOK_FROM) // PAIRS2, lambda i, c: look_ahead(
                TOK_FROM + i * PAIRS2, PAIRS2, range(TOK_FROM, HP, PAIRS2), True), None)

        with jax.named_scope("mod_b"):
            mod_chunks(2, 6)
            for j in range(ND):
                wo_copy(j).wait()
            for cp in b_copies:
                cp.start()

        def set_lhs(mem, s, j):
            tok = pltpu.bitcast(seg_get(1 + s, 1, TOK + j * R // 2, 1, R // 2), BF16)
            head = jnp.concatenate([mem, tok[:16].astype(F32)[E:]], axis=0).astype(BF16)
            lhs[j] = jnp.concatenate([head, tok[16:]], axis=0)

        def finish_tokens(s, row):
            x1 = xs[s].astype(F32) + _rows(mod[2], SEG) * aout[...]
            h = _ln(x1) * _rows(1.0 + mod[4], SEG) + _rows(mod[3], SEG)
            seg_put(row, X1, x1)
            seg_put(row, HB, h)
            seg_put(row, HN, _ln(h).astype(BF16))

        for j in range(ND):
            set_lhs(mem0_ref[:, _lanes(j)].astype(F32), 0, j)
        aout[...] = jnp.zeros_like(aout)
        lhs_u = lhs.bitcast(U32)

        def step(s):
            ri = lax.broadcasted_iota(jnp.int32, (L, LP), 0)
            ci = lax.broadcasted_iota(jnp.int32, (L, LP), 1)
            keep = ((ri < M) | (ri >= ci)) & (ci < L)
            fill = jnp.where(ci < L, -1e9, -jnp.inf).astype(F32)
            zpad = jnp.zeros((LP - L, LANES), F32)

            def project(h, m):
                p = 3 * h + m
                if h < KSPLIT and m == 0:
                    y = acc[pl.ds(0, SEG), _lanes(h)] + _dot(
                        _panels(lhs_u, 0, ND // 2), _panel(wqkv, p, 0, D // 4))
                else:
                    y = _dot(_panels(lhs_u, 0, ND), _panel(wqkv, p))
                parts = [y[:M], seg[1 + s, p], y[M:]]
                if m == 0:
                    return jnp.concatenate(parts, axis=0)
                return jnp.concatenate(parts + [zpad], axis=0).astype(BF16)

            def probs(q, k):
                sc = jnp.where(keep, _dot_nt(q, k) * scale, fill)
                e = jnp.exp(sc - jnp.max(sc, axis=-1, keepdims=True))
                return e / jnp.sum(e, axis=-1, keepdims=True)

            G = HEAD_GROUP
            NG = H // G
            KH = (H - G) * LANES

            for h in range(KSPLIT):
                acc[pl.ds(0, SEG), _lanes(h)] = _dot(
                    _panels(lhs_u, ND // 2, ND // 2), _panel(wqkv, 3 * h, D // 4, D // 4))
            prev = None
            for g in range(NG + 1):
                if g == FINISH_AT:
                    finish_tokens(jnp.maximum(s - 1, 0), s)
                heads = range(g * G, (g + 1) * G) if g < NG else ()
                q = [project(h, 0) for h in heads]
                if prev is not None:
                    pr = [probs(a, b) for a, b in zip(prev[0], prev[1])]
                k = [project(h, 1) for h in heads]
                v = [project(h, 2) for h in heads]
                if g == NG:
                    for j in range(WO_SPLIT):
                        acc[:, _lanes(j)] = _dot(obuf[:, pl.ds(0, KH)], _panel(wo, j, 0, KH // 2))
                if prev is not None:
                    for u in range(G):
                        obuf[:, _lanes((g - 1) * G + u)] = _dot(pr[u], prev[2][u])
                prev = (q, k, v)
            for j in reversed(range(ND)):
                if j < WO_SPLIT:
                    y = acc[:, _lanes(j)] + _dot(
                        obuf[:, _lanes(H - G, G)], _panel(wo, j, KH // 2, G * LANES // 2))
                else:
                    y = _dot(obuf[...], _panel(wo, j))
                set_lhs(y[:M], jnp.minimum(s + 1, NSEG - 1), j)
                aout[:, _lanes(j)] = y[M:]

        def steps(i, carry):
            for u in range(UNROLL):
                step(i * UNROLL + u)

        with jax.named_scope("steps"):
            lax.fori_loop(0, NSEG // UNROLL, steps, None)
            for s in range(NSEG // UNROLL * UNROLL, NSEG):
                step(s)
        finish_tokens(NSEG - 1, NSEG)

    pl.run_scoped(
        attention_phase,
        pltpu.VMEM((3 * H, D // 2, LANES), U32),
        pltpu.VMEM((ND, H * LANES // 2, LANES), U32),
        pltpu.VMEM((NSEG, SEG, D), BF16),
        pltpu.VMEM((NSEG * E, D), F32),
        pltpu.VMEM((ND, NSEG * E, LANES), BF16),
        pltpu.VMEM((ND, SEG, LANES), BF16),
        pltpu.VMEM((L, H * LANES), F32),
        pltpu.VMEM((SEG, D), F32),
        pltpu.VMEM((L, D), F32),
        pltpu.SemaphoreType.DMA((H // 2,)),
        pltpu.SemaphoreType.DMA((2,)),
        pltpu.SemaphoreType.DMA(()),
    )

    def mixer_phase(gbuf, obuf, ops, sem_out):
        NT = S // TM
        TS = TM // SEG
        ops_u = ops.bitcast(U32)
        for cp in b_copies:
            cp.wait()
        gbuf[:, pl.ds(0, 8), :] = jnp.zeros((ND, 8, LANES), F32)
        gbuf[:, pl.ds(S + 8, 8), :] = jnp.zeros((ND, 8, LANES), F32)

        def gate(t):
            for j in range(ND):
                a = pltpu.bitcast(seg_get(1 + t * TS, TS, HN, ND, R // 2), BF16)
                gbuf[j, pl.ds(pl.multiple_of(t * TM + 8, 8), TM), :] = jax.nn.gelu(
                    _dot(a, _panel(wb, j)), approximate=True)

        def mix(t):
            for j in range(ND):
                shifted = jnp.concatenate(
                    [gbuf[k, pl.ds(t * TM + 8 + (-1, 1, -2, 2)[4 * k // ND], TM), :]
                     for k in range(ND)], axis=1)
                y = seg_get(1 + t * TS, TS, HB + j * R, 1) + _dot(shifted, _panel(wb, ND + j))
                seg_put(1 + t * TS, HB + j * R, y, TS)

        def up_in(t):
            def task(u, after=lambda v: v):
                v = _ln(after(seg_get(1 + t * TS + u, 1, HB, ND))).astype(BF16)
                for j in range(ND):
                    ops[j, pl.ds(u * SEG, SEG), :] = v[:, j * LANES:(j + 1) * LANES]
            return [functools.partial(task, u) for u in range(TS)]

        def up():
            for j in range(NF):
                ops[ND + j] = jax.nn.gelu(
                    _dot(_panels(ops_u, 0, ND), _panel(wb, 2 * ND + j)),
                    approximate=True).astype(BF16)

        def down(t, pin, tasks):
            done = []
            nk = NF // DOWN_SPLIT
            per = -(-len(tasks) // (ND * DOWN_SPLIT - TASK_LAG))
            for j in range(ND):
                y = seg_get(1 + t * TS, TS, HB + j * R, 1)
                for k in range(0, NF, nk):
                    if len(done) >= TASK_LAG:
                        m = jnp.concatenate([done[-TASK_LAG][:SEG]] * ND, axis=1)
                        for task in tasks[:per]:
                            task(lambda v: jnp.where(pin == 0, v, m))
                        tasks = tasks[per:]
                    a = jnp.concatenate([_panel(ops_u, ND + k + pin),
                                         _panels(ops_u, ND + k + 1, nk - 1)], axis=1)
                    y = y + _dot(a, _panel(w4, j, k * LANES // 2, nk * LANES // 2))
                    done.append(y)
                y = seg_get(1 + t * TS, TS, X1 + j * R, 1) + _rows(mod[5, :, _lanes(j)], TM) * y
                obuf[pl.ds(pl.multiple_of(t * TM, TM), TM), _lanes(j)] = y.astype(BF16)

        def out_copy(t):
            r = pl.ds(pl.multiple_of(t * TM, TM), TM)
            return pltpu.make_async_copy(obuf.at[r], out_hbm.at[r], sem_out)

        def tile(t, pin, ahead):
            if ahead >= 2 and GATE_AHEAD:
                gate(t + 2)
            up()
            if ahead >= 1:
                mix(t + 1)
            down(t, pin, up_in(t + 1) if ahead >= 1 else [])
            out_copy(t).start()
            return pin

        with jax.named_scope("gate"):
            if GATE_AHEAD:
                gate(0)
                gate(1)
            else:
                lax.fori_loop(0, NT, lambda t, c: gate(t), None, unroll=2)
            mix(0)
            for task in up_in(0):
                task()
        last = 2 if GATE_AHEAD else 1
        with jax.named_scope("mlp"):
            pin = lax.fori_loop(0, NT - last, lambda t, c: tile(t, _pin(t), 2), 0)
        with jax.named_scope("mlp2"):
            for t in range(NT - last, NT):
                tile(t, pin, NT - 1 - t)
        for t in range(NT):
            out_copy(t).wait()

    pl.run_scoped(
        mixer_phase,
        pltpu.VMEM((ND, S + 16, LANES), F32),
        pltpu.VMEM((S, D), BF16),
        pltpu.VMEM((ND + NF, TM, LANES), BF16),
        pltpu.SemaphoreType.DMA(()))


@functools.partial(jax.jit, static_argnames=("A_seg_len",))
def pallas_adaLN_cond__memory_aug_recurrent_mem_tr__mixer_s_mlp__prompt_kernel(
    A_x, A_mem0, A_Wq, A_Wk, A_Wv, A_Wo, A_seg_len, B_x, B_w1, B_w2, B_w3, B_w4, c, w_mod,
):
    del B_x
    B, S, D = A_x.shape
    H, Dh = A_Wq.shape[1:]
    M = A_mem0.shape[1]
    F = B_w3.shape[1]
    SEG = A_seg_len
    assert B == 1 and Dh == LANES and M == 8 and SEG % 16 == 0 and S % SEG == 0
    ND, NF = D // LANES, F // LANES
    hbm = pl.BlockSpec(memory_space=pl.ANY)
    vmem = pl.BlockSpec(memory_space=pltpu.VMEM)
    out = pl.pallas_call(
        functools.partial(_kernel, S=S, D=D, H=H, M=M, SEG=SEG, F=F),
        out_shape=jax.ShapeDtypeStruct((S, D), A_x.dtype),
        in_specs=[hbm, vmem, hbm, hbm, hbm, hbm, hbm, hbm, hbm, hbm, vmem, hbm],
        out_specs=hbm,
        scratch_shapes=[
            pltpu.VMEM((max(6 * ND, 2 * ND + NF), D // 2, LANES), U32),
            pltpu.VMEM((ND, F // 2, LANES), U32),
            pltpu.VMEM((S // SEG + 1, 3 * H + ND * SEG // 16, 8, LANES), F32),
            pltpu.VMEM((6, 8, D), F32),
            pltpu.SemaphoreType.DMA((6,)),
            pltpu.SemaphoreType.DMA(()),
        ],
        compiler_params=pltpu.CompilerParams(vmem_limit_bytes=110 * 1024 * 1024),
    )(A_x.reshape(S // SEG, SEG, D), A_mem0.reshape(M, D),
      *(w.reshape(D // 2, 2, H, Dh) for w in (A_Wq, A_Wk, A_Wv)),
      A_Wo.reshape(H * Dh, D), B_w1, B_w2, B_w3, B_w4, c, w_mod)
    return out.reshape(B, S, D)
```

```python
import functools

import jax
import jax.numpy as jnp
import numpy as np
from jax import lax
import jax.experimental.pallas as pl
import jax.experimental.pallas.tpu as pltpu

F32 = jnp.float32
BF16 = jnp.bfloat16
U32 = jnp.uint32
LANES = 128
EPS = 1e-5
MASKED = -1e9

HEAD_GROUP = 4
UNROLL = 2
PREFETCH = 4
TM = 128


def _ln(x):
    m = jnp.mean(x, axis=-1, keepdims=True)
    d = x - m
    v = jnp.mean(d * d, axis=-1, keepdims=True)
    return d * lax.rsqrt(v + EPS)


def _dot(a, b):
    return jnp.dot(a, b, preferred_element_type=F32)


def _dot_nt(a, b):
    return lax.dot_general(a, b, (((1,), (1,)), ((), ())), preferred_element_type=F32)


def _panel(ref, p, r0=None, nr=None):
    w = ref[p] if r0 is None else ref[p, pl.ds(r0, nr), :]
    return pltpu.bitcast(w, BF16)


def _panels(ref, p0, n):
    return jnp.concatenate([_panel(ref, p0 + j) for j in range(n)], axis=1)


def _pin(i):
    return i >> 24


def _after(pin, v, y):
    return jnp.where(pin == 0, v, jnp.concatenate([y[:v.shape[0]]] * (v.shape[1] // LANES), axis=1))


def _lanes(j, n=1):
    return pl.ds(j * LANES, n * LANES)


def _rows(v, n):
    return jnp.concatenate([v] * (n // 8), axis=0)


def _start(copies):
    for cp in copies:
        cp.start()


def _wait(copies):
    for cp in copies:
        cp.wait()


def _kernel(x_hbm, mem0_ref, wq_hbm, wk_hbm, wv_hbm, wo_hbm, w1_hbm, w2_hbm, w3_hbm, w4_hbm,
            c_ref, wmod_hbm, out_hbm,
            wb, w4, seg, mod, sem_mod, sem_b,
            *, S, D, H, M, SEG, F):
    NSEG = S // SEG
    E = M
    L = M + SEG
    LP = -(-L // 16) * 16
    ND = D // LANES
    NF = F // LANES
    R = SEG // 8
    scale = LANES ** -0.5
    TOK = 3 * H
    X1, HB, HN = 0, R * ND, 2 * R * ND

    def seg_put(row, slot, v, n=1):
        if v.dtype != F32:
            v = pltpu.bitcast(v, F32)
        r = v.shape[0] // (8 * n)
        for j in range(v.shape[1] // LANES):
            seg[pl.ds(row, n), pl.ds(slot + j * r, r)] = (
                v[:, j * LANES:(j + 1) * LANES].reshape(n, r, 8, LANES))

    def seg_get(row, n, slot, cols, r=R):
        return jnp.concatenate(
            [seg[pl.ds(row, n), pl.ds(slot + j * r, r)].reshape(n * r * 8, LANES)
             for j in range(cols)], axis=1)

    w_u = [r.bitcast(U32) for r in (wq_hbm, wk_hbm, wv_hbm)]
    wo_u, w1_u, w2_u, w3_u, w4_u, wmod_u = (
        r.bitcast(U32) for r in (wo_hbm, w1_hbm, w2_hbm, w3_hbm, w4_hbm, wmod_hbm))

    mixer_copies = [
        pltpu.make_async_copy(w.at[:, _lanes(j)], dst.at[p0 + j], sem_b)
        for w, dst, p0 in ((w1_u, wb, 0), (w2_u, wb, ND), (w3_u, wb, 2 * ND), (w4_u, w4, 0))
        for j in range(w.shape[1] // LANES)]

    def mod_copies(lo, hi):
        return [pltpu.make_async_copy(wmod_u.at[:, _lanes(j)], wb.at[j], sem_mod.at[j // ND])
                for j in range(lo, hi)]

    def mod_chunks(lo, hi, arrived=()):
        cv = c_ref[...].astype(F32)
        sc = jnp.broadcast_to(cv * jax.nn.sigmoid(cv), (8, D))
        _wait(mod_copies(lo * ND, hi * ND))
        _start(arrived)
        for j in range(lo * ND, hi * ND):
            mod[j // ND, :, _lanes(j % ND)] = _dot(sc, _panel(wb, j))

    def attention_phase(wqkv, wo, xs, xn, he, lhs, obuf, aout, acc, sem_w, sem_x, sem_wo):
        HP = H // 2

        def w_copies(hp):
            return [pltpu.make_async_copy(w_u[m].at[:, i, hp, :], wqkv.at[6 * hp + 3 * i + m],
                                          sem_w.at[hp]) for m in range(3) for i in range(2)]

        def wo_copies(lo, hi):
            return [pltpu.make_async_copy(wo_u.at[:, _lanes(j)], wo.at[j], sem_wo)
                    for j in range(lo, hi)]

        def x_copies(lo, hi):
            return [pltpu.make_async_copy(x_hbm.at[:, pl.ds(i * E, E), :],
                                          xs.at[:, pl.ds(i * E, E), :], sem_x.at[min(i, 1)])
                    for i in range(lo, hi)]

        def modulate_a(n):
            return n * _rows(1.0 + mod[1], n.shape[0]) + _rows(mod[0], n.shape[0])

        first = w_copies(0)
        _start(x_copies(0, 1) + mod_copies(0, ND // 2))
        _wait(x_copies(0, 1))
        _start(mod_copies(ND // 2, 2 * ND) + first[:4])

        def early_norm(t, carry):
            xv = xs[pl.ds(t * 16, 16), pl.ds(0, E), :].astype(F32).reshape(16 * E, D)
            xn[pl.ds(pl.multiple_of(t * 16 * E, 16 * E), 16 * E), :] = _ln(xv)
        lax.fori_loop(0, NSEG // 16, early_norm, None)

        mod_chunks(0, 1)
        mod_chunks(1, 2, first[4:])
        hv = modulate_a(xn[...]).astype(BF16)
        for j in range(ND):
            he[j] = hv[:, j * LANES:(j + 1) * LANES]
        _wait(first)
        for hp in range(1, PREFETCH):
            _start(w_copies(hp))

        extra = ([(x_copies, i, i + 1) for i in range(1, R)]
                 + [(mod_copies, j, j + 4) for j in range(2 * ND, 6 * ND, 4)]
                 + [(wo_copies, j, j + 2) for j in range(0, ND, 2)])
        assert R - 1 <= HP // 2 and len(extra) <= HP

        def look_ahead(hp0, pairs, starts, tokens):
            for v in range(pairs):
                @pl.when(hp0 + v + PREFETCH < HP)
                def _():
                    _start(w_copies(hp0 + v + PREFETCH))
            for k in starts:
                @pl.when(hp0 == k)
                def _():
                    for copies, lo, hi in extra[k:k + pairs]:
                        _start(copies(lo, hi))

            @pl.when(hp0 > 0)
            def _():
                for v in range(pairs):
                    _wait(w_copies(hp0 + v))
            n = NSEG // (HP // 2)
            for v in range(pairs):
                hp = hp0 + v
                todo = list(range(n)) if tokens else []
                for m in range(3):
                    p = 6 * hp + m
                    a, b = wqkv[p], wqkv[p + 3]
                    w = ((a & np.uint32(0xFFFF)) | (b << 16),
                         (a >> 16) | (b & np.uint32(0xFFFF0000)))
                    for u in range(2):
                        wqkv[p + 3 * u] = w[u]
                        y = _dot(_panels(he.bitcast(U32), 0, ND), pltpu.bitcast(w[u], BF16))
                        seg[pl.ds(1, NSEG), p + 3 * u] = y.reshape(NSEG, E, LANES)
                        for i in todo[:-(-n // 5)]:
                            s = (hp - HP // 2) * n + i
                            xv = _after(_pin(hp0), xs[s].astype(F32), y)
                            seg_put(1 + s, TOK, modulate_a(_ln(xv)).astype(BF16))
                        todo = todo[-(-n // 5):]

        lax.fori_loop(0, HP // 2, lambda i, c: look_ahead(i, 1, range(HP // 2), False), None)
        _wait(x_copies(1, R))
        lax.fori_loop(
            0, HP // 4,
            lambda i, c: look_ahead(HP // 2 + 2 * i, 2, range(HP // 2, HP, 2), True), None)

        mod_chunks(2, 6)
        _wait(wo_copies(0, ND))
        _start(mixer_copies)

        def set_lhs(mem, s, j):
            tok = pltpu.bitcast(seg_get(1 + s, 1, TOK + j * R // 2, 1, R // 2), BF16)
            head = jnp.concatenate([mem, tok[:16].astype(F32)[E:]], axis=0).astype(BF16)
            lhs[j] = jnp.concatenate([head, tok[16:]], axis=0)

        def finish_tokens(s, row):
            x1 = xs[s].astype(F32) + _rows(mod[2], SEG) * aout[...]
            h = _ln(x1) * _rows(1.0 + mod[4], SEG) + _rows(mod[3], SEG)
            seg_put(row, X1, x1)
            seg_put(row, HB, h)
            seg_put(row, HN, _ln(h).astype(BF16))

        for j in range(ND):
            set_lhs(mem0_ref[:, _lanes(j)].astype(F32), 0, j)
        aout[...] = jnp.zeros_like(aout)
        lhs_u = lhs.bitcast(U32)

        def step(s):
            G = HEAD_GROUP
            NG = H // G
            KH = (H - G) * LANES
            ri = lax.broadcasted_iota(jnp.int32, (L, LP), 0)
            ci = lax.broadcasted_iota(jnp.int32, (L, LP), 1)
            keep = ((ri < M) | (ri >= ci)) & (ci < L)
            fill = jnp.where(ci < L, MASKED, -jnp.inf).astype(F32)
            zpad = jnp.zeros((LP - L, LANES), F32)

            def project(h, m):
                p = 3 * h + m
                if h < G and m == 0:
                    y = acc[pl.ds(0, SEG), _lanes(h)] + _dot(
                        _panels(lhs_u, 0, ND // 2), _panel(wqkv, p, 0, D // 4))
                else:
                    y = _dot(_panels(lhs_u, 0, ND), _panel(wqkv, p))
                parts = [y[:M], seg[1 + s, p], y[M:]]
                if m == 0:
                    return jnp.concatenate(parts, axis=0)
                return jnp.concatenate(parts + [zpad], axis=0).astype(BF16)

            def probs(q, k):
                sc = jnp.where(keep, _dot_nt(q, k) * scale, fill)
                e = jnp.exp(sc - jnp.max(sc, axis=-1, keepdims=True))
                return e / jnp.sum(e, axis=-1, keepdims=True)

            for h in range(G):
                acc[pl.ds(0, SEG), _lanes(h)] = _dot(
                    _panels(lhs_u, ND // 2, ND // 2), _panel(wqkv, 3 * h, D // 4, D // 4))
            finish_tokens(jnp.maximum(s - 1, 0), s)
            prev = None
            for g in range(NG + 1):
                heads = range(g * G, (g + 1) * G) if g < NG else ()
                q = [project(h, 0) for h in heads]
                if prev is not None:
                    pr = [probs(a, b) for a, b in zip(prev[0], prev[1])]
                k = [project(h, 1) for h in heads]
                v = [project(h, 2) for h in heads]
                if g == NG:
                    for j in range(ND // 2):
                        acc[:, _lanes(j)] = _dot(obuf[:, pl.ds(0, KH)], _panel(wo, j, 0, KH // 2))
                if prev is not None:
                    for u in range(G):
                        obuf[:, _lanes((g - 1) * G + u)] = _dot(pr[u], prev[2][u])
                prev = (q, k, v)
            for j in reversed(range(ND)):
                if j < ND // 2:
                    y = acc[:, _lanes(j)] + _dot(
                        obuf[:, _lanes(H - G, G)], _panel(wo, j, KH // 2, G * LANES // 2))
                else:
                    y = _dot(obuf[...], _panel(wo, j))
                set_lhs(y[:M], jnp.minimum(s + 1, NSEG - 1), j)
                aout[:, _lanes(j)] = y[M:]

        def steps(i, carry):
            for u in range(UNROLL):
                step(i * UNROLL + u)

        lax.fori_loop(0, NSEG // UNROLL, steps, None)
        _wait(mixer_copies)
        finish_tokens(NSEG - 1, NSEG)

    pl.run_scoped(
        attention_phase,
        pltpu.VMEM((3 * H, D // 2, LANES), U32),
        pltpu.VMEM((ND, H * LANES // 2, LANES), U32),
        pltpu.VMEM((NSEG, SEG, D), BF16),
        pltpu.VMEM((NSEG * E, D), F32),
        pltpu.VMEM((ND, NSEG * E, LANES), BF16),
        pltpu.VMEM((ND, SEG, LANES), BF16),
        pltpu.VMEM((L, H * LANES), F32),
        pltpu.VMEM((SEG, D), F32),
        pltpu.VMEM((L, D), F32),
        pltpu.SemaphoreType.DMA((H // 2,)),
        pltpu.SemaphoreType.DMA((2,)),
        pltpu.SemaphoreType.DMA(()),
    )

    def mixer_phase(gbuf, obuf, ops, sem_out):
        NT = S // TM
        TS = TM // SEG
        ops_u = ops.bitcast(U32)
        gbuf[:, pl.ds(0, 8), :] = jnp.zeros((ND, 8, LANES), F32)
        gbuf[:, pl.ds(S + 8, 8), :] = jnp.zeros((ND, 8, LANES), F32)

        def gate(t):
            for j in range(ND):
                a = pltpu.bitcast(seg_get(1 + t * TS, TS, HN, ND, R // 2), BF16)
                gbuf[j, pl.ds(pl.multiple_of(t * TM + 8, 8), TM), :] = jax.nn.gelu(
                    _dot(a, _panel(wb, j)), approximate=True)

        def mix(t):
            for j in range(ND):
                shifted = jnp.concatenate(
                    [gbuf[k, pl.ds(t * TM + 8 + (-1, 1, -2, 2)[4 * k // ND], TM), :]
                     for k in range(ND)], axis=1)
                y = seg_get(1 + t * TS, TS, HB + j * R, 1) + _dot(shifted, _panel(wb, ND + j))
                seg_put(1 + t * TS, HB + j * R, y, TS)

        def norm(t, u, when=lambda v: v):
            v = _ln(when(seg_get(1 + t * TS + u, 1, HB, ND))).astype(BF16)
            for j in range(ND):
                ops[j, pl.ds(u * SEG, SEG), :] = v[:, j * LANES:(j + 1) * LANES]

        def out_copy(t):
            r = pl.ds(pl.multiple_of(t * TM, TM), TM)
            return pltpu.make_async_copy(obuf.at[r], out_hbm.at[r], sem_out)

        def tile(t, pin, ahead):
            if ahead >= 2:
                gate(t + 2)
            for j in range(NF):
                ops[ND + j] = jax.nn.gelu(
                    _dot(_panels(ops_u, 0, ND), _panel(wb, 2 * ND + j)),
                    approximate=True).astype(BF16)
            if ahead >= 1:
                mix(t + 1)
            done = []
            for j in range(ND):
                if ahead >= 1 and 2 <= j < 2 + TS:
                    norm(t + 1, j - 2, lambda v: _after(pin, v, done[-2]))
                a = jnp.concatenate(
                    [_panel(ops_u, ND + pin), _panels(ops_u, ND + 1, NF - 1)], axis=1)
                y = seg_get(1 + t * TS, TS, HB + j * R, 1) + _dot(a, _panel(w4, j))
                done.append(y)
                y = seg_get(1 + t * TS, TS, X1 + j * R, 1) + _rows(mod[5, :, _lanes(j)], TM) * y
                obuf[pl.ds(pl.multiple_of(t * TM, TM), TM), _lanes(j)] = y.astype(BF16)
            out_copy(t).start()
            return pin

        gate(0)
        gate(1)
        mix(0)
        for u in range(TS):
            norm(0, u)
        pin = lax.fori_loop(0, NT - 2, lambda t, c: tile(t, _pin(t), 2), 0)
        tile(NT - 2, pin, 1)
        tile(NT - 1, pin, 0)
        _wait([out_copy(t) for t in range(NT)])

    pl.run_scoped(
        mixer_phase,
        pltpu.VMEM((ND, S + 16, LANES), F32),
        pltpu.VMEM((S, D), BF16),
        pltpu.VMEM((ND + NF, TM, LANES), BF16),
        pltpu.SemaphoreType.DMA(()))


@functools.partial(jax.jit, static_argnames=("A_seg_len",))
def pallas_adaLN_cond__memory_aug_recurrent_mem_tr__mixer_s_mlp__prompt_kernel(
    A_x, A_mem0, A_Wq, A_Wk, A_Wv, A_Wo, A_seg_len, B_x, B_w1, B_w2, B_w3, B_w4, c, w_mod,
):
    del B_x
    B, S, D = A_x.shape
    H, Dh = A_Wq.shape[1:]
    M = A_mem0.shape[1]
    F = B_w3.shape[1]
    SEG = A_seg_len
    assert (B, D, H, Dh, M, SEG) == (1, 1024, 32, LANES, 8, 32) and A_x.dtype == BF16
    assert S % (16 * SEG) == 0 and F % LANES == 0
    ND, NF = D // LANES, F // LANES
    hbm = pl.BlockSpec(memory_space=pl.ANY)
    vmem = pl.BlockSpec(memory_space=pltpu.VMEM)
    out = pl.pallas_call(
        functools.partial(_kernel, S=S, D=D, H=H, M=M, SEG=SEG, F=F),
        out_shape=jax.ShapeDtypeStruct((S, D), A_x.dtype),
        in_specs=[hbm, vmem, hbm, hbm, hbm, hbm, hbm, hbm, hbm, hbm, vmem, hbm],
        out_specs=hbm,
        scratch_shapes=[
            pltpu.VMEM((max(6 * ND, 2 * ND + NF), D // 2, LANES), U32),
            pltpu.VMEM((ND, F // 2, LANES), U32),
            pltpu.VMEM((S // SEG + 1, 3 * H + ND * SEG // 16, 8, LANES), F32),
            pltpu.VMEM((6, 8, D), F32),
            pltpu.SemaphoreType.DMA((6,)),
            pltpu.SemaphoreType.DMA(()),
        ],
        compiler_params=pltpu.CompilerParams(vmem_limit_bytes=110 * 1024 * 1024),
    )(A_x.reshape(S // SEG, SEG, D), A_mem0.reshape(M, D),
      *(w.reshape(D // 2, 2, H, Dh) for w in (A_Wq, A_Wk, A_Wv)),
      A_Wo.reshape(H * Dh, D), B_w1, B_w2, B_w3, B_w4, c, w_mod)
    return out.reshape(B, S, D)
```

```python
import functools

import jax
import jax.numpy as jnp
import numpy as np
from jax import lax
import jax.experimental.pallas as pl
import jax.experimental.pallas.tpu as pltpu

F32 = jnp.float32
BF16 = jnp.bfloat16
U32 = jnp.uint32
LANES = 128
EPS = 1e-5
MASKED = -1e9

HEAD_GROUP = 4
UNROLL = 2
PREFETCH = 3
TM = 128


def _ln(x):
    m = jnp.mean(x, axis=-1, keepdims=True)
    d = x - m
    v = jnp.mean(d * d, axis=-1, keepdims=True)
    return d * lax.rsqrt(v + EPS)


def _dot(a, b):
    return jnp.dot(a, b, preferred_element_type=F32)


def _dot_nt(a, b):
    return lax.dot_general(a, b, (((1,), (1,)), ((), ())), preferred_element_type=F32)


def _panel(ref, p, r0=None, nr=None):
    w = ref[p] if r0 is None else ref[p, pl.ds(r0, nr), :]
    return pltpu.bitcast(w, BF16)


def _panels(ref, p0, n):
    return jnp.concatenate([_panel(ref, p0 + j) for j in range(n)], axis=1)


def _pin(i):
    return i >> 24


def _after(pin, v, y):
    return jnp.where(pin == 0, v, jnp.concatenate([y[:v.shape[0]]] * (v.shape[1] // LANES), axis=1))


def _lanes(j, n=1):
    return pl.ds(j * LANES, n * LANES)


def _rows(v, n):
    return jnp.concatenate([v] * (n // 8), axis=0)


def _start(copies):
    for cp in copies:
        cp.start()


def _wait(copies):
    for cp in copies:
        cp.wait()


def _kernel(x_hbm, mem0_ref, wq_hbm, wk_hbm, wv_hbm, wo_hbm, w1_hbm, w2_hbm, w3_hbm, w4_hbm,
            c_ref, wmod_hbm, out_hbm,
            wb, w4, seg, mod, sem_mod, sem_b,
            *, S, D, H, M, SEG, F):
    NSEG = S // SEG
    E = M
    L = M + SEG
    LP = -(-L // 16) * 16
    ND = D // LANES
    NF = F // LANES
    R = SEG // 8
    scale = LANES ** -0.5
    TOK = 3 * H
    X1, HB, HN = 0, R * ND, 2 * R * ND

    def seg_put(row, slot, v, n=1):
        if v.dtype != F32:
            v = pltpu.bitcast(v, F32)
        r = v.shape[0] // (8 * n)
        for j in range(v.shape[1] // LANES):
            seg[pl.ds(row, n), pl.ds(slot + j * r, r)] = (
                v[:, j * LANES:(j + 1) * LANES].reshape(n, r, 8, LANES))

    def seg_get(row, n, slot, cols, r=R):
        return jnp.concatenate(
            [seg[pl.ds(row, n), pl.ds(slot + j * r, r)].reshape(n * r * 8, LANES)
             for j in range(cols)], axis=1)

    w_u = [r.bitcast(U32) for r in (wq_hbm, wk_hbm, wv_hbm)]
    wo_u, w1_u, w2_u, w3_u, w4_u, wmod_u = (
        r.bitcast(U32) for r in (wo_hbm, w1_hbm, w2_hbm, w3_hbm, w4_hbm, wmod_hbm))

    mixer_copies = [
        pltpu.make_async_copy(w.at[:, _lanes(j)], dst.at[p0 + j], sem_b)
        for w, dst, p0 in ((w1_u, wb, 0), (w2_u, wb, ND), (w3_u, wb, 2 * ND), (w4_u, w4, 0))
        for j in range(w.shape[1] // LANES)]

    def mod_copies(lo, hi):
        return [pltpu.make_async_copy(wmod_u.at[:, _lanes(j)], wb.at[j], sem_mod.at[j // ND])
                for j in range(lo, hi)]

    def mod_chunks(lo, hi, arrived=()):
        cv = c_ref[...].astype(F32)
        sc = jnp.broadcast_to(cv * jax.nn.sigmoid(cv), (8, D))
        _wait(mod_copies(lo * ND, hi * ND))
        _start(arrived)
        for j in range(lo * ND, hi * ND):
            mod[j // ND, :, _lanes(j % ND)] = _dot(sc, _panel(wb, j))

    def attention_phase(wqkv, wo, xs, xn, he, lhs, obuf, aout, acc, sem_w, sem_x, sem_wo):
        HP = H // 2

        def w_copies(hp, which=(0, 1, 2)):
            return [pltpu.make_async_copy(w_u[m].at[:, i, hp, :], wqkv.at[6 * hp + 3 * i + m],
                                          sem_w.at[3 * hp + m]) for m in which for i in range(2)]

        def wo_copies(lo, hi):
            return [pltpu.make_async_copy(wo_u.at[:, _lanes(j)], wo.at[j], sem_wo)
                    for j in range(lo, hi)]

        def x_copies(lo, hi):
            return [pltpu.make_async_copy(x_hbm.at[:, pl.ds(i * E, E), :],
                                          xs.at[:, pl.ds(i * E, E), :], sem_x.at[min(i, 1)])
                    for i in range(lo, hi)]

        def modulate_a(n):
            return n * _rows(1.0 + mod[1], n.shape[0]) + _rows(mod[0], n.shape[0])

        _start(x_copies(0, 1) + mod_copies(0, ND // 2))
        _wait(x_copies(0, 1))
        _start(mod_copies(ND // 2, 2 * ND))

        def early_norm(t, carry):
            xv = xs[pl.ds(t * 16, 16), pl.ds(0, E), :].astype(F32).reshape(16 * E, D)
            xn[pl.ds(pl.multiple_of(t * 16 * E, 16 * E), 16 * E), :] = _ln(xv)
        lax.fori_loop(0, NSEG // 16, early_norm, None)

        mod_chunks(0, 1, w_copies(0, (0,)))
        mod_chunks(1, 2, w_copies(0, (1, 2)))
        hv = modulate_a(xn[...]).astype(BF16)
        for j in range(ND):
            he[j] = hv[:, j * LANES:(j + 1) * LANES]

        extra = ([(x_copies, i, i + 1) for i in range(1, R)]
                 + [(mod_copies, j, j + 4) for j in range(2 * ND, 6 * ND, 4)]
                 + [(wo_copies, j, j + 2) for j in range(0, ND, 2)])
        assert R <= HP // 2 and len(extra) < HP

        def look_ahead(p, side=None):
            a, b = wqkv[p], wqkv[p + 3]
            w = ((a & np.uint32(0xFFFF)) | (b << 16), (a >> 16) | (b & np.uint32(0xFFFF0000)))
            for u in range(2):
                wqkv[p + 3 * u] = w[u]
                y = _dot(_panels(he.bitcast(U32), 0, ND), pltpu.bitcast(w[u], BF16))
                seg[pl.ds(1, NSEG), p + 3 * u] = y.reshape(NSEG, E, LANES)
                if side is not None:
                    side(y)

        def head_pairs(hp0, pairs, starts, tokens):
            for v in range(pairs):
                @pl.when(hp0 + v + PREFETCH < HP)
                def _():
                    _start(w_copies(hp0 + v + PREFETCH))
            for k in starts:
                @pl.when(hp0 == k)
                def _():
                    for copies, lo, hi in extra[k - 1:k - 1 + pairs]:
                        _start(copies(lo, hi))
            for v in range(pairs):
                _wait(w_copies(hp0 + v))
            n = NSEG // (HP // 2)
            for v in range(pairs):
                todo = list(range(n))

                def modulate_tokens(y):
                    for i in todo[:-(-n // 5)]:
                        s = (hp0 + v - HP // 2) * n + i
                        xv = _after(_pin(hp0), xs[s].astype(F32), y)
                        seg_put(1 + s, TOK, modulate_a(_ln(xv)).astype(BF16))
                    del todo[:-(-n // 5)]

                for m in range(3):
                    look_ahead(6 * (hp0 + v) + m, modulate_tokens if tokens else None)

        for m in range(3):
            _wait(w_copies(0, (m,)))
            if m < PREFETCH:
                _start(w_copies(m + 1))
            look_ahead(m)
        lax.fori_loop(1, HP // 2, lambda i, c: head_pairs(i, 1, range(1, HP // 2), False), None)
        _wait(x_copies(1, R))
        lax.fori_loop(
            0, HP // 4,
            lambda i, c: head_pairs(HP // 2 + 2 * i, 2, range(HP // 2, HP, 2), True), None)

        mod_chunks(2, 6)
        _wait(wo_copies(0, ND))
        _start(mixer_copies)

        def set_lhs(mem, s, j):
            tok = pltpu.bitcast(seg_get(1 + s, 1, TOK + j * R // 2, 1, R // 2), BF16)
            head = jnp.concatenate([mem, tok[:16].astype(F32)[E:]], axis=0).astype(BF16)
            lhs[j] = jnp.concatenate([head, tok[16:]], axis=0)

        def finish_tokens(s, row):
            x1 = xs[s].astype(F32) + _rows(mod[2], SEG) * aout[...]
            h = _ln(x1) * _rows(1.0 + mod[4], SEG) + _rows(mod[3], SEG)
            seg_put(row, X1, x1)
            seg_put(row, HB, h)
            seg_put(row, HN, _ln(h).astype(BF16))

        for j in range(ND):
            set_lhs(mem0_ref[:, _lanes(j)].astype(F32), 0, j)
        aout[...] = jnp.zeros_like(aout)
        lhs_u = lhs.bitcast(U32)

        def step(s):
            G = HEAD_GROUP
            NG = H // G
            KH = (H - G) * LANES
            ri = lax.broadcasted_iota(jnp.int32, (L, LP), 0)
            ci = lax.broadcasted_iota(jnp.int32, (L, LP), 1)
            keep = ((ri < M) | (ri >= ci)) & (ci < L)
            fill = jnp.where(ci < L, MASKED, -jnp.inf).astype(F32)
            zpad = jnp.zeros((LP - L, LANES), F32)

            def project(h, m):
                p = 3 * h + m
                if h < G and m == 0:
                    y = acc[pl.ds(0, SEG), _lanes(h)] + _dot(
                        _panels(lhs_u, 0, ND // 2), _panel(wqkv, p, 0, D // 4))
                else:
                    y = _dot(_panels(lhs_u, 0, ND), _panel(wqkv, p))
                parts = [y[:M], seg[1 + s, p], y[M:]]
                if m == 0:
                    return jnp.concatenate(parts, axis=0)
                return jnp.concatenate(parts + [zpad], axis=0).astype(BF16)

            def probs(q, k):
                sc = jnp.where(keep, _dot_nt(q, k) * scale, fill)
                e = jnp.exp(sc - jnp.max(sc, axis=-1, keepdims=True))
                return e / jnp.sum(e, axis=-1, keepdims=True)

            for h in range(G):
                acc[pl.ds(0, SEG), _lanes(h)] = _dot(
                    _panels(lhs_u, ND // 2, ND // 2), _panel(wqkv, 3 * h, D // 4, D // 4))
            finish_tokens(jnp.maximum(s - 1, 0), s)
            prev = None
            for g in range(NG + 1):
                heads = range(g * G, (g + 1) * G) if g < NG else ()
                q = [project(h, 0) for h in heads]
                if prev is not None:
                    pr = [probs(a, b) for a, b in zip(prev[0], prev[1])]
                k = [project(h, 1) for h in heads]
                v = [project(h, 2) for h in heads]
                if g == NG:
                    for j in range(ND // 2):
                        acc[:, _lanes(j)] = _dot(obuf[:, pl.ds(0, KH)], _panel(wo, j, 0, KH // 2))
                if prev is not None:
                    for u in range(G):
                        obuf[:, _lanes((g - 1) * G + u)] = _dot(pr[u], prev[2][u])
                prev = (q, k, v)
            for j in reversed(range(ND)):
                if j < ND // 2:
                    y = acc[:, _lanes(j)] + _dot(
                        obuf[:, _lanes(H - G, G)], _panel(wo, j, KH // 2, G * LANES // 2))
                else:
                    y = _dot(obuf[...], _panel(wo, j))
                set_lhs(y[:M], jnp.minimum(s + 1, NSEG - 1), j)
                aout[:, _lanes(j)] = y[M:]

        def steps(i, carry):
            for u in range(UNROLL):
                step(i * UNROLL + u)

        lax.fori_loop(0, NSEG // UNROLL, steps, None)
        _wait(mixer_copies)
        finish_tokens(NSEG - 1, NSEG)

    pl.run_scoped(
        attention_phase,
        pltpu.VMEM((3 * H, D // 2, LANES), U32),
        pltpu.VMEM((ND, H * LANES // 2, LANES), U32),
        pltpu.VMEM((NSEG, SEG, D), BF16),
        pltpu.VMEM((NSEG * E, D), F32),
        pltpu.VMEM((ND, NSEG * E, LANES), BF16),
        pltpu.VMEM((ND, SEG, LANES), BF16),
        pltpu.VMEM((L, H * LANES), F32),
        pltpu.VMEM((SEG, D), F32),
        pltpu.VMEM((L, D), F32),
        pltpu.SemaphoreType.DMA((3 * H // 2,)),
        pltpu.SemaphoreType.DMA((2,)),
        pltpu.SemaphoreType.DMA(()),
    )

    def mixer_phase(gbuf, obuf, ops, sem_out):
        NT = S // TM
        TS = TM // SEG
        ops_u = ops.bitcast(U32)
        gbuf[:, pl.ds(0, 8), :] = jnp.zeros((ND, 8, LANES), F32)
        gbuf[:, pl.ds(S + 8, 8), :] = jnp.zeros((ND, 8, LANES), F32)

        def gate(t):
            for j in range(ND):
                a = pltpu.bitcast(seg_get(1 + t * TS, TS, HN, ND, R // 2), BF16)
                gbuf[j, pl.ds(pl.multiple_of(t * TM + 8, 8), TM), :] = jax.nn.gelu(
                    _dot(a, _panel(wb, j)), approximate=True)

        def mix(t):
            for j in range(ND):
                shifted = jnp.concatenate(
                    [gbuf[k, pl.ds(t * TM + 8 + (-1, 1, -2, 2)[4 * k // ND], TM), :]
                     for k in range(ND)], axis=1)
                y = seg_get(1 + t * TS, TS, HB + j * R, 1) + _dot(shifted, _panel(wb, ND + j))
                seg_put(1 + t * TS, HB + j * R, y, TS)

        def norm(t, u, when=lambda v: v):
            v = _ln(when(seg_get(1 + t * TS + u, 1, HB, ND))).astype(BF16)
            for j in range(ND):
                ops[j, pl.ds(u * SEG, SEG), :] = v[:, j * LANES:(j + 1) * LANES]

        def out_copy(t):
            r = pl.ds(pl.multiple_of(t * TM, TM), TM)
            return pltpu.make_async_copy(obuf.at[r], out_hbm.at[r], sem_out)

        def tile(t, pin, ahead):
            if ahead >= 2:
                gate(t + 2)
            for j in range(NF):
                ops[ND + j] = jax.nn.gelu(
                    _dot(_panels(ops_u, 0, ND), _panel(wb, 2 * ND + j)),
                    approximate=True).astype(BF16)
            if ahead >= 1:
                mix(t + 1)
            done = []
            for j in range(ND):
                if ahead >= 1 and 2 <= j < 2 + TS:
                    norm(t + 1, j - 2, lambda v: _after(pin, v, done[-2]))
                a = jnp.concatenate(
                    [_panel(ops_u, ND + pin), _panels(ops_u, ND + 1, NF - 1)], axis=1)
                y = seg_get(1 + t * TS, TS, HB + j * R, 1) + _dot(a, _panel(w4, j))
                done.append(y)
                y = seg_get(1 + t * TS, TS, X1 + j * R, 1) + _rows(mod[5, :, _lanes(j)], TM) * y
                obuf[pl.ds(pl.multiple_of(t * TM, TM), TM), _lanes(j)] = y.astype(BF16)
            out_copy(t).start()
            return pin

        gate(0)
        gate(1)
        mix(0)
        for u in range(TS):
            norm(0, u)
        pin = lax.fori_loop(0, NT - 2, lambda t, c: tile(t, _pin(t), 2), 0)
        tile(NT - 2, pin, 1)
        tile(NT - 1, pin, 0)
        _wait([out_copy(t) for t in range(NT)])

    pl.run_scoped(
        mixer_phase,
        pltpu.VMEM((ND, S + 16, LANES), F32),
        pltpu.VMEM((S, D), BF16),
        pltpu.VMEM((ND + NF, TM, LANES), BF16),
        pltpu.SemaphoreType.DMA(()))


@functools.partial(jax.jit, static_argnames=("A_seg_len",))
def pallas_adaLN_cond__memory_aug_recurrent_mem_tr__mixer_s_mlp__prompt_kernel(
    A_x, A_mem0, A_Wq, A_Wk, A_Wv, A_Wo, A_seg_len, B_x, B_w1, B_w2, B_w3, B_w4, c, w_mod,
):
    del B_x
    B, S, D = A_x.shape
    H, Dh = A_Wq.shape[1:]
    M = A_mem0.shape[1]
    F = B_w3.shape[1]
    SEG = A_seg_len
    assert (B, D, H, Dh, M, SEG) == (1, 1024, 32, LANES, 8, 32) and A_x.dtype == BF16
    assert S % (16 * SEG) == 0 and F % LANES == 0
    ND, NF = D // LANES, F // LANES
    hbm = pl.BlockSpec(memory_space=pl.ANY)
    vmem = pl.BlockSpec(memory_space=pltpu.VMEM)
    out = pl.pallas_call(
        functools.partial(_kernel, S=S, D=D, H=H, M=M, SEG=SEG, F=F),
        out_shape=jax.ShapeDtypeStruct((S, D), A_x.dtype),
        in_specs=[hbm, vmem, hbm, hbm, hbm, hbm, hbm, hbm, hbm, hbm, vmem, hbm],
        out_specs=hbm,
        scratch_shapes=[
            pltpu.VMEM((max(6 * ND, 2 * ND + NF), D // 2, LANES), U32),
            pltpu.VMEM((ND, F // 2, LANES), U32),
            pltpu.VMEM((S // SEG + 1, 3 * H + ND * SEG // 16, 8, LANES), F32),
            pltpu.VMEM((6, 8, D), F32),
            pltpu.SemaphoreType.DMA((6,)),
            pltpu.SemaphoreType.DMA(()),
        ],
        compiler_params=pltpu.CompilerParams(vmem_limit_bytes=110 * 1024 * 1024),
    )(A_x.reshape(S // SEG, SEG, D), A_mem0.reshape(M, D),
      *(w.reshape(D // 2, 2, H, Dh) for w in (A_Wq, A_Wk, A_Wv)),
      A_Wo.reshape(H * Dh, D), B_w1, B_w2, B_w3, B_w4, c, w_mod)
    return out.reshape(B, S, D)
```

```python
import functools

import jax
import jax.numpy as jnp
import numpy as np
from jax import lax
import jax.experimental.pallas as pl
import jax.experimental.pallas.tpu as pltpu

F32 = jnp.float32
BF16 = jnp.bfloat16
U32 = jnp.uint32
LANES = 128
EPS = 1e-5
MASKED = -1e9

HEAD_GROUP = 4
UNROLL = 3
PREFETCH = 3
TM = 128


def _ln(x):
    m = jnp.mean(x, axis=-1, keepdims=True)
    d = x - m
    v = jnp.mean(d * d, axis=-1, keepdims=True)
    return d * lax.rsqrt(v + EPS)


def _dot(a, b):
    return jnp.dot(a, b, preferred_element_type=F32)


def _dot_nt(a, b):
    return lax.dot_general(a, b, (((1,), (1,)), ((), ())), preferred_element_type=F32)


def _panel(ref, p, r0=None, nr=None):
    w = ref[p] if r0 is None else ref[p, pl.ds(r0, nr), :]
    return pltpu.bitcast(w, BF16)


def _panels(ref, p0, n):
    return jnp.concatenate([_panel(ref, p0 + j) for j in range(n)], axis=1)


def _pin(i):
    return i >> 24


def _after(pin, v, y):
    return jnp.where(pin == 0, v, jnp.concatenate([y[:v.shape[0]]] * (v.shape[1] // LANES), axis=1))


def _lanes(j, n=1):
    return pl.ds(j * LANES, n * LANES)


def _rows(v, n):
    return jnp.concatenate([v] * (n // 8), axis=0)


def _start(copies):
    for cp in copies:
        cp.start()


def _wait(copies):
    for cp in copies:
        cp.wait()


def _kernel(x_hbm, mem0_ref, wq_hbm, wk_hbm, wv_hbm, wo_hbm, w1_hbm, w2_hbm, w3_hbm, w4_hbm,
            c_ref, wmod_hbm, out_hbm,
            wb, w4, seg, mod, sem_mod, sem_b,
            *, S, D, H, M, SEG, F):
    NSEG = S // SEG
    E = M
    L = M + SEG
    LP = -(-L // 16) * 16
    ND = D // LANES
    NF = F // LANES
    R = SEG // 8
    scale = LANES ** -0.5
    TOK = 3 * H
    X1, HB, HN = 0, R * ND, 2 * R * ND

    def seg_put(row, slot, v, n=1):
        if v.dtype != F32:
            v = pltpu.bitcast(v, F32)
        r = v.shape[0] // (8 * n)
        for j in range(v.shape[1] // LANES):
            seg[pl.ds(row, n), pl.ds(slot + j * r, r)] = (
                v[:, j * LANES:(j + 1) * LANES].reshape(n, r, 8, LANES))

    def seg_get(row, n, slot, cols, r=R):
        return jnp.concatenate(
            [seg[pl.ds(row, n), pl.ds(slot + j * r, r)].reshape(n * r * 8, LANES)
             for j in range(cols)], axis=1)

    w_u = [r.bitcast(U32) for r in (wq_hbm, wk_hbm, wv_hbm)]
    wo_u, w1_u, w2_u, w3_u, w4_u, wmod_u = (
        r.bitcast(U32) for r in (wo_hbm, w1_hbm, w2_hbm, w3_hbm, w4_hbm, wmod_hbm))

    mixer_copies = [
        pltpu.make_async_copy(w.at[:, _lanes(j)], dst.at[p0 + j], sem_b)
        for w, dst, p0 in ((w1_u, wb, 0), (w2_u, wb, ND), (w3_u, wb, 2 * ND), (w4_u, w4, 0))
        for j in range(w.shape[1] // LANES)]

    def mod_copies(lo, hi):
        return [pltpu.make_async_copy(wmod_u.at[:, _lanes(j)], wb.at[j], sem_mod.at[j // ND])
                for j in range(lo, hi)]

    def cond():
        cv = c_ref[...].astype(F32)
        return jnp.broadcast_to(cv * jax.nn.sigmoid(cv), (8, D))

    def mod_chunk(i, arrived):
        sc = cond()
        _wait(mod_copies(i * ND, (i + 1) * ND))
        _start(arrived)
        for j in range(ND):
            mod[i, :, _lanes(j)] = _dot(sc, _panel(wb, i * ND + j))

    def attention_phase(wqkv, wo, xs, xn, he, lhs, obuf, aout, acc, sem_w, sem_x, sem_wo):
        HP = H // 2

        def w_copies(hp, which=(0, 1, 2)):
            return [pltpu.make_async_copy(w_u[m].at[:, i, hp, :], wqkv.at[6 * hp + 3 * i + m],
                                          sem_w.at[3 * hp + m]) for m in which for i in range(2)]

        def wo_copies(lo, hi):
            return [pltpu.make_async_copy(wo_u.at[:, _lanes(j)], wo.at[j], sem_wo)
                    for j in range(lo, hi)]

        def x_copies(lo, hi):
            return [pltpu.make_async_copy(x_hbm.at[:, pl.ds(i * E, E), :],
                                          xs.at[:, pl.ds(i * E, E), :], sem_x.at[min(i, 1)])
                    for i in range(lo, hi)]

        def modulate_a(n):
            return n * _rows(1.0 + mod[1], n.shape[0]) + _rows(mod[0], n.shape[0])

        _start(x_copies(0, 1) + mod_copies(0, ND // 2))
        _wait(x_copies(0, 1))
        _start(mod_copies(ND // 2, 2 * ND))

        def early_norm(t, carry):
            xv = xs[pl.ds(t * 16, 16), pl.ds(0, E), :].astype(F32).reshape(16 * E, D)
            xn[pl.ds(pl.multiple_of(t * 16 * E, 16 * E), 16 * E), :] = _ln(xv)
        lax.fori_loop(0, NSEG // 16, early_norm, None)

        mod_chunk(0, w_copies(0, (0,)))
        mod_chunk(1, w_copies(0, (1, 2)))
        hv = modulate_a(xn[...]).astype(BF16)
        for j in range(ND):
            he[j] = hv[:, j * LANES:(j + 1) * LANES]

        extra = ([(x_copies, i, i + 1) for i in range(1, R)]
                 + [(mod_copies, j, j + 4) for j in range(2 * ND, 6 * ND, 4)]
                 + [(wo_copies, j, j + 2) for j in range(0, ND, 2)])
        assert HP == 16 and PREFETCH == 3 and len(extra) < HP

        def look_ahead(p, small=None, side=None):
            a, b = wqkv[p], wqkv[p + 3]
            w = ((a & np.uint32(0xFFFF)) | (b << 16), (a >> 16) | (b & np.uint32(0xFFFF0000)))
            he_u = he.bitcast(U32)
            for u in range(2):
                wqkv[p + 3 * u] = w[u]
                wu = pltpu.bitcast(w[u], BF16)
                if small is None:
                    seg_put(1, p + 3 * u, _dot(_panels(he_u, 0, ND), wu), NSEG)
                    continue
                seg_put(1, p + 3 * u, _dot(_panels(he_u, 0, ND // 2), wu[:D // 2]), NSEG)
                small()
                y = seg_get(1, NSEG, p + 3 * u, 1, 1) + _dot(
                    _panels(he_u, ND // 2, ND // 2), wu[D // 2:])
                seg_put(1, p + 3 * u, y, NSEG)
                side(y)
                small()

        def fetch(hp0, pairs, starts):
            for v in range(pairs):
                @pl.when(hp0 + v + PREFETCH < HP)
                def _():
                    _start(w_copies(hp0 + v + PREFETCH))
            for k in starts:
                @pl.when(hp0 == k)
                def _():
                    for copies, lo, hi in extra[k - 1:k - 1 + pairs]:
                        _start(copies(lo, hi))
            for v in range(pairs):
                _wait(w_copies(hp0 + v))

        def one_pair(hp, carry):
            fetch(hp, 1, range(1, HP // 2))
            for m in range(3):
                look_ahead(6 * hp + m)

        def two_pairs(i, carry):
            hp0, pin = HP // 2 + 2 * i, _pin(i)
            fetch(hp0, 2, range(HP // 2, HP, 2))
            for k in range(4):
                @pl.when(i == k)
                def _():
                    _wait(mod_copies((2 + k) * ND, (3 + k) * ND))
            sc = cond()
            halves = [(j, h) for j in range(ND) for h in range(2)]

            def mod_half():
                if halves:
                    j, h = halves.pop(0)
                    y = _dot(sc[:, h * D // 2:(h + 1) * D // 2],
                             _panel(wb, (2 + i) * ND + j, h * D // 4, D // 4))
                    if h:
                        y = y + seg[pin, j]
                        mod[2 + i, :, _lanes(j)] = y
                    seg[pin, j] = y

            n = NSEG // 8
            for v in range(2):
                todo = list(range(n))

                def modulate_tokens(y):
                    for k in todo[:-(-n // 5)]:
                        s = (2 * i + v) * n + k
                        xv = _after(pin, xs[s].astype(F32), y)
                        seg_put(1 + s, TOK, modulate_a(_ln(xv)).astype(BF16))
                    del todo[:-(-n // 5)]

                for m in range(3):
                    look_ahead(6 * (hp0 + v) + m, mod_half, modulate_tokens)

        for m in range(3):
            _wait(w_copies(0, (m,)))
            _start(w_copies(m + 1))
            look_ahead(m)
        lax.fori_loop(1, HP // 2, one_pair, None)
        _wait(x_copies(1, R))
        lax.fori_loop(0, 4, two_pairs, None)

        _wait(wo_copies(0, ND))
        _start(mixer_copies)

        def set_lhs(mem, s, j):
            tok = pltpu.bitcast(seg_get(1 + s, 1, TOK + j * R // 2, 1, R // 2), BF16)
            head = jnp.concatenate([mem, tok[:16].astype(F32)[E:]], axis=0).astype(BF16)
            lhs[j] = jnp.concatenate([head, tok[16:]], axis=0)

        def finish_tokens(s, row):
            x1 = xs[s].astype(F32) + _rows(mod[2], SEG) * aout[...]
            h = _ln(x1) * _rows(1.0 + mod[4], SEG) + _rows(mod[3], SEG)
            seg_put(row, X1, x1)
            seg_put(row, HB, h)
            seg_put(row, HN, _ln(h).astype(BF16))

        for j in range(ND):
            set_lhs(mem0_ref[:, _lanes(j)].astype(F32), 0, j)
        aout[...] = jnp.zeros_like(aout)
        lhs_u = lhs.bitcast(U32)

        def step(s):
            G = HEAD_GROUP
            NG = H // G
            KH = (H - G) * LANES
            ri = lax.broadcasted_iota(jnp.int32, (L, LP), 0)
            ci = lax.broadcasted_iota(jnp.int32, (L, LP), 1)
            keep = ((ri < M) | (ri >= ci)) & (ci < L)
            fill = jnp.where(ci < L, MASKED, -jnp.inf).astype(F32)
            zpad = jnp.zeros((LP - L, LANES), F32)

            def project(h, m):
                p = 3 * h + m
                if h < G and m == 0:
                    y = acc[pl.ds(0, SEG), _lanes(h)] + _dot(
                        _panels(lhs_u, 0, ND // 2), _panel(wqkv, p, 0, D // 4))
                else:
                    y = _dot(_panels(lhs_u, 0, ND), _panel(wqkv, p))
                parts = [y[:M], seg[1 + s, p], y[M:]]
                if m == 0:
                    return jnp.concatenate(parts, axis=0)
                return jnp.concatenate(parts + [zpad], axis=0).astype(BF16)

            def probs(q, k):
                sc = jnp.where(keep, _dot_nt(q, k) * scale, fill)
                e = jnp.exp(sc - jnp.max(sc, axis=-1, keepdims=True))
                return e / jnp.sum(e, axis=-1, keepdims=True)

            for h in range(G):
                acc[pl.ds(0, SEG), _lanes(h)] = _dot(
                    _panels(lhs_u, ND // 2, ND // 2), _panel(wqkv, 3 * h, D // 4, D // 4))
            finish_tokens(jnp.maximum(s - 1, 0), s)
            prev = None
            for g in range(NG + 1):
                heads = range(g * G, (g + 1) * G) if g < NG else ()
                q = [project(h, 0) for h in heads]
                if prev is not None:
                    pr = [probs(a, b) for a, b in zip(prev[0], prev[1])]
                k = [project(h, 1) for h in heads]
                v = [project(h, 2) for h in heads]
                if g == NG:
                    for j in range(ND // 2):
                        acc[:, _lanes(j)] = _dot(obuf[:, pl.ds(0, KH)], _panel(wo, j, 0, KH // 2))
                if prev is not None:
                    for u in range(G):
                        obuf[:, _lanes((g - 1) * G + u)] = _dot(pr[u], prev[2][u])
                prev = (q, k, v)
            for j in reversed(range(ND)):
                if j < ND // 2:
                    y = acc[:, _lanes(j)] + _dot(
                        obuf[:, _lanes(H - G, G)], _panel(wo, j, KH // 2, G * LANES // 2))
                else:
                    y = _dot(obuf[...], _panel(wo, j))
                set_lhs(y[:M], jnp.minimum(s + 1, NSEG - 1), j)
                aout[:, _lanes(j)] = y[M:]

        def steps(i, carry):
            for u in range(UNROLL):
                step(i * UNROLL + u)

        lax.fori_loop(0, NSEG // UNROLL, steps, None)
        for s in range(NSEG // UNROLL * UNROLL, NSEG):
            step(s)
        _wait(mixer_copies)
        finish_tokens(NSEG - 1, NSEG)

    pl.run_scoped(
        attention_phase,
        pltpu.VMEM((3 * H, D // 2, LANES), U32),
        pltpu.VMEM((ND, H * LANES // 2, LANES), U32),
        pltpu.VMEM((NSEG, SEG, D), BF16),
        pltpu.VMEM((NSEG * E, D), F32),
        pltpu.VMEM((ND, NSEG * E, LANES), BF16),
        pltpu.VMEM((ND, SEG, LANES), BF16),
        pltpu.VMEM((L, H * LANES), F32),
        pltpu.VMEM((SEG, D), F32),
        pltpu.VMEM((L, D), F32),
        pltpu.SemaphoreType.DMA((3 * H // 2,)),
        pltpu.SemaphoreType.DMA((2,)),
        pltpu.SemaphoreType.DMA(()),
    )

    def mixer_phase(gbuf, obuf, ops, sem_out):
        NT = S // TM
        TS = TM // SEG
        ops_u = ops.bitcast(U32)
        gbuf[:, pl.ds(0, 8), :] = jnp.zeros((ND, 8, LANES), F32)
        gbuf[:, pl.ds(S + 8, 8), :] = jnp.zeros((ND, 8, LANES), F32)

        def gate(t):
            for j in range(ND):
                a = pltpu.bitcast(seg_get(1 + t * TS, TS, HN, ND, R // 2), BF16)
                gbuf[j, pl.ds(pl.multiple_of(t * TM + 8, 8), TM), :] = jax.nn.gelu(
                    _dot(a, _panel(wb, j)), approximate=True)

        def mix(t):
            for j in range(ND):
                shifted = jnp.concatenate(
                    [gbuf[k, pl.ds(t * TM + 8 + (-1, 1, -2, 2)[4 * k // ND], TM), :]
                     for k in range(ND)], axis=1)
                y = seg_get(1 + t * TS, TS, HB + j * R, 1) + _dot(shifted, _panel(wb, ND + j))
                seg_put(1 + t * TS, HB + j * R, y, TS)

        def norm(t, u, when=lambda v: v):
            v = _ln(when(seg_get(1 + t * TS + u, 1, HB, ND))).astype(BF16)
            for j in range(ND):
                ops[j, pl.ds(u * SEG, SEG), :] = v[:, j * LANES:(j + 1) * LANES]

        def out_copy(t):
            r = pl.ds(pl.multiple_of(t * TM, TM), TM)
            return pltpu.make_async_copy(obuf.at[r], out_hbm.at[r], sem_out)

        def tile(t, pin, ahead):
            if ahead >= 2:
                gate(t + 2)
            for j in range(NF):
                ops[ND + j] = jax.nn.gelu(
                    _dot(_panels(ops_u, 0, ND), _panel(wb, 2 * ND + j)),
                    approximate=True).astype(BF16)
            if ahead >= 1:
                mix(t + 1)
            done = []
            for j in range(ND):
                if ahead >= 1 and 2 <= j < 2 + TS:
                    norm(t + 1, j - 2, lambda v: _after(pin, v, done[-2]))
                a = jnp.concatenate(
                    [_panel(ops_u, ND + pin), _panels(ops_u, ND + 1, NF - 1)], axis=1)
                y = seg_get(1 + t * TS, TS, HB + j * R, 1) + _dot(a, _panel(w4, j))
                done.append(y)
                y = seg_get(1 + t * TS, TS, X1 + j * R, 1) + _rows(mod[5, :, _lanes(j)], TM) * y
                obuf[pl.ds(pl.multiple_of(t * TM, TM), TM), _lanes(j)] = y.astype(BF16)
            out_copy(t).start()
            return pin

        gate(0)
        gate(1)
        mix(0)
        for u in range(TS):
            norm(0, u)
        pin = lax.fori_loop(0, NT - 2, lambda t, c: tile(t, _pin(t), 2), 0)
        tile(NT - 2, pin, 1)
        tile(NT - 1, pin, 0)
        _wait([out_copy(t) for t in range(NT)])

    pl.run_scoped(
        mixer_phase,
        pltpu.VMEM((ND, S + 16, LANES), F32),
        pltpu.VMEM((S, D), BF16),
        pltpu.VMEM((ND + NF, TM, LANES), BF16),
        pltpu.SemaphoreType.DMA(()))


@functools.partial(jax.jit, static_argnames=("A_seg_len",))
def pallas_adaLN_cond__memory_aug_recurrent_mem_tr__mixer_s_mlp__prompt_kernel(
    A_x, A_mem0, A_Wq, A_Wk, A_Wv, A_Wo, A_seg_len, B_x, B_w1, B_w2, B_w3, B_w4, c, w_mod,
):
    del B_x
    B, S, D = A_x.shape
    H, Dh = A_Wq.shape[1:]
    M = A_mem0.shape[1]
    F = B_w3.shape[1]
    SEG = A_seg_len
    assert (B, D, H, Dh, M, SEG) == (1, 1024, 32, LANES, 8, 32) and A_x.dtype == BF16
    assert S % (16 * SEG) == 0 and F % LANES == 0
    ND, NF = D // LANES, F // LANES
    hbm = pl.BlockSpec(memory_space=pl.ANY)
    vmem = pl.BlockSpec(memory_space=pltpu.VMEM)
    out = pl.pallas_call(
        functools.partial(_kernel, S=S, D=D, H=H, M=M, SEG=SEG, F=F),
        out_shape=jax.ShapeDtypeStruct((S, D), A_x.dtype),
        in_specs=[hbm, vmem, hbm, hbm, hbm, hbm, hbm, hbm, hbm, hbm, vmem, hbm],
        out_specs=hbm,
        scratch_shapes=[
            pltpu.VMEM((max(6 * ND, 2 * ND + NF), D // 2, LANES), U32),
            pltpu.VMEM((ND, F // 2, LANES), U32),
            pltpu.VMEM((S // SEG + 1, 3 * H + ND * SEG // 16, 8, LANES), F32),
            pltpu.VMEM((6, 8, D), F32),
            pltpu.SemaphoreType.DMA((6,)),
            pltpu.SemaphoreType.DMA(()),
        ],
        compiler_params=pltpu.CompilerParams(vmem_limit_bytes=110 * 1024 * 1024),
    )(A_x.reshape(S // SEG, SEG, D), A_mem0.reshape(M, D),
      *(w.reshape(D // 2, 2, H, Dh) for w in (A_Wq, A_Wk, A_Wv)),
      A_Wo.reshape(H * Dh, D), B_w1, B_w2, B_w3, B_w4, c, w_mod)
    return out.reshape(B, S, D)
```

```python
import functools

import jax
import jax.numpy as jnp
import numpy as np
from jax import lax
import jax.experimental.pallas as pl
import jax.experimental.pallas.tpu as pltpu

F32 = jnp.float32
BF16 = jnp.bfloat16
U32 = jnp.uint32
LANES = 128
EPS = 1e-5
MASKED = -1e9

HEAD_GROUP = 4
UNROLL = 3
PREFETCH = 3
TM = 128


def _ln(x):
    m = jnp.mean(x, axis=-1, keepdims=True)
    d = x - m
    v = jnp.mean(d * d, axis=-1, keepdims=True)
    return d * lax.rsqrt(v + EPS)


def _inverse(z):
    r = (pltpu if hasattr(pltpu, "reciprocal") else pl).reciprocal(z, approx=True)
    return r + r * (1.0 - z * r)


def _dot(a, b):
    return jnp.dot(a, b, preferred_element_type=F32)


def _dot_nt(a, b):
    return lax.dot_general(a, b, (((1,), (1,)), ((), ())), preferred_element_type=F32)


def _panel(ref, p, r0=None, nr=None):
    w = ref[p] if r0 is None else ref[p, pl.ds(r0, nr), :]
    return pltpu.bitcast(w, BF16)


def _panels(ref, p0, n):
    return jnp.concatenate([_panel(ref, p0 + j) for j in range(n)], axis=1)


def _pin(i):
    return i >> 24


def _after(pin, v, y):
    return jnp.where(pin == 0, v, jnp.concatenate([y[:v.shape[0]]] * (v.shape[1] // LANES), axis=1))


def _lanes(j, n=1):
    return pl.ds(j * LANES, n * LANES)


def _rows(v, n):
    return jnp.concatenate([v] * (n // 8), axis=0)


def _start(copies):
    for cp in copies:
        cp.start()


def _wait(copies):
    for cp in copies:
        cp.wait()


def _kernel(x_hbm, mem0_ref, wq_hbm, wk_hbm, wv_hbm, wo_hbm, w1_hbm, w2_hbm, w3_hbm, w4_hbm,
            c_ref, wmod_hbm, out_hbm,
            wb, w4, seg, mod, sem_mod, sem_b,
            *, S, D, H, M, SEG, F):
    NSEG = S // SEG
    E = M
    L = M + SEG
    LP = -(-L // 16) * 16
    ND = D // LANES
    NF = F // LANES
    R = SEG // 8
    scale = LANES ** -0.5
    TOK = 3 * H
    X1, HB, HN = 0, R * ND, 2 * R * ND

    def seg_put(row, slot, v, n=1):
        if v.dtype != F32:
            v = pltpu.bitcast(v, F32)
        r = v.shape[0] // (8 * n)
        for j in range(v.shape[1] // LANES):
            seg[pl.ds(row, n), pl.ds(slot + j * r, r)] = (
                v[:, j * LANES:(j + 1) * LANES].reshape(n, r, 8, LANES))

    def seg_get(row, n, slot, cols, r=R):
        return jnp.concatenate(
            [seg[pl.ds(row, n), pl.ds(slot + j * r, r)].reshape(n * r * 8, LANES)
             for j in range(cols)], axis=1)

    w_u = [r.bitcast(U32) for r in (wq_hbm, wk_hbm, wv_hbm)]
    wo_u, w1_u, w2_u, w3_u, w4_u, wmod_u = (
        r.bitcast(U32) for r in (wo_hbm, w1_hbm, w2_hbm, w3_hbm, w4_hbm, wmod_hbm))

    mixer_copies = [
        pltpu.make_async_copy(w.at[:, _lanes(j)], dst.at[p0 + j], sem_b)
        for w, dst, p0 in ((w1_u, wb, 0), (w2_u, wb, ND), (w3_u, wb, 2 * ND), (w4_u, w4, 0))
        for j in range(w.shape[1] // LANES)]

    def mod_copies(lo, hi):
        return [pltpu.make_async_copy(wmod_u.at[:, _lanes(j)], wb.at[j], sem_mod.at[j // ND])
                for j in range(lo, hi)]

    def cond():
        cv = c_ref[...].astype(F32)
        return jnp.broadcast_to(cv * jax.nn.sigmoid(cv), (8, D))

    def mod_chunk(i, arrived):
        sc = cond()
        _wait(mod_copies(i * ND, (i + 1) * ND))
        _start(arrived)
        for j in range(ND):
            mod[i, :, _lanes(j)] = _dot(sc, _panel(wb, i * ND + j))

    def attention_phase(wqkv, wo, xs, xn, he, lhs, obuf, aout, acc, sem_w, sem_x, sem_wo):
        HP = H // 2

        def w_copies(hp, which=(0, 1, 2)):
            return [pltpu.make_async_copy(w_u[m].at[:, i, hp, :], wqkv.at[6 * hp + 3 * i + m],
                                          sem_w.at[3 * hp + m]) for m in which for i in range(2)]

        def wo_copies(lo, hi):
            return [pltpu.make_async_copy(wo_u.at[:, _lanes(j)], wo.at[j], sem_wo)
                    for j in range(lo, hi)]

        def x_copies(lo, hi):
            return [pltpu.make_async_copy(x_hbm.at[:, pl.ds(i * E, E), :],
                                          xs.at[:, pl.ds(i * E, E), :], sem_x.at[min(i, 1)])
                    for i in range(lo, hi)]

        def modulate_a(n):
            return n * _rows(1.0 + mod[1], n.shape[0]) + _rows(mod[0], n.shape[0])

        _start(x_copies(0, 1) + mod_copies(0, ND // 2))
        _wait(x_copies(0, 1))
        _start(mod_copies(ND // 2, 2 * ND))

        def early_norm(t, carry):
            xv = xs[pl.ds(t * 16, 16), pl.ds(0, E), :].astype(F32).reshape(16 * E, D)
            xn[pl.ds(pl.multiple_of(t * 16 * E, 16 * E), 16 * E), :] = _ln(xv)
        lax.fori_loop(0, NSEG // 16, early_norm, None)

        mod_chunk(0, w_copies(0, (0,)))
        mod_chunk(1, w_copies(0, (1, 2)))
        hv = modulate_a(xn[...]).astype(BF16)
        for j in range(ND):
            he[j] = hv[:, j * LANES:(j + 1) * LANES]

        extra = ([(x_copies, i, i + 1) for i in range(1, R)]
                 + [(mod_copies, j, j + 4) for j in range(2 * ND, 6 * ND, 4)]
                 + [(wo_copies, j, j + 2) for j in range(0, ND, 2)])
        assert HP == 16 and PREFETCH == 3 and len(extra) < HP

        def look_ahead(p, small=None, side=None):
            a, b = wqkv[p], wqkv[p + 3]
            w = ((a & np.uint32(0xFFFF)) | (b << 16), (a >> 16) | (b & np.uint32(0xFFFF0000)))
            he_u = he.bitcast(U32)
            for u in range(2):
                wqkv[p + 3 * u] = w[u]
                wu = pltpu.bitcast(w[u], BF16)
                if small is None:
                    seg_put(1, p + 3 * u, _dot(_panels(he_u, 0, ND), wu), NSEG)
                    continue
                seg_put(1, p + 3 * u, _dot(_panels(he_u, 0, ND // 2), wu[:D // 2]), NSEG)
                small()
                y = seg_get(1, NSEG, p + 3 * u, 1, 1) + _dot(
                    _panels(he_u, ND // 2, ND // 2), wu[D // 2:])
                seg_put(1, p + 3 * u, y, NSEG)
                side(y)
                small()

        def fetch(hp0, pairs, starts):
            for v in range(pairs):
                @pl.when(hp0 + v + PREFETCH < HP)
                def _():
                    _start(w_copies(hp0 + v + PREFETCH))
            for k in starts:
                @pl.when(hp0 == k)
                def _():
                    for copies, lo, hi in extra[k - 1:k - 1 + pairs]:
                        _start(copies(lo, hi))
            for v in range(pairs):
                _wait(w_copies(hp0 + v))

        def one_pair(hp, carry):
            fetch(hp, 1, range(1, HP // 2))
            for m in range(3):
                look_ahead(6 * hp + m)

        def two_pairs(i, carry):
            hp0, pin = HP // 2 + 2 * i, _pin(i)
            fetch(hp0, 2, range(HP // 2, HP, 2))
            for k in range(4):
                @pl.when(i == k)
                def _():
                    _wait(mod_copies((2 + k) * ND, (3 + k) * ND))
            sc = cond()
            halves = [(j, h) for j in range(ND) for h in range(2)]

            def mod_half():
                if halves:
                    j, h = halves.pop(0)
                    y = _dot(sc[:, h * D // 2:(h + 1) * D // 2],
                             _panel(wb, (2 + i) * ND + j, h * D // 4, D // 4))
                    if h:
                        y = y + seg[pin, j]
                        mod[2 + i, :, _lanes(j)] = y
                    seg[pin, j] = y

            n = NSEG // 8
            for v in range(2):
                todo = list(range(n))

                def modulate_tokens(y):
                    for k in todo[:-(-n // 5)]:
                        s = (2 * i + v) * n + k
                        xv = _after(pin, xs[s].astype(F32), y)
                        seg_put(1 + s, TOK, modulate_a(_ln(xv)).astype(BF16))
                    del todo[:-(-n // 5)]

                for m in range(3):
                    look_ahead(6 * (hp0 + v) + m, mod_half, modulate_tokens)

        for m in range(3):
            _wait(w_copies(0, (m,)))
            _start(w_copies(m + 1))
            look_ahead(m)
        lax.fori_loop(1, HP // 2, one_pair, None)
        _wait(x_copies(1, R))
        lax.fori_loop(0, 4, two_pairs, None)

        _wait(wo_copies(0, ND))
        _start(mixer_copies)

        def set_lhs(mem, s, j):
            tok = pltpu.bitcast(seg_get(1 + s, 1, TOK + j * R // 2, 1, R // 2), BF16)
            head = jnp.concatenate([mem, tok[:16].astype(F32)[E:]], axis=0).astype(BF16)
            lhs[j] = jnp.concatenate([head, tok[16:]], axis=0)

        def finish_tokens(s, row):
            x1 = xs[s].astype(F32) + _rows(mod[2], SEG) * aout[...]
            h = _ln(x1) * _rows(1.0 + mod[4], SEG) + _rows(mod[3], SEG)
            seg_put(row, X1, x1)
            seg_put(row, HB, h)
            seg_put(row, HN, _ln(h))

        for j in range(ND):
            set_lhs(mem0_ref[:, _lanes(j)].astype(F32), 0, j)
        aout[...] = jnp.zeros_like(aout)
        lhs_u = lhs.bitcast(U32)

        def step(s):
            G = HEAD_GROUP
            NG = H // G
            KH = (H - G) * LANES
            ri = lax.broadcasted_iota(jnp.int32, (L, LP), 0)
            ci = lax.broadcasted_iota(jnp.int32, (L, LP), 1)
            keep = ((ri < M) | (ri >= ci)) & (ci < L)
            fill = jnp.where(ci < L, MASKED, -jnp.inf).astype(F32)
            zpad = jnp.zeros((LP - L, LANES), F32)

            def project(h, m):
                p = 3 * h + m
                if h < G and m == 0:
                    y = acc[pl.ds(0, SEG), _lanes(h)] + _dot(
                        _panels(lhs_u, 0, ND // 2), _panel(wqkv, p, 0, D // 4))
                else:
                    y = _dot(_panels(lhs_u, 0, ND), _panel(wqkv, p))
                parts = [y[:M], seg[1 + s, p], y[M:]]
                if m == 0:
                    return jnp.concatenate(parts, axis=0)
                return jnp.concatenate(parts + [zpad], axis=0).astype(BF16)

            def probs(q, k):
                sc = jnp.where(keep, _dot_nt(q, k) * scale, fill)
                e = jnp.exp(sc - jnp.max(sc, axis=-1, keepdims=True))
                return e * _inverse(jnp.sum(e, axis=-1, keepdims=True))

            for h in range(G):
                acc[pl.ds(0, SEG), _lanes(h)] = _dot(
                    _panels(lhs_u, ND // 2, ND // 2), _panel(wqkv, 3 * h, D // 4, D // 4))
            finish_tokens(jnp.maximum(s - 1, 0), s)
            prev = None
            for g in range(NG + 1):
                heads = range(g * G, (g + 1) * G) if g < NG else ()
                q = [project(h, 0) for h in heads]
                if prev is not None:
                    pr = [probs(a, b) for a, b in zip(prev[0], prev[1])]
                k = [project(h, 1) for h in heads]
                v = [project(h, 2) for h in heads]
                if g == NG:
                    for j in range(ND // 2):
                        acc[:, _lanes(j)] = _dot(obuf[:, pl.ds(0, KH)], _panel(wo, j, 0, KH // 2))
                if prev is not None:
                    for u in range(G):
                        obuf[:, _lanes((g - 1) * G + u)] = _dot(pr[u], prev[2][u])
                prev = (q, k, v)
            for j in reversed(range(ND)):
                if j < ND // 2:
                    y = acc[:, _lanes(j)] + _dot(
                        obuf[:, _lanes(H - G, G)], _panel(wo, j, KH // 2, G * LANES // 2))
                else:
                    y = _dot(obuf[...], _panel(wo, j))
                set_lhs(y[:M], jnp.minimum(s + 1, NSEG - 1), j)
                aout[:, _lanes(j)] = y[M:]

        def steps(i, carry):
            for u in range(UNROLL):
                step(i * UNROLL + u)

        lax.fori_loop(0, NSEG // UNROLL, steps, None)
        for s in range(NSEG // UNROLL * UNROLL, NSEG):
            step(s)
        _wait(mixer_copies)
        finish_tokens(NSEG - 1, NSEG)

    pl.run_scoped(
        attention_phase,
        pltpu.VMEM((3 * H, D // 2, LANES), U32),
        pltpu.VMEM((ND, H * LANES // 2, LANES), U32),
        pltpu.VMEM((NSEG, SEG, D), BF16),
        pltpu.VMEM((NSEG * E, D), F32),
        pltpu.VMEM((ND, NSEG * E, LANES), BF16),
        pltpu.VMEM((ND, SEG, LANES), BF16),
        pltpu.VMEM((L, H * LANES), F32),
        pltpu.VMEM((SEG, D), F32),
        pltpu.VMEM((L, D), F32),
        pltpu.SemaphoreType.DMA((3 * H // 2,)),
        pltpu.SemaphoreType.DMA((2,)),
        pltpu.SemaphoreType.DMA(()),
    )

    def mixer_phase(gbuf, obuf, ops, sem_out):
        NT = S // TM
        TS = TM // SEG
        ops_u = ops.bitcast(U32)
        gbuf[:, pl.ds(0, 8), :] = jnp.zeros((ND, 8, LANES), F32)
        gbuf[:, pl.ds(S + 8, 8), :] = jnp.zeros((ND, 8, LANES), F32)

        def gate(t):
            for j in range(ND):
                a = seg_get(1 + t * TS, TS, HN, ND)
                gbuf[j, pl.ds(pl.multiple_of(t * TM + 8, 8), TM), :] = jax.nn.gelu(
                    _dot(a, _panel(wb, j)), approximate=True)

        def mix(t):
            for j in range(ND):
                shifted = jnp.concatenate(
                    [gbuf[k, pl.ds(t * TM + 8 + (-1, 1, -2, 2)[4 * k // ND], TM), :]
                     for k in range(ND)], axis=1)
                y = seg_get(1 + t * TS, TS, HB + j * R, 1) + _dot(shifted, _panel(wb, ND + j))
                seg_put(1 + t * TS, HB + j * R, y, TS)

        def norm(t, u, when=lambda v: v):
            v = _ln(when(seg_get(1 + t * TS + u, 1, HB, ND))).astype(BF16)
            for j in range(ND):
                ops[j, pl.ds(u * SEG, SEG), :] = v[:, j * LANES:(j + 1) * LANES]

        def out_copy(t):
            r = pl.ds(pl.multiple_of(t * TM, TM), TM)
            return pltpu.make_async_copy(obuf.at[r], out_hbm.at[r], sem_out)

        def tile(t, pin, ahead):
            if ahead >= 2:
                gate(t + 2)
            for j in range(NF):
                ops[ND + j] = jax.nn.gelu(
                    _dot(_panels(ops_u, 0, ND), _panel(wb, 2 * ND + j)),
                    approximate=True).astype(BF16)
            if ahead >= 1:
                mix(t + 1)
            done = []
            for j in range(ND):
                if ahead >= 1 and 2 <= j < 2 + TS:
                    norm(t + 1, j - 2, lambda v: _after(pin, v, done[-2]))
                a = jnp.concatenate(
                    [_panel(ops_u, ND + pin), _panels(ops_u, ND + 1, NF - 1)], axis=1)
                y = seg_get(1 + t * TS, TS, HB + j * R, 1) + _dot(a, _panel(w4, j))
                done.append(y)
                y = seg_get(1 + t * TS, TS, X1 + j * R, 1) + _rows(mod[5, :, _lanes(j)], TM) * y
                obuf[pl.ds(pl.multiple_of(t * TM, TM), TM), _lanes(j)] = y.astype(BF16)
            out_copy(t).start()
            return pin

        gate(0)
        gate(1)
        mix(0)
        for u in range(TS):
            norm(0, u)
        pin = lax.fori_loop(0, NT - 2, lambda t, c: tile(t, _pin(t), 2), 0)
        tile(NT - 2, pin, 1)
        tile(NT - 1, pin, 0)
        _wait([out_copy(t) for t in range(NT)])

    pl.run_scoped(
        mixer_phase,
        pltpu.VMEM((ND, S + 16, LANES), F32),
        pltpu.VMEM((S, D), BF16),
        pltpu.VMEM((ND + NF, TM, LANES), BF16),
        pltpu.SemaphoreType.DMA(()))


@functools.partial(jax.jit, static_argnames=("A_seg_len",))
def pallas_adaLN_cond__memory_aug_recurrent_mem_tr__mixer_s_mlp__prompt_kernel(
    A_x, A_mem0, A_Wq, A_Wk, A_Wv, A_Wo, A_seg_len, B_x, B_w1, B_w2, B_w3, B_w4, c, w_mod,
):
    del B_x
    B, S, D = A_x.shape
    H, Dh = A_Wq.shape[1:]
    M = A_mem0.shape[1]
    F = B_w3.shape[1]
    SEG = A_seg_len
    assert (B, D, H, Dh, M, SEG) == (1, 1024, 32, LANES, 8, 32) and A_x.dtype == BF16
    assert S % (16 * SEG) == 0 and F % LANES == 0
    ND, NF = D // LANES, F // LANES
    hbm = pl.BlockSpec(memory_space=pl.ANY)
    vmem = pl.BlockSpec(memory_space=pltpu.VMEM)
    out = pl.pallas_call(
        functools.partial(_kernel, S=S, D=D, H=H, M=M, SEG=SEG, F=F),
        out_shape=jax.ShapeDtypeStruct((S, D), A_x.dtype),
        in_specs=[hbm, vmem, hbm, hbm, hbm, hbm, hbm, hbm, hbm, hbm, vmem, hbm],
        out_specs=hbm,
        scratch_shapes=[
            pltpu.VMEM((max(6 * ND, 2 * ND + NF), D // 2, LANES), U32),
            pltpu.VMEM((ND, F // 2, LANES), U32),
            pltpu.VMEM((S // SEG + 1, 3 * H + ND * SEG // 16, 8, LANES), F32),
            pltpu.VMEM((6, 8, D), F32),
            pltpu.SemaphoreType.DMA((6,)),
            pltpu.SemaphoreType.DMA(()),
        ],
        compiler_params=pltpu.CompilerParams(vmem_limit_bytes=110 * 1024 * 1024),
    )(A_x.reshape(S // SEG, SEG, D), A_mem0.reshape(M, D),
      *(w.reshape(D // 2, 2, H, Dh) for w in (A_Wq, A_Wk, A_Wv)),
      A_Wo.reshape(H * Dh, D), B_w1, B_w2, B_w3, B_w4, c, w_mod)
    return out.reshape(B, S, D)
```
